```python
import jax
import jax.numpy as jnp

def _softmax(x, axis=-1):
    return jax.nn.softmax(x, axis=axis)

def _gelu(x):
    return jax.nn.gelu(x, approximate=True)

def _silu(x):
    return jax.nn.silu(x)

def _sigmoid(x):
    return jax.nn.sigmoid(x)

def _layernorm(x, axis=-1, eps=1e-05):
    m = jnp.mean(x, axis=axis, keepdims=True)
    v = jnp.var(x, axis=axis, keepdims=True)
    return (x - m) / jnp.sqrt(v + eps)

def _scatter_add(tgt, idx, src, axis=0):
    return tgt.at[idx].add(src)

def _segment_sum(src, seg, n):
    return jax.ops.segment_sum(src, seg, n)

class _Rng:

    def __init__(self, key):
        self._k = key

    def _next(self):
        self._k, sub = jax.random.split(self._k)
        return sub

    def normal(self, shape):
        return jax.random.normal(self._next(), shape, dtype=jnp.bfloat16)

    def randint(self, lo, hi, shape):
        return jax.random.randint(self._next(), shape, lo, hi, dtype=jnp.int32)

    def uniform(self, shape, lo=0.0, hi=1.0):
        return jax.random.uniform(self._next(), shape, jnp.bfloat16, lo, hi)

    def permutation(self, n):
        return jax.random.permutation(self._next(), n)
kernel_name = 'concat_heads__memory_aug_recurrent_mem_tr__compressed_kv_cla__prompt'

def setup_inputs():
    _rng = _Rng(jax.random.key(int.from_bytes(__import__("os").urandom(4), "little")))
    _w = lambda a: (lambda t: t.astype(jnp.bfloat16) if jnp.issubdtype(t.dtype, jnp.floating) else t)(jnp.asarray(a))

    def _A_setup():
        B, S, Dm = (1, 2048, 448)
        H, Dh = (16, 256)
        M, seg = (8, 32)
        seg = min(seg, S)
        S = S // seg * seg
        return {'x': _w((lambda *s: _rng.normal(s) * 0.05)(B, S, Dm)), 'mem0': _w((lambda *s: _rng.normal(s) * 0.05)(B, M, Dm)), 'Wq': _w((lambda *s: _rng.normal(s) * 0.05)(Dm, H, Dh) * Dm ** (-0.5)), 'Wk': _w((lambda *s: _rng.normal(s) * 0.05)(Dm, H, Dh) * Dm ** (-0.5)), 'Wv': _w((lambda *s: _rng.normal(s) * 0.05)(Dm, H, Dh) * Dm ** (-0.5)), 'Wo': _w((lambda *s: _rng.normal(s) * 0.05)(H, Dh, Dm) * (H * Dh) ** (-0.5)), 'seg_len': seg}
    _A_in = _A_setup()

    def _B_setup():
        B, H, Sq, Sk, D, M = (1, 16, 2048, 2048, 256, 448)
        Dc = 4 * D
        return {'x': _w((lambda *s: _rng.normal(s) * 0.05)(B, Sq, M)), 'c_kv': _w((lambda *s: _rng.normal(s) * 0.05)(B, Sk, Dc)), 'w_q': _w((lambda *s: _rng.normal(s) * 0.05)(M, H, D) * M ** (-0.5)), 'w_uk': _w((lambda *s: _rng.normal(s) * 0.05)(Dc, H, D) * Dc ** (-0.5)), 'w_uv': _w((lambda *s: _rng.normal(s) * 0.05)(Dc, H, D) * Dc ** (-0.5)), 'w_o': _w((lambda *s: _rng.normal(s) * 0.05)(H, D, M) * (H * D) ** (-0.5))}
    _B_in = _B_setup()
    return {'A_x': _A_in['x'], 'A_mem0': _A_in['mem0'], 'A_Wq': _A_in['Wq'], 'A_Wk': _A_in['Wk'], 'A_Wv': _A_in['Wv'], 'A_Wo': _A_in['Wo'], 'A_seg_len': _A_in['seg_len'], 'B_x': _B_in['x'], 'B_c_kv': _B_in['c_kv'], 'B_w_q': _B_in['w_q'], 'B_w_uk': _B_in['w_uk'], 'B_w_uv': _B_in['w_uv'], 'B_w_o': _B_in['w_o']}

def reference(A_x, A_mem0, A_Wq, A_Wk, A_Wv, A_Wo, A_seg_len, B_x, B_c_kv, B_w_q, B_w_uk, B_w_uv, B_w_o):

    def _A_ref(x, mem0, Wq, Wk, Wv, Wo, seg_len):
        B, S, Dm = x.shape
        H, Dh = (Wq.shape[1], Wq.shape[2])
        M = mem0.shape[1]
        scale = Dh ** (-0.5)
        n_seg = S // seg_len
        L = M + seg_len
        idx = jnp.arange(L)
        mask = (idx[:, None] < M) | (idx[:, None] >= idx[None, :])
        mem = mem0
        outs = []
        for s in range(n_seg):
            xs = x[:, s * seg_len:(s + 1) * seg_len, :].copy()
            h = jnp.concatenate([mem, xs], axis=1)
            q = jnp.einsum('btd,dhe->bhte', h, Wq)
            k = jnp.einsum('btd,dhe->bhte', h, Wk)
            v = jnp.einsum('btd,dhe->bhte', h, Wv)
            scores = jnp.einsum('bhqe,bhke->bhqk', q, k) * scale
            scores = jnp.where(mask[None, None], scores, -1000000000.0)
            p = _softmax(scores, axis=-1)
            o = jnp.einsum('bhqk,bhke->bhqe', p, v)
            o = jnp.einsum('bhte,hed->btd', o, Wo)
            mem = o[:, :M, :].copy()
            outs.append(o[:, M:, :])
        return jnp.concatenate(outs, axis=1)

    def _B_ref(x, c_kv, w_q, w_uk, w_uv, w_o):
        B, Sq, M = (x.shape[0], x.shape[1], x.shape[2])
        Sk = c_kv.shape[1]
        H, D = (w_q.shape[1], w_q.shape[2])
        q = jnp.einsum('bqm,mhd->bhqd', x, w_q)
        k = jnp.einsum('bkc,chd->bhkd', c_kv, w_uk)
        v = jnp.einsum('bkc,chd->bhkd', c_kv, w_uv)
        scores = jnp.einsum('bhqd,bhkd->bhqk', q, k) * D ** (-0.5)
        off = Sk - Sq
        qi = jnp.arange(Sq)[:, None]
        kj = jnp.arange(Sk)[None, :]
        cmask = kj <= qi + off
        scores = jnp.where(cmask[None, None], scores, -1000000000.0)
        p = _softmax(scores, axis=-1)
        ctx = jnp.einsum('bhqk,bhkd->bhqd', p, v)
        return jnp.einsum('bhqd,hdm->bqm', ctx, w_o)
    a = _A_ref(A_x, A_mem0, A_Wq, A_Wk, A_Wv, A_Wo, A_seg_len)
    b = _B_ref(B_x, B_c_kv, B_w_q, B_w_uk, B_w_uv, B_w_o)
    return jnp.concatenate([a, b], axis=-1)
```

```python
import functools

import jax
import jax.numpy as jnp
from jax import lax
import jax.experimental.pallas as pl
import jax.experimental.pallas.tpu as pltpu

F32 = jnp.float32
BF16 = jnp.bfloat16
NT = (((1,), (1,)), ((), ()))
NEG = -1000000000.0

S = 2048
DM = 448
H = 16
DH = 256
HD = H * DH
DC = 1024
MEM = 8
SEG = 32
L = SEG + MEM
NPAIR = S // (2 * SEG)

BQ = 256
HB = BQ // 2
NQ = S // BQ
PB = 512


def _dot(a, b):
    return jnp.dot(a, b, preferred_element_type=F32)


def _dot_nt(a, b):
    return lax.dot_general(a, b, NT, preferred_element_type=F32)


def _kernel(axt_hbm, mem0_ref, awq_hbm, awk_hbm, awv_hbm, awot_hbm,
            bxt_hbm, ckv_hbm, bwq_hbm, bwk_hbm, bwv_hbm, bwot_hbm,
            out_hbm,
            wk_s, wv_s, ckv_s, bwot_s, q_s, rawa_s, awot_s, axt_s, sems, osem):
    scale = DH ** -0.5

    def cp(src, dst, i):
        return pltpu.make_async_copy(src, dst, sems.at[i])

    cp_ckv = cp(ckv_hbm, ckv_s, 4)
    cp_bwot = cp(bwot_hbm, bwot_s, 5)
    cp_awq = cp(awq_hbm, rawa_s.at[0], 6)
    cp_awk = cp(awk_hbm, rawa_s.at[1], 7)
    cp_awv = cp(awv_hbm, rawa_s.at[2], 8)
    cp_awot = cp(awot_hbm, awot_s, 9)
    cp_axt = [cp(axt_hbm.at[:, pl.ds(j * 128, 128)], axt_s.at[j], 10)
              for j in range(S // 128)]

    def prologue(bxt_s, bx_s, rawq_s, wq_s, rawk_s, rawv_s):
        cp_bxt = cp(bxt_hbm, bxt_s, 0)
        cp_bwq = cp(bwq_hbm, rawq_s, 1)
        cp_bwk = cp(bwk_hbm, rawk_s, 2)
        cp_bwv = cp(bwv_hbm, rawv_s, 3)
        cp_bxt.start()
        cp_bwq.start()
        cp_bxt.wait()
        cp_bwq.wait()
        cp_bwk.start()
        cp_bwv.start()
        cp_ckv.start()
        cp_bwot.start()

        def relayout(src, dst, r0, n):
            w = jnp.swapaxes(src[pl.ds(r0, n)], 0, 1)
            for h in range(H):
                dst[h, pl.ds(r0, n), :] = w[h]

        def qproj(h):
            for r in range(S // PB):
                rows = slice(r * PB, (r + 1) * PB)
                q_s[h, rows, :] = (_dot(bx_s[rows, :], wq_s[h]) * scale).astype(BF16)

        for j in range(S // PB):
            bx_s[j * PB:(j + 1) * PB, :] = bxt_s[:, j * PB:(j + 1) * PB].T
        for c in range(DM // 64):
            relayout(rawq_s, wq_s, c * 64, 64)

        def blk(h0, side):
            def body(i, c):
                qproj(h0 + i)
                side(i)
                return c
            lax.fori_loop(0, 4, body, 0)

        def side_relayout(src, dst):
            def side(i):
                for c in range(4):
                    relayout(src, dst, pl.multiple_of(i * 256 + c * 64, 64), 64)
            return side

        blk(0, lambda i: None)
        cp_bwk.wait()
        blk(4, side_relayout(rawk_s, wk_s))
        cp_bwv.wait()
        for c in cp_axt:
            c.start()
        cp_awot.start()
        cp_awq.start()
        cp_awk.start()
        cp_awv.start()
        blk(8, side_relayout(rawv_s, wv_s))
        blk(12, lambda i: None)

    pl.run_scoped(
        prologue,
        pltpu.VMEM((DM, S), BF16), pltpu.VMEM((S, DM), BF16),
        pltpu.VMEM((DM, H, DH), BF16), pltpu.VMEM((H, DM, DH), BF16),
        pltpu.VMEM((DC, H, DH), BF16), pltpu.VMEM((DC, H, DH), BF16),
    )

    def main(wa_s, awo_s, ax_s, k_s, v_s, acc_s, stage_s, qkv0, qkv1, oa, ob):
        cp_ckv.wait()
        cp_bwot.wait()
        for c in cp_axt:
            c.wait()
        cp_awot.wait()
        cp_awq.wait()
        cp_awk.wait()
        cp_awv.wait()
        acc_s[...] = jnp.zeros_like(acc_s)

        tri = (lax.broadcasted_iota(jnp.int32, (HB, HB), 1)
               <= lax.broadcasted_iota(jnp.int32, (HB, HB), 0))
        tri2 = (lax.broadcasted_iota(jnp.int32, (BQ, HB), 1)
                <= lax.broadcasted_iota(jnp.int32, (BQ, HB), 0))

        def kvproj(w_ref, dst, h):
            for r in range(S // PB):
                rows = slice(r * PB, (r + 1) * PB)
                dst[rows, :] = _dot(ckv_s[rows, :], w_ref[h]).astype(BF16)

        def qk(h, i):
            d0 = i * BQ
            q = q_s[h, d0:d0 + BQ, :]
            so = _dot_nt(q, k_s[0:d0, :]) if i > 0 else None
            s1 = _dot_nt(q, k_s[d0:d0 + HB, :])
            s2 = _dot_nt(q[HB:], k_s[d0 + HB:d0 + BQ, :])
            return so, s1, s2

        def soft_pv_out(h, i, ss):
            so, s1, s2 = ss
            d0 = i * BQ
            s1 = jnp.where(tri2, s1, NEG)
            s2 = jnp.where(tri, s2, NEG)
            m = jnp.max(s1, axis=1, keepdims=True)
            if so is not None:
                m = jnp.maximum(m, jnp.max(so, axis=1, keepdims=True))
            mb = jnp.maximum(m[HB:], jnp.max(s2, axis=1, keepdims=True))
            m = jnp.concatenate([m[:HB], mb], axis=0)
            p1 = jnp.exp(s1 - m)
            p2 = jnp.exp(s2 - mb)
            l = jnp.sum(p1, axis=1, keepdims=True)
            acc = _dot(p1.astype(BF16), v_s[d0:d0 + HB, :])
            if so is not None:
                po = jnp.exp(so - m)
                l = l + jnp.sum(po, axis=1, keepdims=True)
                acc = acc + _dot(po.astype(BF16), v_s[0:d0, :])
            l2 = l[HB:] + jnp.sum(p2, axis=1, keepdims=True)
            acc2 = acc[HB:] + _dot(p2.astype(BF16), v_s[d0 + HB:d0 + BQ, :])
            ctx = jnp.concatenate(
                [acc[:HB] * (1.0 / l[:HB]), acc2 * (1.0 / l2)], axis=0).astype(BF16)
            acc_s[d0:d0 + BQ, :] += _dot_nt(ctx, bwot_s[h])

        def head(h, c):
            r0 = pl.multiple_of(jnp.minimum(h, DM // 32 - 1) * 32, 32)
            for t in range(3):
                wa_s[pl.ds(r0, 32), t * HD:(t + 1) * HD] = (
                    rawa_s[t, pl.ds(r0, 32)].reshape(32, HD))
            awo_s[pl.ds(pl.multiple_of(h * DH, DH), DH), :] = awot_s[h].T
            ax_s[pl.ds(pl.multiple_of(h * 128, 128), 128), :] = axt_s[h].T

            kvproj(wk_s, k_s, h)
            order = list(range(NQ - 1, -1, -1))
            ss = qk(h, order[0])
            kvproj(wv_s, v_s, h)
            for n, i in enumerate(order):
                nxt = qk(h, order[n + 1]) if n + 1 < NQ else None
                soft_pv_out(h, i, ss)
                ss = nxt
            return c

        lax.fori_loop(0, H, head, 0)

        row = lax.broadcasted_iota(jnp.int32, (L, L), 0)
        col = lax.broadcasted_iota(jnp.int32, (L, L), 1)
        mask = (row >= SEG) | (col >= SEG) | (col <= row)
        CH = 1024

        def proj(lhs, t, dests):
            for j in range(HD // CH):
                c0 = t * HD + j * CH
                r = _dot(lhs, wa_s[:, c0:c0 + CH])
                if t == 0:
                    r = r * scale
                r = r.astype(BF16)
                for (a, n, d, b) in dests:
                    d[b:b + n, c0:c0 + CH] = r[a:a + n]

        def seg(lhs, dests, qkv, odests):
            proj(lhs, 0, dests)
            proj(lhs, 1, dests)
            scs = [_dot_nt(qkv[:, h * DH:(h + 1) * DH],
                           qkv[:, HD + h * DH:HD + (h + 1) * DH]) for h in range(H)]
            proj(lhs, 2, dests)
            for h in range(H):
                c0 = h * DH
                sc = jnp.where(mask, scs[h], NEG)
                m = jnp.max(sc, axis=1, keepdims=True)
                e = jnp.exp(sc - m)
                l = jnp.sum(e, axis=1, keepdims=True)
                p = (e * (1.0 / l)).astype(BF16)
                o = _dot(p, qkv[:, 2 * HD + c0:2 * HD + c0 + DH]).astype(BF16)
                for (a, n, d, b) in odests:
                    d[b:b + n, c0:c0 + DH] = o[a:a + n]

        def out_copy(base):
            return pltpu.make_async_copy(
                stage_s.at[pl.ds(base, 2 * SEG)], out_hbm.at[pl.ds(base, 2 * SEG)], osem)

        def pair(j, mem):
            base = pl.multiple_of(j * 2 * SEG, 2 * SEG)
            stage_s[pl.ds(base, 2 * SEG), DM:2 * DM] = (
                acc_s[pl.ds(base, 2 * SEG), :].astype(BF16))
            x0 = ax_s[pl.ds(base, SEG), :]
            x1 = ax_s[pl.ds(base + SEG, SEG), :]
            lhs1 = jnp.concatenate([x0, x1[0:8], mem], axis=0)
            seg(lhs1, [(0, 32, qkv0, 0), (32, 8, qkv1, 0), (40, 8, qkv0, 32)], qkv0,
                [(0, 24, oa, 0), (24, 8, ob, 40), (32, 8, oa, 24)])
            out1 = _dot(oa[...], awo_s[...]).astype(BF16)
            stage_s[pl.ds(base, 24), 0:DM] = out1[0:24]
            lhs2 = jnp.concatenate([x1[16:32], out1[24:32], x1[8:16]], axis=0)
            seg(lhs2, [(0, 16, qkv1, 16), (16, 8, qkv1, 32), (24, 8, qkv1, 8)], qkv1,
                [(0, 40, ob, 0)])
            out2 = _dot(ob[...], awo_s[...]).astype(BF16)
            stage_s[pl.ds(base + SEG, SEG), 0:DM] = out2[0:32]
            stage_s[pl.ds(base + 24, 8), 0:DM] = out2[40:48]
            out_copy(base).start()
            return out2[32:40]

        lax.fori_loop(0, NPAIR, pair, mem0_ref[...])
        for j in range(NPAIR):
            out_copy(j * 2 * SEG).wait()

    pl.run_scoped(
        main,
        pltpu.VMEM((DM, 3 * HD), BF16), pltpu.VMEM((HD, DM), BF16),
        pltpu.VMEM((S, DM), BF16),
        pltpu.VMEM((S, DH), BF16), pltpu.VMEM((S, DH), BF16),
        pltpu.VMEM((S, DM), F32), pltpu.VMEM((S, 2 * DM), BF16),
        pltpu.VMEM((L, 3 * HD), BF16), pltpu.VMEM((L, 3 * HD), BF16),
        pltpu.VMEM((32, HD), BF16), pltpu.VMEM((48, HD), BF16),
    )


@functools.partial(jax.jit, static_argnames=("A_seg_len",))
def pallas_concat_heads__memory_aug_recurrent_mem_tr__compressed_kv_cla__prompt_kernel(
    A_x: jax.Array,
    A_mem0: jax.Array,
    A_Wq: jax.Array,
    A_Wk: jax.Array,
    A_Wv: jax.Array,
    A_Wo: jax.Array,
    A_seg_len: int,
    B_x: jax.Array,
    B_c_kv: jax.Array,
    B_w_q: jax.Array,
    B_w_uk: jax.Array,
    B_w_uv: jax.Array,
    B_w_o: jax.Array,
):
    assert A_seg_len == SEG
    assert A_x.shape == (1, S, DM) and A_mem0.shape == (1, MEM, DM)
    assert A_Wq.shape == (DM, H, DH) and A_Wo.shape == (H, DH, DM)
    assert B_x.shape == (1, S, DM) and B_c_kv.shape == (1, S, DC)
    assert B_w_q.shape == (DM, H, DH) and B_w_uk.shape == (DC, H, DH)
    assert B_w_o.shape == (H, DH, DM)

    axt = jnp.swapaxes(A_x, 1, 2).reshape(DM, S)
    bxt = jnp.swapaxes(B_x, 1, 2).reshape(DM, S)
    awot = jnp.swapaxes(A_Wo, 1, 2)
    bwot = jnp.swapaxes(B_w_o, 1, 2)

    any_spec = pl.BlockSpec(memory_space=pl.ANY)
    out = pl.pallas_call(
        _kernel,
        out_shape=jax.ShapeDtypeStruct((S, 2 * DM), BF16),
        in_specs=[any_spec, pl.BlockSpec(memory_space=pltpu.VMEM)] + [any_spec] * 10,
        out_specs=any_spec,
        scratch_shapes=[
            pltpu.VMEM((H, DC, DH), BF16),
            pltpu.VMEM((H, DC, DH), BF16),
            pltpu.VMEM((S, DC), BF16),
            pltpu.VMEM((H, DM, DH), BF16),
            pltpu.VMEM((H, S, DH), BF16),
            pltpu.VMEM((3, DM, H, DH), BF16),
            pltpu.VMEM((H, DM, DH), BF16),
            pltpu.VMEM((S // 128, DM, 128), BF16),
            pltpu.SemaphoreType.DMA((11,)),
            pltpu.SemaphoreType.DMA,
        ],
        compiler_params=pltpu.CompilerParams(vmem_limit_bytes=120 * 1024 * 1024),
    )(axt, A_mem0.reshape(MEM, DM), A_Wq, A_Wk, A_Wv, awot,
      bxt, B_c_kv.reshape(S, DC), B_w_q, B_w_uk, B_w_uv, bwot)
    return out.reshape(1, S, 2 * DM)
```

```python
import functools

import jax
import jax.numpy as jnp
from jax import lax
import jax.experimental.pallas as pl
import jax.experimental.pallas.tpu as pltpu

F32 = jnp.float32
BF16 = jnp.bfloat16
NT = (((1,), (1,)), ((), ()))
NEG = -1000000000.0

S = 2048
DM = 448
H = 16
DH = 256
HD = H * DH
DC = 1024
MEM = 8
SEG = 32
L = SEG + MEM
NPAIR = S // (2 * SEG)

BQ = 256
HB = BQ // 2
NQ = S // BQ
PB = 512
QB = 128
KB = 128
N_HEAD_ITERS = H
N_PAIR_ITERS = NPAIR


def _dot(a, b):
    return jnp.dot(a, b, preferred_element_type=F32)


def _dot_nt(a, b):
    return lax.dot_general(a, b, NT, preferred_element_type=F32)


def _kernel(axt_hbm, mem0_ref, awq_hbm, awk_hbm, awv_hbm, awot_hbm,
            bxt_hbm, ckv_hbm, bwq_hbm, bwk_hbm, bwv_hbm, bwot_hbm,
            out_hbm,
            wk_s, wv_s, ckv_s, bwot_s, q_s, acc_s, rawa_s, awot_s, axt_s, sems, osem):
    scale = DH ** -0.5

    def cp(src, dst, i):
        return pltpu.make_async_copy(src, dst, sems.at[i])

    cp_ckv = cp(ckv_hbm, ckv_s, 6)
    cp_bwot = cp(bwot_hbm, bwot_s, 7)
    cp_awot = cp(awot_hbm, awot_s, 8)
    cp_axt = [cp(axt_hbm.at[:, pl.ds(j * 128, 128)], axt_s.at[j], 9)
              for j in range(S // 128)]
    cp_aw = [cp(w, rawa_s.at[t, pl.ds(0, DM)], 10 + t)
             for t, w in enumerate((awq_hbm, awk_hbm, awv_hbm))]

    def prologue(bxt_s, bx_s, rawq_s, wq_s, rawk_s, rawv_s):
        cp_bxt = [cp(bxt_hbm.at[:, pl.ds(j * 128, 128)], bxt_s.at[j], 0 if j < 4 else 1)
                  for j in range(S // 128)]
        cp_bwq = [cp(bwq_hbm.at[:, pl.ds(t * 8, 8), :], rawq_s.at[t], 2 + t)
                  for t in range(2)]
        cp_bwk = cp(bwk_hbm, rawk_s, 4)
        cp_bwv = cp(bwv_hbm, rawv_s, 5)
        for c in (cp_bwq[:1] + cp_bxt + cp_bwq[1:]
                  + [cp_bwk, cp_bwv, cp_ckv, cp_bwot, cp_awot] + cp_axt + cp_aw):
            c.start()

        for t in range(3):
            rawa_s[t, DM:DM + 32] = jnp.zeros((32, H, DH), BF16)

        def relayout(src, dst, h0, r0, n):
            w = jnp.swapaxes(src[pl.ds(r0, n)], 0, 1)
            for h in range(w.shape[0]):
                dst[h0 + h, pl.ds(r0, n), :] = w[h]

        def xpose(j):
            r0 = j * 128 if isinstance(j, int) else pl.multiple_of(j * 128, 128)
            bx_s[pl.ds(r0, 128), :] = bxt_s[j].T

        def blk(h0, nh, r_lo, r_hi, side):
            def body(i, c):
                h = h0 + i
                for r in range(r_lo, r_hi):
                    rows = slice(r * QB, (r + 1) * QB)
                    q_s[h, rows, :] = (_dot(bx_s[rows, :], wq_s[h]) * scale).astype(BF16)
                    side(i, r - r_lo)
                return c
            lax.fori_loop(0, nh, body, 0)

        def side_zero(i, r):
            acc_s[pl.ds(pl.multiple_of((i * 4 + r) * 128, 128), 128), :] = (
                jnp.zeros((128, DM), F32))

        def side_xpose(i, r):
            if r < 3:
                xpose(4 + i * 3 + r)

        def side_wq(i, r):
            if r < 4:
                r0 = jnp.minimum(i, DM // 64 - 1) * 64 + r * 16
                relayout(rawq_s.at[1], wq_s, 8, pl.multiple_of(r0, 16), 16)

        def side_relayout(src, dst):
            def side(i, r):
                relayout(src, dst, 0, pl.multiple_of(i * 256 + r * 16, 16), 16)
            return side

        cp_bwq[0].wait()
        for c in range(DM // 64):
            relayout(rawq_s.at[0], wq_s, 0, c * 64, 64)
        for c in cp_bxt[:4]:
            c.wait()
        for j in range(4):
            xpose(j)
        blk(0, 4, 0, 4, side_zero)
        for c in cp_bxt[4:]:
            c.wait()
        blk(4, 4, 0, 4, side_xpose)
        cp_bwq[1].wait()
        blk(0, 8, 4, 16, side_wq)
        cp_bwk.wait()
        blk(8, 4, 0, 16, side_relayout(rawk_s, wk_s))
        cp_bwv.wait()
        blk(12, 4, 0, 16, side_relayout(rawv_s, wv_s))

    pl.run_scoped(
        prologue,
        pltpu.VMEM((S // 128, DM, 128), BF16), pltpu.VMEM((S, DM), BF16),
        pltpu.VMEM((2, DM, 8, DH), BF16), pltpu.VMEM((H, DM, DH), BF16),
        pltpu.VMEM((DC, H, DH), BF16), pltpu.VMEM((DC, H, DH), BF16),
    )

    def main(wa_s, awo_s, ax_s, k_s, v_s, stage_s, qkv0, qkv1, oa, ob):
        cp_ckv.wait()
        cp_bwot.wait()
        cp_awot.wait()
        for c in cp_axt:
            c.wait()

        tri = (lax.broadcasted_iota(jnp.int32, (HB, HB), 1)
               <= lax.broadcasted_iota(jnp.int32, (HB, HB), 0))
        tri2 = (lax.broadcasted_iota(jnp.int32, (BQ, HB), 1)
                <= lax.broadcasted_iota(jnp.int32, (BQ, HB), 0))

        def kvproj(w_ref, dst, h, pb, side):
            for r in range(S // pb):
                rows = slice(r * pb, (r + 1) * pb)
                dst[rows, :] = _dot(ckv_s[rows, :], w_ref[h]).astype(BF16)
                side(r)

        def qk(h, i):
            d0 = i * BQ
            q = q_s[h, d0:d0 + BQ, :]
            so = _dot_nt(q, k_s[0:d0, :]) if i > 0 else None
            s1 = _dot_nt(q, k_s[d0:d0 + HB, :])
            s2 = _dot_nt(q[HB:], k_s[d0 + HB:d0 + BQ, :])
            return so, s1, s2

        def soft_pv_out(h, i, ss):
            so, s1, s2 = ss
            d0 = i * BQ
            s1 = jnp.where(tri2, s1, NEG)
            s2 = jnp.where(tri, s2, NEG)
            m = jnp.max(s1, axis=1, keepdims=True)
            if so is not None:
                m = jnp.maximum(m, jnp.max(so, axis=1, keepdims=True))
            mb = jnp.maximum(m[HB:], jnp.max(s2, axis=1, keepdims=True))
            m = jnp.concatenate([m[:HB], mb], axis=0)
            p1 = jnp.exp(s1 - m)
            p2 = jnp.exp(s2 - mb)
            l = jnp.sum(p1, axis=1, keepdims=True)
            acc = _dot(p1.astype(BF16), v_s[d0:d0 + HB, :])
            if so is not None:
                po = jnp.exp(so - m)
                l = l + jnp.sum(po, axis=1, keepdims=True)
                acc = acc + _dot(po.astype(BF16), v_s[0:d0, :])
            l2 = l[HB:] + jnp.sum(p2, axis=1, keepdims=True)
            acc2 = acc[HB:] + _dot(p2.astype(BF16), v_s[d0 + HB:d0 + BQ, :])
            ctx = jnp.concatenate(
                [acc[:HB] * (1.0 / l[:HB]), acc2 * (1.0 / l2)], axis=0).astype(BF16)
            acc_s[d0:d0 + BQ, :] += _dot_nt(ctx, bwot_s[h])

        def head(h, c):
            @pl.when(h == 2)
            def _():
                for cw in cp_aw:
                    cw.wait()

            r0 = jnp.where(h >= 2, (h - 2) * 32, DM)

            def side(r):
                if r < 6:
                    t, half = divmod(r, 2)
                    rr = pl.multiple_of(r0 + half * 16, 16)
                    wa_s[pl.ds(rr, 16), t * HD:(t + 1) * HD] = (
                        rawa_s[t, pl.ds(rr, 16)].reshape(16, HD))
                elif r < 8:
                    e0 = (r - 6) * 128
                    awo_s[pl.ds(pl.multiple_of(h * DH + e0, 128), 128), :] = (
                        awot_s[h, :, e0:e0 + 128].T)
                elif r == 8:
                    ax_s[pl.ds(pl.multiple_of(h * 128, 128), 128), :] = axt_s[h].T

            kvproj(wk_s, k_s, h, KB, side)
            order = list(range(NQ - 1, -1, -1))
            ss = qk(h, order[0])
            kvproj(wv_s, v_s, h, PB, lambda r: None)
            for n, i in enumerate(order):
                nxt = qk(h, order[n + 1]) if n + 1 < NQ else None
                soft_pv_out(h, i, ss)
                ss = nxt
            return c

        lax.fori_loop(0, N_HEAD_ITERS, head, 0)

        row = lax.broadcasted_iota(jnp.int32, (L, L), 0)
        col = lax.broadcasted_iota(jnp.int32, (L, L), 1)
        mask = (row >= SEG) | (col >= SEG) | (col <= row)
        CH = 1024

        def proj(lhs, t, dests):
            for j in range(HD // CH):
                c0 = t * HD + j * CH
                r = _dot(lhs, wa_s[0:DM, c0:c0 + CH])
                if t == 0:
                    r = r * scale
                r = r.astype(BF16)
                for (a, n, d, b) in dests:
                    d[b:b + n, c0:c0 + CH] = r[a:a + n]

        def seg(lhs, dests, qkv, odests):
            proj(lhs, 0, dests)
            proj(lhs, 1, dests)
            scs = [_dot_nt(qkv[:, h * DH:(h + 1) * DH],
                           qkv[:, HD + h * DH:HD + (h + 1) * DH]) for h in range(H)]
            proj(lhs, 2, dests)
            for h in range(H):
                c0 = h * DH
                sc = jnp.where(mask, scs[h], NEG)
                m = jnp.max(sc, axis=1, keepdims=True)
                e = jnp.exp(sc - m)
                l = jnp.sum(e, axis=1, keepdims=True)
                p = (e * (1.0 / l)).astype(BF16)
                o = _dot(p, qkv[:, 2 * HD + c0:2 * HD + c0 + DH]).astype(BF16)
                for (a, n, d, b) in odests:
                    d[b:b + n, c0:c0 + DH] = o[a:a + n]

        def out_copy(base):
            return pltpu.make_async_copy(
                stage_s.at[pl.ds(base, 2 * SEG)], out_hbm.at[pl.ds(base, 2 * SEG)], osem)

        def pair(j, mem):
            base = pl.multiple_of(j * 2 * SEG, 2 * SEG)
            stage_s[pl.ds(base, 2 * SEG), DM:2 * DM] = (
                acc_s[pl.ds(base, 2 * SEG), :].astype(BF16))
            x0 = ax_s[pl.ds(base, SEG), :]
            x1 = ax_s[pl.ds(base + SEG, SEG), :]
            lhs1 = jnp.concatenate([x0, x1[0:8], mem], axis=0)
            seg(lhs1, [(0, 32, qkv0, 0), (32, 8, qkv1, 0), (40, 8, qkv0, 32)], qkv0,
                [(0, 24, oa, 0), (24, 8, ob, 40), (32, 8, oa, 24)])
            out1 = _dot(oa[...], awo_s[...]).astype(BF16)
            stage_s[pl.ds(base, 24), 0:DM] = out1[0:24]
            lhs2 = jnp.concatenate([x1[16:32], out1[24:32], x1[8:16]], axis=0)
            seg(lhs2, [(0, 16, qkv1, 16), (16, 8, qkv1, 32), (24, 8, qkv1, 8)], qkv1,
                [(0, 40, ob, 0)])
            out2 = _dot(ob[...], awo_s[...]).astype(BF16)
            stage_s[pl.ds(base + SEG, SEG), 0:DM] = out2[0:32]
            stage_s[pl.ds(base + 24, 8), 0:DM] = out2[40:48]
            out_copy(base).start()
            return out2[32:40]

        lax.fori_loop(0, N_PAIR_ITERS, pair, mem0_ref[...])
        for j in range(N_PAIR_ITERS):
            out_copy(j * 2 * SEG).wait()

    pl.run_scoped(
        main,
        pltpu.VMEM((DM + 32, 3 * HD), BF16), pltpu.VMEM((HD, DM), BF16),
        pltpu.VMEM((S, DM), BF16),
        pltpu.VMEM((S, DH), BF16), pltpu.VMEM((S, DH), BF16),
        pltpu.VMEM((S, 2 * DM), BF16),
        pltpu.VMEM((L, 3 * HD), BF16), pltpu.VMEM((L, 3 * HD), BF16),
        pltpu.VMEM((32, HD), BF16), pltpu.VMEM((48, HD), BF16),
    )


@functools.partial(jax.jit, static_argnames=("A_seg_len",))
def pallas_concat_heads__memory_aug_recurrent_mem_tr__compressed_kv_cla__prompt_kernel(
    A_x: jax.Array,
    A_mem0: jax.Array,
    A_Wq: jax.Array,
    A_Wk: jax.Array,
    A_Wv: jax.Array,
    A_Wo: jax.Array,
    A_seg_len: int,
    B_x: jax.Array,
    B_c_kv: jax.Array,
    B_w_q: jax.Array,
    B_w_uk: jax.Array,
    B_w_uv: jax.Array,
    B_w_o: jax.Array,
):
    assert A_seg_len == SEG
    assert A_x.shape == (1, S, DM) and A_mem0.shape == (1, MEM, DM)
    assert A_Wq.shape == (DM, H, DH) and A_Wo.shape == (H, DH, DM)
    assert B_x.shape == (1, S, DM) and B_c_kv.shape == (1, S, DC)
    assert B_w_q.shape == (DM, H, DH) and B_w_uk.shape == (DC, H, DH)
    assert B_w_o.shape == (H, DH, DM)

    axt = jnp.swapaxes(A_x, 1, 2).reshape(DM, S)
    bxt = jnp.swapaxes(B_x, 1, 2).reshape(DM, S)
    awot = jnp.swapaxes(A_Wo, 1, 2)
    bwot = jnp.swapaxes(B_w_o, 1, 2)

    any_spec = pl.BlockSpec(memory_space=pl.ANY)
    out = pl.pallas_call(
        _kernel,
        out_shape=jax.ShapeDtypeStruct((S, 2 * DM), BF16),
        in_specs=[any_spec, pl.BlockSpec(memory_space=pltpu.VMEM)] + [any_spec] * 10,
        out_specs=any_spec,
        scratch_shapes=[
            pltpu.VMEM((H, DC, DH), BF16),
            pltpu.VMEM((H, DC, DH), BF16),
            pltpu.VMEM((S, DC), BF16),
            pltpu.VMEM((H, DM, DH), BF16),
            pltpu.VMEM((H, S, DH), BF16),
            pltpu.VMEM((S, DM), F32),
            pltpu.VMEM((3, DM + 32, H, DH), BF16),
            pltpu.VMEM((H, DM, DH), BF16),
            pltpu.VMEM((S // 128, DM, 128), BF16),
            pltpu.SemaphoreType.DMA((13,)),
            pltpu.SemaphoreType.DMA,
        ],
        compiler_params=pltpu.CompilerParams(vmem_limit_bytes=120 * 1024 * 1024),
    )(axt, A_mem0.reshape(MEM, DM), A_Wq, A_Wk, A_Wv, awot,
      bxt, B_c_kv.reshape(S, DC), B_w_q, B_w_uk, B_w_uv, bwot)
    return out.reshape(1, S, 2 * DM)
```

```python
import functools

import jax
import jax.numpy as jnp
from jax import lax
import jax.experimental.pallas as pl
import jax.experimental.pallas.tpu as pltpu

F32 = jnp.float32
BF16 = jnp.bfloat16
NT = (((1,), (1,)), ((), ()))
NEG = -1000000000.0

S = 2048
DM = 448
H = 16
DH = 256
HD = H * DH
DC = 1024
MEM = 8
SEG = 32
L = SEG + MEM
NPAIR = S // (2 * SEG)
NG = 6

BQ = 256
HB = BQ // 2
NQ = S // BQ
PB = 512
QB = 128
KB = 128
N_OPROJ_ITERS = S // 128
N_HEAD_ITERS = H
N_PAIR_ITERS = NPAIR


def _dot(a, b):
    return jnp.dot(a, b, preferred_element_type=F32)


def _dot_nt(a, b):
    return lax.dot_general(a, b, NT, preferred_element_type=F32)


def _kernel(axt_hbm, mem0_ref, awq_hbm, awk_hbm, awv_hbm, awot_hbm,
            bxt_hbm, ckv_hbm, bwq_hbm, bwk_hbm, bwv_hbm, bwot_hbm,
            out_hbm,
            wk_s, wv_s, ckv_s, bwot_s, q_s, rawa_s, awot_s, axt_s, sems, osem):
    scale = DH ** -0.5

    def cp(src, dst, i):
        return pltpu.make_async_copy(src, dst, sems.at[i])

    cp_ckv = cp(ckv_hbm, ckv_s, 6)
    cp_bwot = cp(bwot_hbm, bwot_s, 7)
    cp_awot = cp(awot_hbm, awot_s, 8)
    cp_axt = [cp(axt_hbm.at[:, pl.ds(j * 128, 128)], axt_s.at[j], 9)
              for j in range(S // 128)]
    cp_aw = [cp(w, rawa_s.at[t, pl.ds(0, DM)], 10 + t)
             for t, w in enumerate((awq_hbm, awk_hbm, awv_hbm))]

    def prologue(bxt_s, bx_s, rawq_s, wq_s, rawk_s, rawv_s):
        cp_bxt = [cp(bxt_hbm.at[:, pl.ds(j * 128, 128)], bxt_s.at[j], 0 if j < 4 else 1)
                  for j in range(S // 128)]
        cp_bwq = [cp(bwq_hbm.at[:, pl.ds(t * 8, 8), :], rawq_s.at[t], 2 + t)
                  for t in range(2)]
        cp_bwk = cp(bwk_hbm, rawk_s, 4)
        cp_bwv = cp(bwv_hbm, rawv_s, 5)
        for c in (cp_bwq[:1] + cp_bxt + cp_bwq[1:]
                  + [cp_bwk, cp_bwv, cp_ckv, cp_bwot, cp_awot] + cp_axt + cp_aw):
            c.start()

        def relayout(src, dst, h0, r0, n):
            w = jnp.swapaxes(src[pl.ds(r0, n)], 0, 1)
            for h in range(w.shape[0]):
                dst[h0 + h, pl.ds(r0, n), :] = w[h]

        def xpose(j):
            r0 = j * 128 if isinstance(j, int) else pl.multiple_of(j * 128, 128)
            bx_s[pl.ds(r0, 128), :] = bxt_s[j].T

        def blk(h0, nh, r_lo, r_hi, side):
            def body(i, c):
                h = h0 + i
                for r in range(r_lo, r_hi):
                    rows = slice(r * QB, (r + 1) * QB)
                    q_s[h, rows, :] = (_dot(bx_s[rows, :], wq_s[h]) * scale).astype(BF16)
                    side(i, r - r_lo)
                return c
            lax.fori_loop(0, nh, body, 0)

        def side_xpose(i, r):
            if r < 3:
                xpose(4 + i * 3 + r)

        def side_wq(i, r):
            if r < 4:
                r0 = jnp.minimum(i, DM // 64 - 1) * 64 + r * 16
                relayout(rawq_s.at[1], wq_s, 8, pl.multiple_of(r0, 16), 16)

        def side_relayout(src, dst):
            def side(i, r):
                relayout(src, dst, 0, pl.multiple_of(i * 256 + r * 16, 16), 16)
            return side

        cp_bwq[0].wait()
        for c in range(DM // 64):
            relayout(rawq_s.at[0], wq_s, 0, c * 64, 64)
        for c in cp_bxt[:4]:
            c.wait()
        for j in range(4):
            xpose(j)
        blk(0, 4, 0, 4, lambda i, r: None)
        for c in cp_bxt[4:]:
            c.wait()
        blk(4, 4, 0, 4, side_xpose)
        cp_bwq[1].wait()
        blk(0, 8, 4, 16, side_wq)
        cp_bwk.wait()
        blk(8, 4, 0, 16, side_relayout(rawk_s, wk_s))
        cp_bwv.wait()
        blk(12, 4, 0, 16, side_relayout(rawv_s, wv_s))

    pl.run_scoped(
        prologue,
        pltpu.VMEM((S // 128, DM, 128), BF16), pltpu.VMEM((S, DM), BF16),
        pltpu.VMEM((2, DM, 8, DH), BF16), pltpu.VMEM((H, DM, DH), BF16),
        pltpu.VMEM((DC, H, DH), BF16), pltpu.VMEM((DC, H, DH), BF16),
    )

    def main(wqk_s, awv_s, wz_s, ax_s, k_s, v_s, stage_s, ot_s,
             qs0, qs1, ks0, ks1, zs0, zs1):
        cp_ckv.wait()

        tri = (lax.broadcasted_iota(jnp.int32, (HB, HB), 1)
               <= lax.broadcasted_iota(jnp.int32, (HB, HB), 0))
        tri2 = (lax.broadcasted_iota(jnp.int32, (BQ, HB), 1)
                <= lax.broadcasted_iota(jnp.int32, (BQ, HB), 0))

        def kvproj(w_ref, dst, h, pb, lo, hi):
            for r0 in range(lo, hi, pb):
                dst[r0:r0 + pb, :] = _dot(ckv_s[r0:r0 + pb, :], w_ref[h]).astype(BF16)

        def qk(h, i):
            d0 = i * BQ
            q = q_s[h, d0:d0 + BQ, :]
            so = _dot_nt(q, k_s[0:d0, :]) if i > 0 else None
            s1 = _dot_nt(q, k_s[d0:d0 + HB, :])
            s2 = _dot_nt(q[HB:], k_s[d0 + HB:d0 + BQ, :])
            return so, s1, s2

        def soft_pv_out(h, i, ss):
            so, s1, s2 = ss
            d0 = i * BQ
            s1 = jnp.where(tri2, s1, NEG)
            s2 = jnp.where(tri, s2, NEG)
            m = jnp.max(s1, axis=1, keepdims=True)
            if so is not None:
                m = jnp.maximum(m, jnp.max(so, axis=1, keepdims=True))
            mb = jnp.maximum(m[HB:], jnp.max(s2, axis=1, keepdims=True))
            m = jnp.concatenate([m[:HB], mb], axis=0)
            p1 = jnp.exp(s1 - m)
            p2 = jnp.exp(s2 - mb)
            l = jnp.sum(p1, axis=1, keepdims=True)
            acc = _dot(p1.astype(BF16), v_s[d0:d0 + HB, :])
            if so is not None:
                po = jnp.exp(so - m)
                l = l + jnp.sum(po, axis=1, keepdims=True)
                acc = acc + _dot(po.astype(BF16), v_s[0:d0, :])
            l2 = l[HB:] + jnp.sum(p2, axis=1, keepdims=True)
            acc2 = acc[HB:] + _dot(p2.astype(BF16), v_s[d0 + HB:d0 + BQ, :])
            ctx = jnp.concatenate(
                [acc[:HB] * (1.0 / l[:HB]), acc2 * (1.0 / l2)], axis=0).astype(BF16)
            q_s[h, d0:d0 + BQ, :] = ctx

        def head(h, c):
            kvproj(wk_s, k_s, h, KB, 0, S)
            order = list(range(NQ - 1, -1, -1))
            ss = qk(h, order[0])
            kvproj(wv_s, v_s, h, PB, 0, S)
            for n, i in enumerate(order):
                nxt = qk(h, order[n + 1]) if n + 1 < NQ else None
                soft_pv_out(h, i, ss)
                ss = nxt
            return c

        lax.fori_loop(0, N_HEAD_ITERS, head, 0)

        cp_bwot.wait()
        cp_awot.wait()
        for c in cp_axt + cp_aw:
            c.wait()
        ot_s[0] = jnp.zeros((DM, 128), F32)

        def flush(r0):
            stage_s[pl.ds(r0, 128), DM:2 * DM] = ot_s[0].T.astype(BF16)

        def oproj(j, c):
            r0 = pl.multiple_of(j * 128, 128)
            w0 = jnp.minimum(j, DM // 32 - 1) * 32
            pin_w = jnp.maximum(j, DM)
            pin_h = jnp.maximum(j, H)
            pin_o = jnp.where(j >= 0, 1, 0)
            acc = None
            for h in range(H):
                r = _dot_nt(bwot_s[h], q_s[h, pl.ds(r0, 128), :])
                acc = r if acc is None else acc + r
                if h == 0:
                    ot_s[pin_o, 0:8, :] = r[0:8]
                    flush(pl.multiple_of(jnp.maximum(j - 1, 0) * 128, 128))
                elif h in (3, 6, 9, 12):
                    half, g = divmod(h // 3 - 1, 2)
                    rr = pl.multiple_of(w0 + half * 16, 16)
                    rawa_s[2, pin_w, :, 0:128] = r[0:16].astype(BF16)
                    w = jnp.swapaxes(rawa_s[2, pl.ds(rr, 16), g * 8:(g + 1) * 8, :], 0, 1)
                    for u in range(8):
                        awv_s[g * 8 + u, pl.ds(rr, 16), :] = w[u]
                elif h == 14:
                    axt_s[pin_h, 0:16, :] = r[0:16].astype(BF16)
                    ax_s[pl.ds(r0, 128), :] = axt_s[j].T
            ot_s[0] = acc
            return c

        lax.fori_loop(0, N_OPROJ_ITERS, oproj, 0)
        flush(S - 128)

        RC = DM // 4

        def wzprep(i, c):
            for n in range(8):
                rc, u = divmod(n, 2)
                rows = slice(rc * RC, (rc + 1) * RC)
                w = _dot_nt(awv_s[2 * i + u, rows, :], awot_s[2 * i + u]).astype(BF16)
                wz_s[i, rows, u * 512:u * 512 + 384] = w[:, 0:384]
                wz_s[i, rows, 384 + u * 64:448 + u * 64] = w[:, 384:DM]
                if n < 7:
                    piece = i * 7 + n
                    t = jnp.where(piece >= DM // 16, 1, 0)
                    rr = pl.multiple_of((piece - t * (DM // 16)) * 16, 16)
                    wqk_s[t, pl.ds(rr, 16), :] = rawa_s[t, pl.ds(rr, 16)].reshape(16, HD)
            return c

        lax.fori_loop(0, H // 2, wzprep, 0)

        for ks in (ks0, ks1):
            ks[...] = jnp.zeros_like(ks)
        for zs in (zs0, zs1):
            for g in range(NG):
                lo = 3 * L if g < NG - 1 else L
                zs[g * 128 + lo:(g + 1) * 128, :] = jnp.zeros((128 - lo, 512), BF16)

        row = lax.broadcasted_iota(jnp.int32, (3 * L, 128), 0)
        col = lax.broadcasted_iota(jnp.int32, (3 * L, 128), 1)
        off = jnp.where(row >= 2 * L, 2 * L, jnp.where(row >= L, L, 0))
        qi = row - off
        kj = col - off
        mask3 = (kj >= 0) & (kj < L) & ((qi >= SEG) | (kj >= SEG) | (kj <= qi))
        CH = 1024

        def proj_qk(lhs, t, dests):
            for jj in range(HD // CH):
                r = _dot(lhs, wqk_s[t, :, jj * CH:(jj + 1) * CH])
                if t == 0:
                    r = r * scale
                r = r.astype(BF16)
                for u in range(CH // DH):
                    g, jx = divmod(jj * (CH // DH) + u, 3)
                    for (a, n, d, b) in dests:
                        d[g, jx * L + b:jx * L + b + n, :] = r[a:a + n, u * DH:(u + 1) * DH]

        def proj_z(lhs, dests):
            for i in range(H // 2):
                r = _dot(lhs, wz_s[i])
                mid = r[:, 384:512]
                parts = [(r[:, 0:384].astype(BF16), mid.astype(BF16)),
                         (r[:, 512:896].astype(BF16), pltpu.roll(mid, 64, 1).astype(BF16))]
                for u in range(2):
                    g, jx = divmod(2 * i + u, 3)
                    for (a, n, d, b) in dests:
                        r0 = g * 128 + jx * L + b
                        d[r0:r0 + n, 0:384] = parts[u][0][a:a + n]
                        d[r0:r0 + n, 384:512] = parts[u][1][a:a + n]

        def seg(lhs, sel, w):
            def dests(refs):
                return [(a, n, refs[v], b) for (a, n, v, b) in sel]
            qs, ks, zs = (qs0, qs1), (ks0, ks1), (zs0, zs1)
            rows = [3 * L] * (NG - 1) + [L]
            proj_qk(lhs, 0, dests(qs))
            proj_qk(lhs, 1, dests(ks))
            scs = [_dot_nt(qs[w][g, 0:rows[g], :], ks[w][g]) for g in range(NG)]
            proj_z(lhs, dests(zs))
            ps = []
            for g in range(NG):
                sc = jnp.where(mask3[0:rows[g]], scs[g], NEG)
                m = jnp.max(sc, axis=1, keepdims=True)
                e = jnp.exp(sc - m)
                l = jnp.sum(e, axis=1, keepdims=True)
                p = e * (1.0 / l)
                if g < NG - 1:
                    p = p[0:L] + p[L:2 * L] + p[2 * L:3 * L]
                ps.append(p.astype(BF16))
            return _dot(jnp.concatenate(ps, axis=1), zs[w][...])[:, 0:DM].astype(BF16)

        def out_copy(base):
            return pltpu.make_async_copy(
                stage_s.at[pl.ds(base, 2 * SEG)], out_hbm.at[pl.ds(base, 2 * SEG)], osem)

        def pair(j, mem):
            base = pl.multiple_of(j * 2 * SEG, 2 * SEG)
            x0 = ax_s[pl.ds(base, SEG), :]
            x1 = ax_s[pl.ds(base + SEG, SEG), :]
            lhs1 = jnp.concatenate([x0, x1[0:8], mem], axis=0)
            out1 = seg(lhs1, [(0, 32, 0, 0), (32, 8, 1, 0), (40, 8, 0, 32)], 0)
            stage_s[pl.ds(base, SEG), 0:DM] = out1[0:SEG]
            lhs2 = jnp.concatenate([x1[16:32], out1[SEG:L], x1[8:16]], axis=0)
            out2 = seg(lhs2, [(0, 16, 1, 16), (16, 8, 1, 32), (24, 8, 1, 8)], 1)
            stage_s[pl.ds(base + SEG, SEG), 0:DM] = out2[0:SEG]
            out_copy(base).start()
            return out2[SEG:L]

        lax.fori_loop(0, N_PAIR_ITERS, pair, mem0_ref[...])
        for j in range(N_PAIR_ITERS):
            out_copy(j * 2 * SEG).wait()

    pl.run_scoped(
        main,
        pltpu.VMEM((2, DM, HD), BF16), pltpu.VMEM((H, DM, DH), BF16),
        pltpu.VMEM((H // 2, DM, 2 * DM), BF16), pltpu.VMEM((S, DM), BF16),
        pltpu.VMEM((S, DH), BF16), pltpu.VMEM((S, DH), BF16),
        pltpu.VMEM((S, 2 * DM), BF16), pltpu.VMEM((2, DM, 128), F32),
        pltpu.VMEM((NG, 128, DH), BF16), pltpu.VMEM((NG, 128, DH), BF16),
        pltpu.VMEM((NG, 128, DH), BF16), pltpu.VMEM((NG, 128, DH), BF16),
        pltpu.VMEM((NG * 128, 512), BF16), pltpu.VMEM((NG * 128, 512), BF16),
    )


@functools.partial(jax.jit, static_argnames=("A_seg_len",))
def pallas_concat_heads__memory_aug_recurrent_mem_tr__compressed_kv_cla__prompt_kernel(
    A_x: jax.Array,
    A_mem0: jax.Array,
    A_Wq: jax.Array,
    A_Wk: jax.Array,
    A_Wv: jax.Array,
    A_Wo: jax.Array,
    A_seg_len: int,
    B_x: jax.Array,
    B_c_kv: jax.Array,
    B_w_q: jax.Array,
    B_w_uk: jax.Array,
    B_w_uv: jax.Array,
    B_w_o: jax.Array,
):
    assert A_seg_len == SEG
    assert A_x.shape == (1, S, DM) and A_mem0.shape == (1, MEM, DM)
    assert A_Wq.shape == (DM, H, DH) and A_Wo.shape == (H, DH, DM)
    assert B_x.shape == (1, S, DM) and B_c_kv.shape == (1, S, DC)
    assert B_w_q.shape == (DM, H, DH) and B_w_uk.shape == (DC, H, DH)
    assert B_w_o.shape == (H, DH, DM)

    axt = jnp.swapaxes(A_x, 1, 2).reshape(DM, S)
    bxt = jnp.swapaxes(B_x, 1, 2).reshape(DM, S)
    awot = jnp.swapaxes(A_Wo, 1, 2)
    bwot = jnp.swapaxes(B_w_o, 1, 2)

    any_spec = pl.BlockSpec(memory_space=pl.ANY)
    out = pl.pallas_call(
        _kernel,
        out_shape=jax.ShapeDtypeStruct((S, 2 * DM), BF16),
        in_specs=[any_spec, pl.BlockSpec(memory_space=pltpu.VMEM)] + [any_spec] * 10,
        out_specs=any_spec,
        scratch_shapes=[
            pltpu.VMEM((H, DC, DH), BF16),
            pltpu.VMEM((H, DC, DH), BF16),
            pltpu.VMEM((S, DC), BF16),
            pltpu.VMEM((H, DM, DH), BF16),
            pltpu.VMEM((H, S, DH), BF16),
            pltpu.VMEM((3, DM + 1, H, DH), BF16),
            pltpu.VMEM((H, DM, DH), BF16),
            pltpu.VMEM((S // 128 + 1, DM, 128), BF16),
            pltpu.SemaphoreType.DMA((13,)),
            pltpu.SemaphoreType.DMA,
        ],
        compiler_params=pltpu.CompilerParams(vmem_limit_bytes=120 * 1024 * 1024),
    )(axt, A_mem0.reshape(MEM, DM), A_Wq, A_Wk, A_Wv, awot,
      bxt, B_c_kv.reshape(S, DC), B_w_q, B_w_uk, B_w_uv, bwot)
    return out.reshape(1, S, 2 * DM)
```

```python
import functools

import jax
import jax.numpy as jnp
from jax import lax
import jax.experimental.pallas as pl
import jax.experimental.pallas.tpu as pltpu

F32 = jnp.float32
BF16 = jnp.bfloat16
NT = (((1,), (1,)), ((), ()))
NEG = -1000000000.0

S = 2048
DM = 448
H = 16
DH = 256
HD = H * DH
DC = 1024
MEM = 8
SEG = 32
L = SEG + MEM
NPAIR = S // (2 * SEG)
NG = 6

BQ = 256
HB = BQ // 2
NQ = S // BQ
PB = 512
QB = 128
KB = 128
N_OPROJ_ITERS = S // 128
N_HEAD_ITERS = H
N_PAIR_ITERS = NPAIR


def _dot(a, b):
    return jnp.dot(a, b, preferred_element_type=F32)


def _dot_nt(a, b):
    return lax.dot_general(a, b, NT, preferred_element_type=F32)


def _kernel(axt_hbm, mem0_ref, awq_hbm, awk_hbm, awv_hbm, awot_hbm,
            bxt_hbm, ckv_hbm, bwq_hbm, bwk_hbm, bwv_hbm, bwot_hbm,
            out_hbm,
            wk_s, wv_s, ckv_s, bwot_s, q_s, rawa_s, awot_s, axt_s, sems, osem):
    scale = DH ** -0.5

    def cp(src, dst, i):
        return pltpu.make_async_copy(src, dst, sems.at[i])

    cp_ckv = cp(ckv_hbm, ckv_s, 6)
    cp_bwot = cp(bwot_hbm, bwot_s, 7)
    cp_awot = cp(awot_hbm, awot_s.at[pl.ds(0, H)], 8)
    cp_axt = [cp(axt_hbm.at[:, pl.ds(j * 128, 128)], axt_s.at[j], 9)
              for j in range(S // 128)]
    cp_aw = [cp(w, rawa_s.at[t, pl.ds(0, DM)], 10 + t)
             for t, w in enumerate((awq_hbm, awk_hbm, awv_hbm))]

    def prologue(bxt_s, bx_s, rawq_s, wq_s, rawk_s, rawv_s):
        cp_bxt = [cp(bxt_hbm.at[:, pl.ds(j * 128, 128)], bxt_s.at[j], 0 if j < 4 else 1)
                  for j in range(S // 128)]
        cp_bwq = [cp(bwq_hbm.at[:, pl.ds(t * 8, 8), :], rawq_s.at[t], 2 + t)
                  for t in range(2)]
        cp_bwk = cp(bwk_hbm, rawk_s, 4)
        cp_bwv = cp(bwv_hbm, rawv_s, 5)
        for c in (cp_bwq[:1] + cp_bxt + cp_bwq[1:]
                  + [cp_bwk, cp_bwv, cp_ckv, cp_bwot, cp_awot] + cp_axt + cp_aw):
            c.start()

        def relayout(src, dst, h0, r0, n):
            w = jnp.swapaxes(src[pl.ds(r0, n)], 0, 1)
            for h in range(w.shape[0]):
                dst[h0 + h, pl.ds(r0, n), :] = w[h]

        def xpose(j):
            r0 = j * 128 if isinstance(j, int) else pl.multiple_of(j * 128, 128)
            bx_s[pl.ds(r0, 128), :] = bxt_s[j].T

        def blk(h0, nh, r_lo, r_hi, side):
            def body(i, c):
                h = h0 + i
                for r in range(r_lo, r_hi):
                    rows = slice(r * QB, (r + 1) * QB)
                    q_s[h, rows, :] = (_dot(bx_s[rows, :], wq_s[h]) * scale).astype(BF16)
                    side(i, r - r_lo)
                return c
            lax.fori_loop(0, nh, body, 0)

        def side_xpose(i, r):
            if r < 3:
                xpose(4 + i * 3 + r)

        def side_wq(i, r):
            if r < 4:
                r0 = jnp.minimum(i, DM // 64 - 1) * 64 + r * 16
                relayout(rawq_s.at[1], wq_s, 8, pl.multiple_of(r0, 16), 16)

        def side_relayout(src, dst):
            def side(i, r):
                relayout(src, dst, 0, pl.multiple_of(i * 256 + r * 16, 16), 16)
            return side

        cp_bwq[0].wait()
        for c in range(DM // 64):
            relayout(rawq_s.at[0], wq_s, 0, c * 64, 64)
        for c in cp_bxt[:4]:
            c.wait()
        for j in range(4):
            xpose(j)
        blk(0, 4, 0, 4, lambda i, r: None)
        for c in cp_bxt[4:]:
            c.wait()
        blk(4, 4, 0, 4, side_xpose)
        cp_bwq[1].wait()
        blk(0, 8, 4, 16, side_wq)
        cp_bwk.wait()
        blk(8, 4, 0, 16, side_relayout(rawk_s, wk_s))
        cp_bwv.wait()
        blk(12, 4, 0, 16, side_relayout(rawv_s, wv_s))

    pl.run_scoped(
        prologue,
        pltpu.VMEM((S // 128, DM, 128), BF16), pltpu.VMEM((S, DM), BF16),
        pltpu.VMEM((2, DM, 8, DH), BF16), pltpu.VMEM((H, DM, DH), BF16),
        pltpu.VMEM((DC, H, DH), BF16), pltpu.VMEM((DC, H, DH), BF16),
    )

    def main(wqk_s, awv_s, awo_s, wz_s, ax_s, k_s, v_s, stage_s, ot_s,
             qs0, qs1, ks0, ks1, zs0, zs1):
        cp_ckv.wait()

        tri = (lax.broadcasted_iota(jnp.int32, (HB, HB), 1)
               <= lax.broadcasted_iota(jnp.int32, (HB, HB), 0))
        tri2 = (lax.broadcasted_iota(jnp.int32, (BQ, HB), 1)
                <= lax.broadcasted_iota(jnp.int32, (BQ, HB), 0))

        def kvproj(w_ref, dst, h, pb, lo, hi):
            for r0 in range(lo, hi, pb):
                dst[r0:r0 + pb, :] = _dot(ckv_s[r0:r0 + pb, :], w_ref[h]).astype(BF16)

        def qk(h, i):
            d0 = i * BQ
            q = q_s[h, d0:d0 + BQ, :]
            so = _dot_nt(q, k_s[0:d0, :]) if i > 0 else None
            s1 = _dot_nt(q, k_s[d0:d0 + HB, :])
            s2 = _dot_nt(q[HB:], k_s[d0 + HB:d0 + BQ, :])
            return so, s1, s2

        def soft_pv_out(h, i, ss):
            so, s1, s2 = ss
            d0 = i * BQ
            s1 = jnp.where(tri2, s1, NEG)
            s2 = jnp.where(tri, s2, NEG)
            m = jnp.max(s1, axis=1, keepdims=True)
            if so is not None:
                m = jnp.maximum(m, jnp.max(so, axis=1, keepdims=True))
            mb = jnp.maximum(m[HB:], jnp.max(s2, axis=1, keepdims=True))
            m = jnp.concatenate([m[:HB], mb], axis=0)
            p1 = jnp.exp(s1 - m)
            p2 = jnp.exp(s2 - mb)
            l = jnp.sum(p1, axis=1, keepdims=True)
            acc = _dot(p1.astype(BF16), v_s[d0:d0 + HB, :])
            if so is not None:
                po = jnp.exp(so - m)
                l = l + jnp.sum(po, axis=1, keepdims=True)
                acc = acc + _dot(po.astype(BF16), v_s[0:d0, :])
            l2 = l[HB:] + jnp.sum(p2, axis=1, keepdims=True)
            acc2 = acc[HB:] + _dot(p2.astype(BF16), v_s[d0 + HB:d0 + BQ, :])
            ctx = jnp.concatenate(
                [acc[:HB] * (1.0 / l[:HB]), acc2 * (1.0 / l2)], axis=0).astype(BF16)
            q_s[h, d0:d0 + BQ, :] = ctx

        def head(h, c):
            kvproj(wk_s, k_s, h, KB, 0, S)
            order = list(range(NQ - 1, -1, -1))
            ss = qk(h, order[0])
            kvproj(wv_s, v_s, h, PB, 0, S)
            for n, i in enumerate(order):
                nxt = qk(h, order[n + 1]) if n + 1 < NQ else None
                soft_pv_out(h, i, ss)
                ss = nxt
            return c

        lax.fori_loop(0, N_HEAD_ITERS, head, 0)

        cp_bwot.wait()
        cp_awot.wait()
        for c in cp_axt + cp_aw:
            c.wait()
        ot_s[0] = jnp.zeros((DM, 128), F32)

        def flush(r0):
            stage_s[pl.ds(r0, 128), DM:2 * DM] = ot_s[0].T.astype(BF16)

        def oproj(j, c):
            r0 = pl.multiple_of(j * 128, 128)
            w0 = jnp.minimum(j, DM // 32 - 1) * 32
            pin_w = jnp.maximum(j, DM)
            pin_h = jnp.maximum(j, H)
            pin_o = jnp.where(j >= 0, 1, 0)
            acc = None
            for h in range(H):
                r = _dot_nt(bwot_s[h], q_s[h, pl.ds(r0, 128), :])
                acc = r if acc is None else acc + r
                if h == 0:
                    ot_s[pin_o, 0:8, :] = r[0:8]
                    flush(pl.multiple_of(jnp.maximum(j - 1, 0) * 128, 128))
                elif h in (3, 6, 9, 12):
                    half, g = divmod(h // 3 - 1, 2)
                    rr = pl.multiple_of(w0 + half * 16, 16)
                    rawa_s[2, pin_w, :, 0:128] = r[0:16].astype(BF16)
                    w = jnp.swapaxes(rawa_s[2, pl.ds(rr, 16), g * 8:(g + 1) * 8, :], 0, 1)
                    for u in range(8):
                        awv_s[g * 8 + u, pl.ds(rr, 16), :] = w[u]
                elif h in (4, 8):
                    e0 = (h // 4 - 1) * 128
                    awot_s[pin_h, 0:16, 0:128] = r[0:16].astype(BF16)
                    tail = awot_s[j, 384:DM, e0:e0 + 128]
                    zero = jnp.zeros_like(tail)
                    odd = (j % 2) == 1
                    wt = jnp.concatenate(
                        [awot_s[j, 0:384, e0:e0 + 128], jnp.where(odd, zero, tail),
                         jnp.where(odd, tail, zero)], axis=0)
                    awo_s[j, e0:e0 + 128, :] = wt.T
                elif h == 14:
                    axt_s[pin_h, 0:16, :] = r[0:16].astype(BF16)
                    ax_s[pl.ds(r0, 128), :] = axt_s[j].T
            ot_s[0] = acc
            return c

        lax.fori_loop(0, N_OPROJ_ITERS, oproj, 0)
        flush(S - 128)

        RC = DM // 4

        def wzprep(i, c):
            for n in range(8):
                rc, u = divmod(n, 2)
                rows = slice(rc * RC, (rc + 1) * RC)
                w = _dot(awv_s[2 * i + u, rows, :], awo_s[2 * i + u])
                wz_s[i, rows, u * 512:u * 512 + 384] = w[:, 0:384].astype(BF16)
                if u == 0:
                    mid = w[:, 384:512]
                else:
                    wz_s[i, rows, 384:512] = (mid + w[:, 384:512]).astype(BF16)
                if n < 7:
                    piece = i * 7 + n
                    t = jnp.where(piece >= DM // 16, 1, 0)
                    rr = pl.multiple_of((piece - t * (DM // 16)) * 16, 16)
                    wr = jnp.swapaxes(rawa_s[t, pl.ds(rr, 16)], 0, 1)
                    for h in range(H):
                        wqk_s[t, pl.ds(rr, 16), h * DH:(h + 1) * DH] = wr[h]
            return c

        lax.fori_loop(0, H // 2, wzprep, 0)

        for ks in (ks0, ks1):
            ks[...] = jnp.zeros_like(ks)
        for zs in (zs0, zs1):
            for g in range(NG):
                lo = 3 * L if g < NG - 1 else L
                zs[g * 128 + lo:(g + 1) * 128, :] = jnp.zeros((128 - lo, 512), BF16)

        row = lax.broadcasted_iota(jnp.int32, (3 * L, 128), 0)
        col = lax.broadcasted_iota(jnp.int32, (3 * L, 128), 1)
        off = jnp.where(row >= 2 * L, 2 * L, jnp.where(row >= L, L, 0))
        qi = row - off
        kj = col - off
        mask3 = (kj >= 0) & (kj < L) & ((qi >= SEG) | (kj >= SEG) | (kj <= qi))
        CH = 1024

        def proj_qk(lhs, t, dests):
            for jj in range(HD // CH):
                r = _dot(lhs, wqk_s[t, :, jj * CH:(jj + 1) * CH])
                if t == 0:
                    r = r * scale
                r = r.astype(BF16)
                for u in range(CH // DH):
                    g, jx = divmod(jj * (CH // DH) + u, 3)
                    for (a, n, d, b) in dests:
                        d[g, jx * L + b:jx * L + b + n, :] = r[a:a + n, u * DH:(u + 1) * DH]

        def proj_z(lhs, dests):
            for i in range(H // 2):
                r = _dot(lhs, wz_s[i])
                mid = r[:, 384:512]
                parts = [(r[:, 0:384].astype(BF16), mid.astype(BF16)),
                         (r[:, 512:896].astype(BF16), pltpu.roll(mid, 64, 1).astype(BF16))]
                for u in range(2):
                    g, jx = divmod(2 * i + u, 3)
                    for (a, n, d, b) in dests:
                        r0 = g * 128 + jx * L + b
                        d[r0:r0 + n, 0:384] = parts[u][0][a:a + n]
                        d[r0:r0 + n, 384:512] = parts[u][1][a:a + n]

        def seg(lhs, sel, w):
            def dests(refs):
                return [(a, n, refs[v], b) for (a, n, v, b) in sel]
            qs, ks, zs = (qs0, qs1), (ks0, ks1), (zs0, zs1)
            rows = [3 * L] * (NG - 1) + [L]
            proj_qk(lhs, 0, dests(qs))
            proj_qk(lhs, 1, dests(ks))
            scs = [_dot_nt(qs[w][g, 0:rows[g], :], ks[w][g]) for g in range(NG)]
            proj_z(lhs, dests(zs))
            ps = []
            for g in range(NG):
                sc = jnp.where(mask3[0:rows[g]], scs[g], NEG)
                m = jnp.max(sc, axis=1, keepdims=True)
                e = jnp.exp(sc - m)
                l = jnp.sum(e, axis=1, keepdims=True)
                p = e * (1.0 / l)
                if g < NG - 1:
                    p = p[0:L] + p[L:2 * L] + p[2 * L:3 * L]
                ps.append(p.astype(BF16))
            return _dot(jnp.concatenate(ps, axis=1), zs[w][...])[:, 0:DM].astype(BF16)

        def out_copy(base):
            return pltpu.make_async_copy(
                stage_s.at[pl.ds(base, 2 * SEG)], out_hbm.at[pl.ds(base, 2 * SEG)], osem)

        def pair(j, mem):
            base = pl.multiple_of(j * 2 * SEG, 2 * SEG)
            x0 = ax_s[pl.ds(base, SEG), :]
            x1 = ax_s[pl.ds(base + SEG, SEG), :]
            lhs1 = jnp.concatenate([x0, x1[0:8], mem], axis=0)
            out1 = seg(lhs1, [(0, 32, 0, 0), (32, 8, 1, 0), (40, 8, 0, 32)], 0)
            stage_s[pl.ds(base, SEG), 0:DM] = out1[0:SEG]
            lhs2 = jnp.concatenate([x1[16:32], out1[SEG:L], x1[8:16]], axis=0)
            out2 = seg(lhs2, [(0, 16, 1, 16), (16, 8, 1, 32), (24, 8, 1, 8)], 1)
            stage_s[pl.ds(base + SEG, SEG), 0:DM] = out2[0:SEG]
            out_copy(base).start()
            return out2[SEG:L]

        lax.fori_loop(0, N_PAIR_ITERS, pair, mem0_ref[...])
        for j in range(N_PAIR_ITERS):
            out_copy(j * 2 * SEG).wait()

    pl.run_scoped(
        main,
        pltpu.VMEM((2, DM, HD), BF16), pltpu.VMEM((H, DM, DH), BF16),
        pltpu.VMEM((H, DH, 512), BF16),
        pltpu.VMEM((H // 2, DM, 2 * DM), BF16), pltpu.VMEM((S, DM), BF16),
        pltpu.VMEM((S, DH), BF16), pltpu.VMEM((S, DH), BF16),
        pltpu.VMEM((S, 2 * DM), BF16), pltpu.VMEM((2, DM, 128), F32),
        pltpu.VMEM((NG, 128, DH), BF16), pltpu.VMEM((NG, 128, DH), BF16),
        pltpu.VMEM((NG, 128, DH), BF16), pltpu.VMEM((NG, 128, DH), BF16),
        pltpu.VMEM((NG * 128, 512), BF16), pltpu.VMEM((NG * 128, 512), BF16),
    )


@functools.partial(jax.jit, static_argnames=("A_seg_len",))
def pallas_concat_heads__memory_aug_recurrent_mem_tr__compressed_kv_cla__prompt_kernel(
    A_x: jax.Array,
    A_mem0: jax.Array,
    A_Wq: jax.Array,
    A_Wk: jax.Array,
    A_Wv: jax.Array,
    A_Wo: jax.Array,
    A_seg_len: int,
    B_x: jax.Array,
    B_c_kv: jax.Array,
    B_w_q: jax.Array,
    B_w_uk: jax.Array,
    B_w_uv: jax.Array,
    B_w_o: jax.Array,
):
    assert A_seg_len == SEG
    assert A_x.shape == (1, S, DM) and A_mem0.shape == (1, MEM, DM)
    assert A_Wq.shape == (DM, H, DH) and A_Wo.shape == (H, DH, DM)
    assert B_x.shape == (1, S, DM) and B_c_kv.shape == (1, S, DC)
    assert B_w_q.shape == (DM, H, DH) and B_w_uk.shape == (DC, H, DH)
    assert B_w_o.shape == (H, DH, DM)

    axt = jnp.swapaxes(A_x, 1, 2).reshape(DM, S)
    bxt = jnp.swapaxes(B_x, 1, 2).reshape(DM, S)
    awot = jnp.swapaxes(A_Wo, 1, 2)
    bwot = jnp.swapaxes(B_w_o, 1, 2)

    any_spec = pl.BlockSpec(memory_space=pl.ANY)
    out = pl.pallas_call(
        _kernel,
        out_shape=jax.ShapeDtypeStruct((S, 2 * DM), BF16),
        in_specs=[any_spec, pl.BlockSpec(memory_space=pltpu.VMEM)] + [any_spec] * 10,
        out_specs=any_spec,
        scratch_shapes=[
            pltpu.VMEM((H, DC, DH), BF16),
            pltpu.VMEM((H, DC, DH), BF16),
            pltpu.VMEM((S, DC), BF16),
            pltpu.VMEM((H, DM, DH), BF16),
            pltpu.VMEM((H, S, DH), BF16),
            pltpu.VMEM((3, DM + 1, H, DH), BF16),
            pltpu.VMEM((H + 1, DM, DH), BF16),
            pltpu.VMEM((S // 128 + 1, DM, 128), BF16),
            pltpu.SemaphoreType.DMA((13,)),
            pltpu.SemaphoreType.DMA,
        ],
        compiler_params=pltpu.CompilerParams(vmem_limit_bytes=120 * 1024 * 1024),
    )(axt, A_mem0.reshape(MEM, DM), A_Wq, A_Wk, A_Wv, awot,
      bxt, B_c_kv.reshape(S, DC), B_w_q, B_w_uk, B_w_uv, bwot)
    return out.reshape(1, S, 2 * DM)
```

```python
import functools

import jax
import jax.numpy as jnp
from jax import lax
import jax.experimental.pallas as pl
import jax.experimental.pallas.tpu as pltpu

F32 = jnp.float32
BF16 = jnp.bfloat16
NT = (((1,), (1,)), ((), ()))
NEG = -1000000000.0

S = 2048
DM = 448
H = 16
DH = 256
HD = H * DH
DC = 1024
MEM = 8
SEG = 32
L = SEG + MEM
NPAIR = S // (2 * SEG)
NG = 6

BQ = 256
HB = BQ // 2
NQ = S // BQ
PB = 512
QB = 128
KB = 128
N_OPROJ_ITERS = S // 128
N_HEAD_ITERS = H
N_PAIR_ITERS = NPAIR


def _dot(a, b):
    return jnp.dot(a, b, preferred_element_type=F32)


def _dot_nt(a, b):
    return lax.dot_general(a, b, NT, preferred_element_type=F32)


def _recip(l):
    r = pl.reciprocal(l, approx=True)
    return r * (2.0 - l * r)


def _kernel(axt_hbm, mem0_ref, awq_hbm, awk_hbm, awv_hbm, awot_hbm,
            bxt_hbm, ckv_hbm, bwq_hbm, bwk_hbm, bwv_hbm, bwot_hbm,
            out_hbm,
            wk_s, wv_s, ckv_s, bwot_s, q_s, rawa_s, awot_s, axt_s, sems, osem):
    scale = DH ** -0.5

    def cp(src, dst, i):
        return pltpu.make_async_copy(src, dst, sems.at[i])

    cp_ckv = cp(ckv_hbm, ckv_s, 6)
    cp_bwot = cp(bwot_hbm, bwot_s, 7)
    cp_awot = cp(awot_hbm, awot_s.at[pl.ds(0, H)], 8)
    cp_axt = [cp(axt_hbm.at[:, pl.ds(j * 128, 128)], axt_s.at[j], 9)
              for j in range(S // 128)]
    cp_aw = [cp(w, rawa_s.at[t, pl.ds(0, DM)], 10 + t)
             for t, w in enumerate((awq_hbm, awk_hbm, awv_hbm))]

    def prologue(bxt_s, bx_s, rawq_s, wq_s, rawk_s, rawv_s):
        cp_bxt = [cp(bxt_hbm.at[:, pl.ds(j * 128, 128)], bxt_s.at[j], 0 if j < 4 else 1)
                  for j in range(S // 128)]
        cp_bwq = [cp(bwq_hbm.at[:, pl.ds(t * 8, 8), :], rawq_s.at[t], 2 + t)
                  for t in range(2)]
        cp_bwk = cp(bwk_hbm, rawk_s, 4)
        cp_bwv = cp(bwv_hbm, rawv_s, 5)
        for c in (cp_bwq[:1] + cp_bxt + cp_bwq[1:]
                  + [cp_bwk, cp_bwv, cp_ckv, cp_bwot, cp_awot] + cp_axt + cp_aw):
            c.start()

        def relayout(src, dst, h0, r0, n):
            w = jnp.swapaxes(src[pl.ds(r0, n)], 0, 1)
            for h in range(w.shape[0]):
                dst[h0 + h, pl.ds(r0, n), :] = w[h]

        def xpose(j):
            r0 = j * 128 if isinstance(j, int) else pl.multiple_of(j * 128, 128)
            bx_s[pl.ds(r0, 128), :] = bxt_s[j].T

        def blk(h0, nh, r_lo, r_hi, side):
            def body(i, c):
                h = h0 + i
                for r in range(r_lo, r_hi):
                    rows = slice(r * QB, (r + 1) * QB)
                    q_s[h, rows, :] = (_dot(bx_s[rows, :], wq_s[h]) * scale).astype(BF16)
                    side(i, r - r_lo)
                return c
            lax.fori_loop(0, nh, body, 0)

        def side_xpose(i, r):
            if r < 3:
                xpose(4 + i * 3 + r)

        def side_wq(i, r):
            if r < 4:
                r0 = jnp.minimum(i, DM // 64 - 1) * 64 + r * 16
                relayout(rawq_s.at[1], wq_s, 8, pl.multiple_of(r0, 16), 16)

        def side_relayout(src, dst):
            def side(i, r):
                relayout(src, dst, 0, pl.multiple_of(i * 256 + r * 16, 16), 16)
            return side

        cp_bwq[0].wait()
        for c in range(DM // 64):
            relayout(rawq_s.at[0], wq_s, 0, c * 64, 64)
        for c in cp_bxt[:4]:
            c.wait()
        for j in range(4):
            xpose(j)
        blk(0, 4, 0, 4, lambda i, r: None)
        for c in cp_bxt[4:]:
            c.wait()
        blk(4, 4, 0, 4, side_xpose)
        cp_bwq[1].wait()
        blk(0, 8, 4, 16, side_wq)
        cp_bwk.wait()
        blk(8, 4, 0, 16, side_relayout(rawk_s, wk_s))
        cp_bwv.wait()
        blk(12, 4, 0, 16, side_relayout(rawv_s, wv_s))

    pl.run_scoped(
        prologue,
        pltpu.VMEM((S // 128, DM, 128), BF16), pltpu.VMEM((S, DM), BF16),
        pltpu.VMEM((2, DM, 8, DH), BF16), pltpu.VMEM((H, DM, DH), BF16),
        pltpu.VMEM((DC, H, DH), BF16), pltpu.VMEM((DC, H, DH), BF16),
    )

    def main(wqk_s, awv_s, awo_s, wz_s, ax_s, k_s, v_s, stage_s, ot_s,
             qs0, qs1, ks0, ks1, zs0, zs1):
        cp_ckv.wait()

        tri = (lax.broadcasted_iota(jnp.int32, (HB, HB), 1)
               <= lax.broadcasted_iota(jnp.int32, (HB, HB), 0))
        tri2 = (lax.broadcasted_iota(jnp.int32, (BQ, HB), 1)
                <= lax.broadcasted_iota(jnp.int32, (BQ, HB), 0))

        def kvproj(w_ref, dst, h, pb, lo, hi):
            for r0 in range(lo, hi, pb):
                dst[r0:r0 + pb, :] = _dot(ckv_s[r0:r0 + pb, :], w_ref[h]).astype(BF16)

        def qk(h, i):
            d0 = i * BQ
            q = q_s[h, d0:d0 + BQ, :]
            so = _dot_nt(q, k_s[0:d0, :]) if i > 0 else None
            s1 = _dot_nt(q, k_s[d0:d0 + HB, :])
            s2 = _dot_nt(q[HB:], k_s[d0 + HB:d0 + BQ, :])
            return so, s1, s2

        def soft_pv_out(h, i, ss):
            so, s1, s2 = ss
            d0 = i * BQ
            s1 = jnp.where(tri2, s1, NEG)
            s2 = jnp.where(tri, s2, NEG)
            m = jnp.max(s1, axis=1, keepdims=True)
            if so is not None:
                m = jnp.maximum(m, jnp.max(so, axis=1, keepdims=True))
            mb = jnp.maximum(m[HB:], jnp.max(s2, axis=1, keepdims=True))
            m = jnp.concatenate([m[:HB], mb], axis=0)
            p1 = jnp.exp(s1 - m)
            p2 = jnp.exp(s2 - mb)
            l = jnp.sum(p1, axis=1, keepdims=True)
            acc = _dot(p1.astype(BF16), v_s[d0:d0 + HB, :])
            if so is not None:
                po = jnp.exp(so - m)
                l = l + jnp.sum(po, axis=1, keepdims=True)
                acc = acc + _dot(po.astype(BF16), v_s[0:d0, :])
            l2 = l[HB:] + jnp.sum(p2, axis=1, keepdims=True)
            acc2 = acc[HB:] + _dot(p2.astype(BF16), v_s[d0 + HB:d0 + BQ, :])
            ctx = jnp.concatenate(
                [acc[:HB] * _recip(l[:HB]), acc2 * _recip(l2)], axis=0).astype(BF16)
            q_s[h, d0:d0 + BQ, :] = ctx

        def head(h, c):
            kvproj(wk_s, k_s, h, KB, 0, S)
            order = list(range(NQ - 1, -1, -1))
            ss = qk(h, order[0])
            kvproj(wv_s, v_s, h, PB, 0, S)
            for n, i in enumerate(order):
                nxt = qk(h, order[n + 1]) if n + 1 < NQ else None
                soft_pv_out(h, i, ss)
                ss = nxt
            return c

        lax.fori_loop(0, N_HEAD_ITERS, head, 0)

        cp_bwot.wait()
        cp_awot.wait()
        for c in cp_axt + cp_aw:
            c.wait()
        ot_s[0] = jnp.zeros((DM, 128), F32)

        def flush(r0):
            stage_s[pl.ds(r0, 128), DM:2 * DM] = ot_s[0].T.astype(BF16)

        def oproj(j, c):
            r0 = pl.multiple_of(j * 128, 128)
            w0 = jnp.minimum(j, DM // 32 - 1) * 32
            pin_w = jnp.maximum(j, DM)
            pin_h = jnp.maximum(j, H)
            pin_o = jnp.where(j >= 0, 1, 0)
            acc = None
            for h in range(H):
                r = _dot_nt(bwot_s[h], q_s[h, pl.ds(r0, 128), :])
                acc = r if acc is None else acc + r
                if h == 0:
                    ot_s[pin_o, 0:8, :] = r[0:8]
                    flush(pl.multiple_of(jnp.maximum(j - 1, 0) * 128, 128))
                elif h in (3, 6, 9, 12):
                    half, g = divmod(h // 3 - 1, 2)
                    rr = pl.multiple_of(w0 + half * 16, 16)
                    rawa_s[2, pin_w, :, 0:128] = r[0:16].astype(BF16)
                    w = jnp.swapaxes(rawa_s[2, pl.ds(rr, 16), g * 8:(g + 1) * 8, :], 0, 1)
                    for u in range(8):
                        awv_s[g * 8 + u, pl.ds(rr, 16), :] = w[u]
                elif h in (4, 8):
                    e0 = (h // 4 - 1) * 128
                    awot_s[pin_h, 0:16, 0:128] = r[0:16].astype(BF16)
                    tail = awot_s[j, 384:DM, e0:e0 + 128]
                    zero = jnp.zeros_like(tail)
                    odd = (j % 2) == 1
                    wt = jnp.concatenate(
                        [awot_s[j, 0:384, e0:e0 + 128], jnp.where(odd, zero, tail),
                         jnp.where(odd, tail, zero)], axis=0)
                    awo_s[j, e0:e0 + 128, :] = wt.T
                elif h == 14:
                    axt_s[pin_h, 0:16, :] = r[0:16].astype(BF16)
                    ax_s[pl.ds(r0, 128), :] = axt_s[j].T
            ot_s[0] = acc
            return c

        lax.fori_loop(0, N_OPROJ_ITERS, oproj, 0)
        flush(S - 128)

        RC = DM // 4

        def wzprep(i, c):
            for n in range(8):
                rc, u = divmod(n, 2)
                rows = slice(rc * RC, (rc + 1) * RC)
                w = _dot(awv_s[2 * i + u, rows, :], awo_s[2 * i + u])
                wz_s[i, rows, u * 512:u * 512 + 384] = w[:, 0:384].astype(BF16)
                if u == 0:
                    mid = w[:, 384:512]
                else:
                    wz_s[i, rows, 384:512] = (mid + w[:, 384:512]).astype(BF16)
                if n < 7:
                    piece = i * 7 + n
                    t = jnp.where(piece >= DM // 16, 1, 0)
                    rr = pl.multiple_of((piece - t * (DM // 16)) * 16, 16)
                    wr = jnp.swapaxes(rawa_s[t, pl.ds(rr, 16)], 0, 1)
                    for h in range(H):
                        wqk_s[t, pl.ds(rr, 16), h * DH:(h + 1) * DH] = wr[h]
            return c

        lax.fori_loop(0, H // 2, wzprep, 0)

        for ks in (ks0, ks1):
            ks[...] = jnp.zeros_like(ks)
        for zs in (zs0, zs1):
            for g in range(NG):
                lo = 3 * L if g < NG - 1 else L
                zs[g * 128 + lo:(g + 1) * 128, :] = jnp.zeros((128 - lo, 512), BF16)

        row = lax.broadcasted_iota(jnp.int32, (3 * L, 128), 0)
        col = lax.broadcasted_iota(jnp.int32, (3 * L, 128), 1)
        off = jnp.where(row >= 2 * L, 2 * L, jnp.where(row >= L, L, 0))
        qi = row - off
        kj = col - off
        mask3 = (kj >= 0) & (kj < L) & ((qi >= SEG) | (kj >= SEG) | (kj <= qi))
        CH = 1024

        def proj_qk(lhs, t, dests):
            for jj in range(HD // CH):
                r = _dot(lhs, wqk_s[t, :, jj * CH:(jj + 1) * CH])
                if t == 0:
                    r = r * scale
                r = r.astype(BF16)
                for u in range(CH // DH):
                    g, jx = divmod(jj * (CH // DH) + u, 3)
                    for (a, n, d, b) in dests:
                        d[g, jx * L + b:jx * L + b + n, :] = r[a:a + n, u * DH:(u + 1) * DH]

        def proj_z(lhs, dests):
            for i in range(H // 2):
                r = _dot(lhs, wz_s[i])
                mid = r[:, 384:512]
                parts = [(r[:, 0:384].astype(BF16), mid.astype(BF16)),
                         (r[:, 512:896].astype(BF16), pltpu.roll(mid, 64, 1).astype(BF16))]
                for u in range(2):
                    g, jx = divmod(2 * i + u, 3)
                    for (a, n, d, b) in dests:
                        r0 = g * 128 + jx * L + b
                        d[r0:r0 + n, 0:384] = parts[u][0][a:a + n]
                        d[r0:r0 + n, 384:512] = parts[u][1][a:a + n]

        def seg(lhs, sel, w):
            def dests(refs):
                return [(a, n, refs[v], b) for (a, n, v, b) in sel]
            qs, ks, zs = (qs0, qs1), (ks0, ks1), (zs0, zs1)
            rows = [3 * L] * (NG - 1) + [L]
            proj_qk(lhs, 0, dests(qs))
            proj_qk(lhs, 1, dests(ks))
            scs = [_dot_nt(qs[w][g, 0:rows[g], :], ks[w][g]) for g in range(NG)]
            proj_z(lhs, dests(zs))
            ps = []
            for g in range(NG):
                sc = jnp.where(mask3[0:rows[g]], scs[g], NEG)
                m = jnp.max(sc, axis=1, keepdims=True)
                e = jnp.exp(sc - m)
                l = jnp.sum(e, axis=1, keepdims=True)
                p = e * _recip(l)
                if g < NG - 1:
                    p = p[0:L] + p[L:2 * L] + p[2 * L:3 * L]
                ps.append(p.astype(BF16))
            return _dot(jnp.concatenate(ps, axis=1), zs[w][...])[:, 0:DM].astype(BF16)

        def out_copy(base):
            return pltpu.make_async_copy(
                stage_s.at[pl.ds(base, 2 * SEG)], out_hbm.at[pl.ds(base, 2 * SEG)], osem)

        def pair(j, mem):
            base = pl.multiple_of(j * 2 * SEG, 2 * SEG)
            x0 = ax_s[pl.ds(base, SEG), :]
            x1 = ax_s[pl.ds(base + SEG, SEG), :]
            lhs1 = jnp.concatenate([x0, x1[0:8], mem], axis=0)
            out1 = seg(lhs1, [(0, 32, 0, 0), (32, 8, 1, 0), (40, 8, 0, 32)], 0)
            stage_s[pl.ds(base, SEG), 0:DM] = out1[0:SEG]
            lhs2 = jnp.concatenate([x1[16:32], out1[SEG:L], x1[8:16]], axis=0)
            out2 = seg(lhs2, [(0, 16, 1, 16), (16, 8, 1, 32), (24, 8, 1, 8)], 1)
            stage_s[pl.ds(base + SEG, SEG), 0:DM] = out2[0:SEG]
            out_copy(base).start()
            return out2[SEG:L]

        lax.fori_loop(0, N_PAIR_ITERS, pair, mem0_ref[...])
        for j in range(N_PAIR_ITERS):
            out_copy(j * 2 * SEG).wait()

    pl.run_scoped(
        main,
        pltpu.VMEM((2, DM, HD), BF16), pltpu.VMEM((H, DM, DH), BF16),
        pltpu.VMEM((H, DH, 512), BF16),
        pltpu.VMEM((H // 2, DM, 2 * DM), BF16), pltpu.VMEM((S, DM), BF16),
        pltpu.VMEM((S, DH), BF16), pltpu.VMEM((S, DH), BF16),
        pltpu.VMEM((S, 2 * DM), BF16), pltpu.VMEM((2, DM, 128), F32),
        pltpu.VMEM((NG, 128, DH), BF16), pltpu.VMEM((NG, 128, DH), BF16),
        pltpu.VMEM((NG, 128, DH), BF16), pltpu.VMEM((NG, 128, DH), BF16),
        pltpu.VMEM((NG * 128, 512), BF16), pltpu.VMEM((NG * 128, 512), BF16),
    )


@functools.partial(jax.jit, static_argnames=("A_seg_len",))
def pallas_concat_heads__memory_aug_recurrent_mem_tr__compressed_kv_cla__prompt_kernel(
    A_x: jax.Array,
    A_mem0: jax.Array,
    A_Wq: jax.Array,
    A_Wk: jax.Array,
    A_Wv: jax.Array,
    A_Wo: jax.Array,
    A_seg_len: int,
    B_x: jax.Array,
    B_c_kv: jax.Array,
    B_w_q: jax.Array,
    B_w_uk: jax.Array,
    B_w_uv: jax.Array,
    B_w_o: jax.Array,
):
    assert A_seg_len == SEG
    assert A_x.shape == (1, S, DM) and A_mem0.shape == (1, MEM, DM)
    assert A_Wq.shape == (DM, H, DH) and A_Wo.shape == (H, DH, DM)
    assert B_x.shape == (1, S, DM) and B_c_kv.shape == (1, S, DC)
    assert B_w_q.shape == (DM, H, DH) and B_w_uk.shape == (DC, H, DH)
    assert B_w_o.shape == (H, DH, DM)

    axt = jnp.swapaxes(A_x, 1, 2).reshape(DM, S)
    bxt = jnp.swapaxes(B_x, 1, 2).reshape(DM, S)
    awot = jnp.swapaxes(A_Wo, 1, 2)
    bwot = jnp.swapaxes(B_w_o, 1, 2)

    any_spec = pl.BlockSpec(memory_space=pl.ANY)
    out = pl.pallas_call(
        _kernel,
        out_shape=jax.ShapeDtypeStruct((S, 2 * DM), BF16),
        in_specs=[any_spec, pl.BlockSpec(memory_space=pltpu.VMEM)] + [any_spec] * 10,
        out_specs=any_spec,
        scratch_shapes=[
            pltpu.VMEM((H, DC, DH), BF16),
            pltpu.VMEM((H, DC, DH), BF16),
            pltpu.VMEM((S, DC), BF16),
            pltpu.VMEM((H, DM, DH), BF16),
            pltpu.VMEM((H, S, DH), BF16),
            pltpu.VMEM((3, DM + 1, H, DH), BF16),
            pltpu.VMEM((H + 1, DM, DH), BF16),
            pltpu.VMEM((S // 128 + 1, DM, 128), BF16),
            pltpu.SemaphoreType.DMA((13,)),
            pltpu.SemaphoreType.DMA,
        ],
        compiler_params=pltpu.CompilerParams(vmem_limit_bytes=120 * 1024 * 1024),
    )(axt, A_mem0.reshape(MEM, DM), A_Wq, A_Wk, A_Wv, awot,
      bxt, B_c_kv.reshape(S, DC), B_w_q, B_w_uk, B_w_uv, bwot)
    return out.reshape(1, S, 2 * DM)
```

```python
import functools

import jax
import jax.numpy as jnp
from jax import lax
import jax.experimental.pallas as pl
import jax.experimental.pallas.tpu as pltpu

F32 = jnp.float32
BF16 = jnp.bfloat16
NT = (((1,), (1,)), ((), ()))
NEG = -1000000000.0

S = 2048
DM = 448
H = 16
DH = 256
HD = H * DH
DC = 1024
MEM = 8
SEG = 32
L = SEG + MEM
NPAIR = S // (2 * SEG)
NG = 6

BQ = 256
HB = BQ // 2
NQ = S // BQ
PB = 512
QB = 128
KB = 128
N_OPROJ_ITERS = S // 128
N_HEAD_ITERS = H
N_PAIR_ITERS = NPAIR


def _dot(a, b):
    return jnp.dot(a, b, preferred_element_type=F32)


def _dot_nt(a, b):
    return lax.dot_general(a, b, NT, preferred_element_type=F32)


def _recip(l):
    r = pl.reciprocal(l, approx=True)
    return r * (2.0 - l * r)


def _kernel(axt_hbm, mem0_hbm, awq_hbm, awk_hbm, awv_hbm, awot_hbm,
            bxt_hbm, ckv_hbm, bwq_hbm, bwk_hbm, bwv_hbm, bwot_hbm,
            out_hbm,
            wk_s, wv_s, ckv_s, bwot_s, q_s, rawa_s, awot_s, axt_s, mem0_s,
            sems, osem):
    scale = DH ** -0.5

    def cp(src, dst, i):
        return pltpu.make_async_copy(src, dst, sems.at[i])

    cp_ckv = cp(ckv_hbm, ckv_s, 6)
    cp_bwot = cp(bwot_hbm, bwot_s, 7)
    cp_awot = cp(awot_hbm, awot_s.at[pl.ds(0, H)], 8)
    cp_axt = [cp(axt_hbm.at[:, pl.ds(j * 128, 128)], axt_s.at[j], 9)
              for j in range(S // 128)]
    cp_aw = [cp(w, rawa_s.at[t, pl.ds(0, DM)], 10 + t)
             for t, w in enumerate((awq_hbm, awk_hbm, awv_hbm))]

    cp_mem0 = cp(mem0_hbm, mem0_s, 13)

    def prologue(bxt_s, bx_s, rawq_s, wq_s, rawk_s, rawv_s):
        cp_bxt = [cp(bxt_hbm.at[:, pl.ds(j * 128, 128)], bxt_s.at[j], 0 if j < 4 else 1)
                  for j in range(S // 128)]
        RQ = DM // 4
        cp_bwq_lo = [cp(bwq_hbm.at[pl.ds(c * RQ, RQ), pl.ds(0, 8), :],
                        rawq_s.at[0, pl.ds(c * RQ, RQ)], 14 + c) for c in range(4)]
        cp_bwq_hi = cp(bwq_hbm.at[:, pl.ds(8, 8), :], rawq_s.at[1], 3)
        cp_bwk = cp(bwk_hbm, rawk_s, 4)
        cp_bwv = cp(bwv_hbm, rawv_s, 5)
        for c in (cp_bxt[:4] + cp_bwq_lo + cp_bxt[4:]
                  + [cp_bwq_hi, cp_bwk, cp_bwv, cp_ckv, cp_bwot, cp_awot] + cp_axt
                  + cp_aw + [cp_mem0]):
            c.start()

        def relayout(src, dst, h0, r0, n):
            w = jnp.swapaxes(src[pl.ds(r0, n)], 0, 1)
            for h in range(w.shape[0]):
                dst[h0 + h, pl.ds(r0, n), :] = w[h]

        def xpose(j):
            r0 = j * 128 if isinstance(j, int) else pl.multiple_of(j * 128, 128)
            bx_s[pl.ds(r0, 128), :] = bxt_s[j].T

        def blk(h0, nh, r_lo, r_hi, side):
            def body(i, c):
                h = h0 + i
                for r in range(r_lo, r_hi):
                    rows = slice(r * QB, (r + 1) * QB)
                    q_s[h, rows, :] = (_dot(bx_s[rows, :], wq_s[h]) * scale).astype(BF16)
                    side(i, r - r_lo)
                return c
            lax.fori_loop(0, nh, body, 0)

        def side_xpose(i, r):
            if r < 3:
                xpose(4 + i * 3 + r)

        def side_wq(i, r):
            if r < 4:
                r0 = jnp.minimum(i, DM // 64 - 1) * 64 + r * 16
                relayout(rawq_s.at[1], wq_s, 8, pl.multiple_of(r0, 16), 16)

        def side_relayout(src, dst):
            def side(i, r):
                relayout(src, dst, 0, pl.multiple_of(i * 256 + r * 16, 16), 16)
            return side

        for c in cp_bxt[:4]:
            c.wait()
        for j in range(4):
            xpose(j)
        for c in range(4):
            cp_bwq_lo[c].wait()
            relayout(rawq_s.at[0], wq_s, 0, c * RQ, RQ)
        blk(0, 4, 0, 4, lambda i, r: None)
        for c in cp_bxt[4:]:
            c.wait()
        blk(4, 4, 0, 4, side_xpose)
        cp_bwq_hi.wait()
        blk(0, 8, 4, 16, side_wq)
        cp_bwk.wait()
        blk(8, 4, 0, 16, side_relayout(rawk_s, wk_s))
        cp_bwv.wait()
        blk(12, 4, 0, 16, side_relayout(rawv_s, wv_s))

    pl.run_scoped(
        prologue,
        pltpu.VMEM((S // 128, DM, 128), BF16), pltpu.VMEM((S, DM), BF16),
        pltpu.VMEM((2, DM, 8, DH), BF16), pltpu.VMEM((H, DM, DH), BF16),
        pltpu.VMEM((DC, H, DH), BF16), pltpu.VMEM((DC, H, DH), BF16),
    )

    def main(wqk_s, awv_s, awo_s, wz_s, ax_s, k_s, v_s, stage_s, ot_s,
             qs0, qs1, ks0, ks1, zs0, zs1):
        cp_ckv.wait()

        tri = (lax.broadcasted_iota(jnp.int32, (HB, HB), 1)
               <= lax.broadcasted_iota(jnp.int32, (HB, HB), 0))
        tri2 = (lax.broadcasted_iota(jnp.int32, (BQ, HB), 1)
                <= lax.broadcasted_iota(jnp.int32, (BQ, HB), 0))

        def kvproj(w_ref, dst, h, pb, lo, hi):
            for r0 in range(lo, hi, pb):
                dst[r0:r0 + pb, :] = _dot(ckv_s[r0:r0 + pb, :], w_ref[h]).astype(BF16)

        def qk(h, i):
            d0 = i * BQ
            q = q_s[h, d0:d0 + BQ, :]
            so = _dot_nt(q, k_s[0:d0, :]) if i > 0 else None
            s1 = _dot_nt(q, k_s[d0:d0 + HB, :])
            s2 = _dot_nt(q[HB:], k_s[d0 + HB:d0 + BQ, :])
            return so, s1, s2

        def soft_pv_out(h, i, ss):
            so, s1, s2 = ss
            d0 = i * BQ
            s1 = jnp.where(tri2, s1, NEG)
            s2 = jnp.where(tri, s2, NEG)
            m = jnp.max(s1, axis=1, keepdims=True)
            if so is not None:
                m = jnp.maximum(m, jnp.max(so, axis=1, keepdims=True))
            mb = jnp.maximum(m[HB:], jnp.max(s2, axis=1, keepdims=True))
            m = jnp.concatenate([m[:HB], mb], axis=0)
            p1 = jnp.exp(s1 - m)
            p2 = jnp.exp(s2 - mb)
            l = jnp.sum(p1, axis=1, keepdims=True)
            acc = _dot(p1.astype(BF16), v_s[d0:d0 + HB, :])
            if so is not None:
                po = jnp.exp(so - m)
                l = l + jnp.sum(po, axis=1, keepdims=True)
                acc = acc + _dot(po.astype(BF16), v_s[0:d0, :])
            l2 = l[HB:] + jnp.sum(p2, axis=1, keepdims=True)
            acc2 = acc[HB:] + _dot(p2.astype(BF16), v_s[d0 + HB:d0 + BQ, :])
            ctx = jnp.concatenate(
                [acc[:HB] * _recip(l[:HB]), acc2 * _recip(l2)], axis=0).astype(BF16)
            q_s[h, d0:d0 + BQ, :] = ctx

        def head(h, c):
            kvproj(wk_s, k_s, h, KB, 0, S)
            order = list(range(NQ - 1, -1, -1))
            ss = qk(h, order[0])
            kvproj(wv_s, v_s, h, PB, 0, S)
            for n, i in enumerate(order):
                nxt = qk(h, order[n + 1]) if n + 1 < NQ else None
                soft_pv_out(h, i, ss)
                ss = nxt
            return c

        lax.fori_loop(0, N_HEAD_ITERS, head, 0)

        cp_bwot.wait()
        cp_awot.wait()
        for c in cp_axt + cp_aw + [cp_mem0]:
            c.wait()
        ot_s[0] = jnp.zeros((DM, 128), F32)

        def flush(r0):
            stage_s[pl.ds(r0, 128), DM:2 * DM] = ot_s[0].T.astype(BF16)

        def oproj(j, c):
            r0 = pl.multiple_of(j * 128, 128)
            w0 = jnp.minimum(j, DM // 32 - 1) * 32
            pin_w = jnp.maximum(j, DM)
            pin_h = jnp.maximum(j, H)
            pin_o = jnp.where(j >= 0, 1, 0)
            acc = None
            for h in range(H):
                r = _dot_nt(bwot_s[h], q_s[h, pl.ds(r0, 128), :])
                acc = r if acc is None else acc + r
                if h == 0:
                    ot_s[pin_o, 0:8, :] = r[0:8]
                    flush(pl.multiple_of(jnp.maximum(j - 1, 0) * 128, 128))
                elif h in (3, 6, 9, 12):
                    half, g = divmod(h // 3 - 1, 2)
                    rr = pl.multiple_of(w0 + half * 16, 16)
                    rawa_s[2, pin_w, :, 0:128] = r[0:16].astype(BF16)
                    w = jnp.swapaxes(rawa_s[2, pl.ds(rr, 16), g * 8:(g + 1) * 8, :], 0, 1)
                    for u in range(8):
                        awv_s[g * 8 + u, pl.ds(rr, 16), :] = w[u]
                elif h in (4, 8):
                    e0 = (h // 4 - 1) * 128
                    awot_s[pin_h, 0:16, 0:128] = r[0:16].astype(BF16)
                    tail = awot_s[j, 384:DM, e0:e0 + 128]
                    zero = jnp.zeros_like(tail)
                    odd = (j % 2) == 1
                    wt = jnp.concatenate(
                        [awot_s[j, 0:384, e0:e0 + 128], jnp.where(odd, zero, tail),
                         jnp.where(odd, tail, zero)], axis=0)
                    awo_s[j, e0:e0 + 128, :] = wt.T
                elif h == 14:
                    axt_s[pin_h, 0:16, :] = r[0:16].astype(BF16)
                    ax_s[pl.ds(r0, 128), :] = axt_s[j].T
            ot_s[0] = acc
            return c

        lax.fori_loop(0, N_OPROJ_ITERS, oproj, 0)
        flush(S - 128)

        RC = DM // 4

        def wzprep(i, c):
            for n in range(8):
                rc, u = divmod(n, 2)
                rows = slice(rc * RC, (rc + 1) * RC)
                w = _dot(awv_s[2 * i + u, rows, :], awo_s[2 * i + u])
                wz_s[i, rows, u * 512:u * 512 + 384] = w[:, 0:384].astype(BF16)
                if u == 0:
                    mid = w[:, 384:512]
                else:
                    wz_s[i, rows, 384:512] = (mid + w[:, 384:512]).astype(BF16)
                if n < 7:
                    piece = i * 7 + n
                    t = jnp.where(piece >= DM // 16, 1, 0)
                    rr = pl.multiple_of((piece - t * (DM // 16)) * 16, 16)
                    wr = jnp.swapaxes(rawa_s[t, pl.ds(rr, 16)], 0, 1)
                    for h in range(H):
                        wqk_s[t, pl.ds(rr, 16), h * DH:(h + 1) * DH] = wr[h]
            return c

        lax.fori_loop(0, H // 2, wzprep, 0)

        for ks in (ks0, ks1):
            ks[...] = jnp.zeros_like(ks)
        for zs in (zs0, zs1):
            for g in range(NG):
                lo = 3 * L if g < NG - 1 else L
                zs[g * 128 + lo:(g + 1) * 128, :] = jnp.zeros((128 - lo, 512), BF16)

        row = lax.broadcasted_iota(jnp.int32, (3 * L, 128), 0)
        col = lax.broadcasted_iota(jnp.int32, (3 * L, 128), 1)
        off = jnp.where(row >= 2 * L, 2 * L, jnp.where(row >= L, L, 0))
        qi = row - off
        kj = col - off
        mask3 = (kj >= 0) & (kj < L) & ((qi >= SEG) | (kj >= SEG) | (kj <= qi))
        CH = 1024

        def proj_qk(lhs, t, dests):
            for jj in range(HD // CH):
                r = _dot(lhs, wqk_s[t, :, jj * CH:(jj + 1) * CH])
                if t == 0:
                    r = r * scale
                r = r.astype(BF16)
                for u in range(CH // DH):
                    g, jx = divmod(jj * (CH // DH) + u, 3)
                    for (a, n, d, b) in dests:
                        d[g, jx * L + b:jx * L + b + n, :] = r[a:a + n, u * DH:(u + 1) * DH]

        def proj_z(lhs, dests):
            for i in range(H // 2):
                r = _dot(lhs, wz_s[i])
                mid = r[:, 384:512]
                parts = [(r[:, 0:384].astype(BF16), mid.astype(BF16)),
                         (r[:, 512:896].astype(BF16), pltpu.roll(mid, 64, 1).astype(BF16))]
                for u in range(2):
                    g, jx = divmod(2 * i + u, 3)
                    for (a, n, d, b) in dests:
                        r0 = g * 128 + jx * L + b
                        d[r0:r0 + n, 0:384] = parts[u][0][a:a + n]
                        d[r0:r0 + n, 384:512] = parts[u][1][a:a + n]

        def seg(lhs, sel, w):
            def dests(refs):
                return [(a, n, refs[v], b) for (a, n, v, b) in sel]
            qs, ks, zs = (qs0, qs1), (ks0, ks1), (zs0, zs1)
            rows = [3 * L] * (NG - 1) + [L]
            proj_qk(lhs, 0, dests(qs))
            proj_qk(lhs, 1, dests(ks))
            scs = [_dot_nt(qs[w][g, 0:rows[g], :], ks[w][g]) for g in range(NG)]
            proj_z(lhs, dests(zs))
            ps = []
            for g in range(NG):
                sc = jnp.where(mask3[0:rows[g]], scs[g], NEG)
                m = jnp.max(sc, axis=1, keepdims=True)
                e = jnp.exp(sc - m)
                l = jnp.sum(e, axis=1, keepdims=True)
                p = e * _recip(l)
                if g < NG - 1:
                    p = p[0:L] + p[L:2 * L] + p[2 * L:3 * L]
                ps.append(p.astype(BF16))
            return _dot(jnp.concatenate(ps, axis=1), zs[w][...])[:, 0:DM].astype(BF16)

        def out_copy(base):
            return pltpu.make_async_copy(
                stage_s.at[pl.ds(base, 2 * SEG)], out_hbm.at[pl.ds(base, 2 * SEG)], osem)

        def pair(j, mem):
            base = pl.multiple_of(j * 2 * SEG, 2 * SEG)
            x0 = ax_s[pl.ds(base, SEG), :]
            x1 = ax_s[pl.ds(base + SEG, SEG), :]
            lhs1 = jnp.concatenate([x0, x1[0:8], mem], axis=0)
            out1 = seg(lhs1, [(0, 32, 0, 0), (32, 8, 1, 0), (40, 8, 0, 32)], 0)
            stage_s[pl.ds(base, SEG), 0:DM] = out1[0:SEG]
            lhs2 = jnp.concatenate([x1[16:32], out1[SEG:L], x1[8:16]], axis=0)
            out2 = seg(lhs2, [(0, 16, 1, 16), (16, 8, 1, 32), (24, 8, 1, 8)], 1)
            stage_s[pl.ds(base + SEG, SEG), 0:DM] = out2[0:SEG]
            out_copy(base).start()
            return out2[SEG:L]

        lax.fori_loop(0, N_PAIR_ITERS, pair, mem0_s[...])
        for j in range(N_PAIR_ITERS):
            out_copy(j * 2 * SEG).wait()

    pl.run_scoped(
        main,
        pltpu.VMEM((2, DM, HD), BF16), pltpu.VMEM((H, DM, DH), BF16),
        pltpu.VMEM((H, DH, 512), BF16),
        pltpu.VMEM((H // 2, DM, 2 * DM), BF16), pltpu.VMEM((S, DM), BF16),
        pltpu.VMEM((S, DH), BF16), pltpu.VMEM((S, DH), BF16),
        pltpu.VMEM((S, 2 * DM), BF16), pltpu.VMEM((2, DM, 128), F32),
        pltpu.VMEM((NG, 128, DH), BF16), pltpu.VMEM((NG, 128, DH), BF16),
        pltpu.VMEM((NG, 128, DH), BF16), pltpu.VMEM((NG, 128, DH), BF16),
        pltpu.VMEM((NG * 128, 512), BF16), pltpu.VMEM((NG * 128, 512), BF16),
    )


@functools.partial(jax.jit, static_argnames=("A_seg_len",))
def pallas_concat_heads__memory_aug_recurrent_mem_tr__compressed_kv_cla__prompt_kernel(
    A_x: jax.Array,
    A_mem0: jax.Array,
    A_Wq: jax.Array,
    A_Wk: jax.Array,
    A_Wv: jax.Array,
    A_Wo: jax.Array,
    A_seg_len: int,
    B_x: jax.Array,
    B_c_kv: jax.Array,
    B_w_q: jax.Array,
    B_w_uk: jax.Array,
    B_w_uv: jax.Array,
    B_w_o: jax.Array,
):
    assert A_seg_len == SEG
    assert A_x.shape == (1, S, DM) and A_mem0.shape == (1, MEM, DM)
    assert A_Wq.shape == (DM, H, DH) and A_Wo.shape == (H, DH, DM)
    assert B_x.shape == (1, S, DM) and B_c_kv.shape == (1, S, DC)
    assert B_w_q.shape == (DM, H, DH) and B_w_uk.shape == (DC, H, DH)
    assert B_w_o.shape == (H, DH, DM)

    axt = jnp.swapaxes(A_x, 1, 2).reshape(DM, S)
    bxt = jnp.swapaxes(B_x, 1, 2).reshape(DM, S)
    awot = jnp.swapaxes(A_Wo, 1, 2)
    bwot = jnp.swapaxes(B_w_o, 1, 2)

    any_spec = pl.BlockSpec(memory_space=pl.ANY)
    out = pl.pallas_call(
        _kernel,
        out_shape=jax.ShapeDtypeStruct((S, 2 * DM), BF16),
        in_specs=[any_spec] * 12,
        out_specs=any_spec,
        scratch_shapes=[
            pltpu.VMEM((H, DC, DH), BF16),
            pltpu.VMEM((H, DC, DH), BF16),
            pltpu.VMEM((S, DC), BF16),
            pltpu.VMEM((H, DM, DH), BF16),
            pltpu.VMEM((H, S, DH), BF16),
            pltpu.VMEM((3, DM + 1, H, DH), BF16),
            pltpu.VMEM((H + 1, DM, DH), BF16),
            pltpu.VMEM((S // 128 + 1, DM, 128), BF16),
            pltpu.VMEM((MEM, DM), BF16),
            pltpu.SemaphoreType.DMA((18,)),
            pltpu.SemaphoreType.DMA,
        ],
        compiler_params=pltpu.CompilerParams(vmem_limit_bytes=120 * 1024 * 1024),
    )(axt, A_mem0.reshape(MEM, DM), A_Wq, A_Wk, A_Wv, awot,
      bxt, B_c_kv.reshape(S, DC), B_w_q, B_w_uk, B_w_uv, bwot)
    return out.reshape(1, S, 2 * DM)
```

```python
import functools

import jax
import jax.numpy as jnp
from jax import lax
import jax.experimental.pallas as pl
import jax.experimental.pallas.tpu as pltpu

F32 = jnp.float32
BF16 = jnp.bfloat16
NT = (((1,), (1,)), ((), ()))
NEG = -1000000000.0

S = 2048
DM = 448
H = 16
DH = 256
HD = H * DH
DC = 1024
MEM = 8
SEG = 32
L = SEG + MEM
NPAIR = S // (2 * SEG)

BQ = 256
HB = BQ // 2
NQ = S // BQ
PB = 512
QB = 128
KB = 128
N_OPROJ_ITERS = S // 128
N_HEAD_ITERS = H
N_PAIR_ITERS = NPAIR


def _dot(a, b):
    return jnp.dot(a, b, preferred_element_type=F32)


def _dot_nt(a, b):
    return lax.dot_general(a, b, NT, preferred_element_type=F32)


def _recip(l):
    r = pl.reciprocal(l, approx=True)
    return r * (2.0 - l * r)


def _kernel(axt_hbm, mem0_hbm, awq_hbm, awk_hbm, awv_hbm, awot_hbm,
            bxt_hbm, ckv_hbm, bwq_hbm, bwk_hbm, bwv_hbm, bwot_hbm,
            out_hbm,
            wk_s, wv_s, ckv_s, bwot_s, q_s, rawa_s, awot_s, axt_s, mem0_s,
            sems, osem):
    scale = DH ** -0.5

    def cp(src, dst, i):
        return pltpu.make_async_copy(src, dst, sems.at[i])

    cp_ckv = cp(ckv_hbm, ckv_s, 6)
    cp_bwot = cp(bwot_hbm, bwot_s, 7)
    cp_awot = cp(awot_hbm, awot_s.at[pl.ds(0, H)], 8)
    cp_axt = [cp(axt_hbm.at[:, pl.ds(j * 128, 128)], axt_s.at[j], 9)
              for j in range(S // 128)]
    cp_aw = [cp(w, rawa_s.at[t, pl.ds(0, DM)], 10 + t)
             for t, w in enumerate((awq_hbm, awk_hbm, awv_hbm))]

    cp_mem0 = cp(mem0_hbm, mem0_s, 13)

    def prologue(bxt_s, bx_s, rawq_s, wq_s, rawk_s, rawv_s):
        cp_bxt = [cp(bxt_hbm.at[:, pl.ds(j * 128, 128)], bxt_s.at[j], 0 if j < 4 else 1)
                  for j in range(S // 128)]
        RQ = DM // 4
        cp_bwq_lo = [cp(bwq_hbm.at[pl.ds(c * RQ, RQ), pl.ds(0, 8), :],
                        rawq_s.at[0, pl.ds(c * RQ, RQ)], 14 + c) for c in range(4)]
        cp_bwq_hi = cp(bwq_hbm.at[:, pl.ds(8, 8), :], rawq_s.at[1], 3)
        cp_bwk = cp(bwk_hbm, rawk_s, 4)
        cp_bwv = cp(bwv_hbm, rawv_s, 5)
        for c in (cp_bxt[:4] + cp_bwq_lo + cp_bxt[4:]
                  + [cp_bwq_hi, cp_bwk, cp_bwv, cp_ckv, cp_bwot, cp_awot] + cp_axt
                  + cp_aw + [cp_mem0]):
            c.start()

        def relayout(src, dst, h0, r0, n):
            w = jnp.swapaxes(src[pl.ds(r0, n)], 0, 1)
            for h in range(w.shape[0]):
                dst[h0 + h, pl.ds(r0, n), :] = w[h]

        def xpose(j):
            r0 = j * 128 if isinstance(j, int) else pl.multiple_of(j * 128, 128)
            bx_s[pl.ds(r0, 128), :] = bxt_s[j].T

        def blk(h0, nh, r_lo, r_hi, side):
            def body(i, c):
                h = h0 + i
                for r in range(r_lo, r_hi):
                    rows = slice(r * QB, (r + 1) * QB)
                    q_s[h, rows, :] = (_dot(bx_s[rows, :], wq_s[h]) * scale).astype(BF16)
                    side(i, r - r_lo)
                return c
            lax.fori_loop(0, nh, body, 0)

        def side_xpose(i, r):
            if r < 3:
                xpose(4 + i * 3 + r)

        def side_wq(i, r):
            if r < 4:
                r0 = jnp.minimum(i, DM // 64 - 1) * 64 + r * 16
                relayout(rawq_s.at[1], wq_s, 8, pl.multiple_of(r0, 16), 16)

        def side_relayout(src, dst):
            def side(i, r):
                relayout(src, dst, 0, pl.multiple_of(i * 256 + r * 16, 16), 16)
            return side

        for c in cp_bxt[:4]:
            c.wait()
        for j in range(4):
            xpose(j)
        for c in range(4):
            cp_bwq_lo[c].wait()
            relayout(rawq_s.at[0], wq_s, 0, c * RQ, RQ)
        blk(0, 4, 0, 4, lambda i, r: None)
        for c in cp_bxt[4:]:
            c.wait()
        blk(4, 4, 0, 4, side_xpose)
        cp_bwq_hi.wait()
        blk(0, 8, 4, 16, side_wq)
        cp_bwk.wait()
        blk(8, 4, 0, 16, side_relayout(rawk_s, wk_s))
        cp_bwv.wait()
        blk(12, 4, 0, 16, side_relayout(rawv_s, wv_s))

    pl.run_scoped(
        prologue,
        pltpu.VMEM((S // 128, DM, 128), BF16), pltpu.VMEM((S, DM), BF16),
        pltpu.VMEM((2, DM, 8, DH), BF16), pltpu.VMEM((H, DM, DH), BF16),
        pltpu.VMEM((DC, H, DH), BF16), pltpu.VMEM((DC, H, DH), BF16),
    )

    def main(wqk_s, awv_s, awo_s, wz_s, wg_s, ax_s, k_s, v_s, stage_s, ot_s,
             ts0, ts1, zs0, zs1):
        cp_ckv.wait()

        tri = (lax.broadcasted_iota(jnp.int32, (HB, HB), 1)
               <= lax.broadcasted_iota(jnp.int32, (HB, HB), 0))
        tri2 = (lax.broadcasted_iota(jnp.int32, (BQ, HB), 1)
                <= lax.broadcasted_iota(jnp.int32, (BQ, HB), 0))

        def kvproj(w_ref, dst, h, pb, lo, hi):
            for r0 in range(lo, hi, pb):
                dst[r0:r0 + pb, :] = _dot(ckv_s[r0:r0 + pb, :], w_ref[h]).astype(BF16)

        def qk(h, i):
            d0 = i * BQ
            q = q_s[h, d0:d0 + BQ, :]
            so = _dot_nt(q, k_s[0:d0, :]) if i > 0 else None
            s1 = _dot_nt(q, k_s[d0:d0 + HB, :])
            s2 = _dot_nt(q[HB:], k_s[d0 + HB:d0 + BQ, :])
            return so, s1, s2

        def soft_pv_out(h, i, ss):
            so, s1, s2 = ss
            d0 = i * BQ
            s1 = jnp.where(tri2, s1, NEG)
            s2 = jnp.where(tri, s2, NEG)
            m = jnp.max(s1, axis=1, keepdims=True)
            if so is not None:
                m = jnp.maximum(m, jnp.max(so, axis=1, keepdims=True))
            mb = jnp.maximum(m[HB:], jnp.max(s2, axis=1, keepdims=True))
            m = jnp.concatenate([m[:HB], mb], axis=0)
            p1 = jnp.exp(s1 - m)
            p2 = jnp.exp(s2 - mb)
            l = jnp.sum(p1, axis=1, keepdims=True)
            acc = _dot(p1.astype(BF16), v_s[d0:d0 + HB, :])
            if so is not None:
                po = jnp.exp(so - m)
                l = l + jnp.sum(po, axis=1, keepdims=True)
                acc = acc + _dot(po.astype(BF16), v_s[0:d0, :])
            l2 = l[HB:] + jnp.sum(p2, axis=1, keepdims=True)
            acc2 = acc[HB:] + _dot(p2.astype(BF16), v_s[d0 + HB:d0 + BQ, :])
            ctx = jnp.concatenate(
                [acc[:HB] * _recip(l[:HB]), acc2 * _recip(l2)], axis=0).astype(BF16)
            q_s[h, d0:d0 + BQ, :] = ctx

        def head(h, c):
            kvproj(wk_s, k_s, h, KB, 0, S)
            order = list(range(NQ - 1, -1, -1))
            ss = qk(h, order[0])
            kvproj(wv_s, v_s, h, PB, 0, S)
            for n, i in enumerate(order):
                nxt = qk(h, order[n + 1]) if n + 1 < NQ else None
                soft_pv_out(h, i, ss)
                ss = nxt
            return c

        lax.fori_loop(0, N_HEAD_ITERS, head, 0)

        cp_bwot.wait()
        cp_awot.wait()
        for c in cp_axt + cp_aw + [cp_mem0]:
            c.wait()
        ot_s[0] = jnp.zeros((DM, 128), F32)

        def flush(r0):
            stage_s[pl.ds(r0, 128), DM:2 * DM] = ot_s[0].T.astype(BF16)

        def oproj(j, c):
            r0 = pl.multiple_of(j * 128, 128)
            w0 = jnp.minimum(j, DM // 32 - 1) * 32
            pin_w = jnp.maximum(j, DM)
            pin_h = jnp.maximum(j, H)
            pin_o = jnp.where(j >= 0, 1, 0)
            acc = None
            for h in range(H):
                r = _dot_nt(bwot_s[h], q_s[h, pl.ds(r0, 128), :])
                acc = r if acc is None else acc + r
                if h == 0:
                    ot_s[pin_o, 0:8, :] = r[0:8]
                    flush(pl.multiple_of(jnp.maximum(j - 1, 0) * 128, 128))
                elif h in (3, 6, 9, 12):
                    half, g = divmod(h // 3 - 1, 2)
                    rr = pl.multiple_of(w0 + half * 16, 16)
                    rawa_s[2, pin_w, :, 0:128] = r[0:16].astype(BF16)
                    w = jnp.swapaxes(rawa_s[2, pl.ds(rr, 16), g * 8:(g + 1) * 8, :], 0, 1)
                    for u in range(8):
                        awv_s[g * 8 + u, pl.ds(rr, 16), :] = w[u]
                elif h in (4, 8):
                    e0 = (h // 4 - 1) * 128
                    awot_s[pin_h, 0:16, 0:128] = r[0:16].astype(BF16)
                    tail = awot_s[j, 384:DM, e0:e0 + 128]
                    zero = jnp.zeros_like(tail)
                    odd = (j % 2) == 1
                    wt = jnp.concatenate(
                        [awot_s[j, 0:384, e0:e0 + 128], jnp.where(odd, zero, tail),
                         jnp.where(odd, tail, zero)], axis=0)
                    awo_s[j, e0:e0 + 128, :] = wt.T
                elif h == 14:
                    axt_s[pin_h, 0:16, :] = r[0:16].astype(BF16)
                    ax_s[pl.ds(r0, 128), :] = axt_s[j].T
            ot_s[0] = acc
            return c

        lax.fori_loop(0, N_OPROJ_ITERS, oproj, 0)
        flush(S - 128)

        RC = DM // 4

        def wzprep(i, c):
            for n in range(8):
                rc, u = divmod(n, 2)
                rows = slice(rc * RC, (rc + 1) * RC)
                w = _dot(awv_s[2 * i + u, rows, :], awo_s[2 * i + u])
                wz_s[i, rows, u * 512:u * 512 + 384] = w[:, 0:384].astype(BF16)
                if u == 0:
                    mid = w[:, 384:512]
                else:
                    wz_s[i, rows, 384:512] = (mid + w[:, 384:512]).astype(BF16)
                if n < 7:
                    piece = i * 7 + n
                    t = jnp.where(piece >= DM // 16, 1, 0)
                    rr = pl.multiple_of((piece - t * (DM // 16)) * 16, 16)
                    ro = pl.multiple_of(rr + jnp.where(piece >= DM // 16 + 24, 64, 0), 16)
                    wr = jnp.swapaxes(rawa_s[t, pl.ds(rr, 16)], 0, 1)
                    for h in range(H):
                        wqk_s[t, h, pl.ds(ro if h % 2 else rr, 16), :] = wr[h]
            return c

        for h in range(H):
            lo = 384 if h % 2 else DM
            wqk_s[1, h, lo:lo + 64, :] = jnp.zeros((64, DH), BF16)
        lax.fori_loop(0, H // 2, wzprep, 0)

        def gprep(i, c):
            for n in range(8):
                rc, u = divmod(n, 2)
                rows = slice(rc * RC, (rc + 1) * RC)
                w = _dot_nt(wqk_s[0, 2 * i + u, rows, :], wqk_s[1, 2 * i + u]) * scale
                wg_s[i, rows, u * 512:u * 512 + 384] = w[:, 0:384].astype(BF16)
                if u == 0:
                    mid = w[:, 384:512]
                else:
                    wg_s[i, rows, 384:512] = (mid + w[:, 384:512]).astype(BF16)
            return c

        lax.fori_loop(0, H // 2, gprep, 0)

        key = lax.broadcasted_iota(jnp.int32, (L, H * L), 0)
        qry = lax.broadcasted_iota(jnp.int32, (L, H * L), 1) % L
        mask = (qry >= SEG) | (key >= SEG) | (key <= qry)
        lane = lax.broadcasted_iota(jnp.int32, (8, 128), 1)
        lane_l = lax.broadcasted_iota(jnp.int32, (L, 128), 1)
        NT_ = H * L // 128
        tile_heads = [[h for h in range(H) if h * L < (t + 1) * 128 and (h + 1) * L > t * 128]
                      for t in range(NT_)]

        def proj(lhs, w_ref, dests):
            for i in range(H // 2):
                r = _dot(lhs, w_ref[i])
                mid = r[:, 384:512]
                parts = [(r[:, 0:384].astype(BF16), mid.astype(BF16)),
                         (r[:, 512:896].astype(BF16), pltpu.roll(mid, 64, 1).astype(BF16))]
                for u in range(2):
                    for (a, n, d, b) in dests:
                        r0 = (2 * i + u) * L + b
                        d[r0:r0 + n, 0:384] = parts[u][0][a:a + n]
                        d[r0:r0 + n, 384:512] = parts[u][1][a:a + n]

        def seg(lhs, keys, sel, w):
            def dests(refs):
                return [(a, n, refs[v], b) for (a, n, v, b) in sel]
            ts, zs = (ts0, ts1), (zs0, zs1)
            proj(lhs, wg_s, dests(ts))
            sc = _dot_nt(keys, ts[w][:, 0:DM])
            proj(lhs, wz_s, dests(zs))
            sc = jnp.where(mask, sc, NEG)
            e = jnp.exp(sc - jnp.max(sc, axis=0, keepdims=True))
            p = e * _recip(jnp.sum(e, axis=0, keepdims=True))
            rs = []
            for t in range(NT_):
                pt = p[:, t * 128:(t + 1) * 128]
                grp = [None] * 16
                for h in tile_heads[t]:
                    for kk in range(L // 8):
                        g = (h * (L // 8) + kk) % 16
                        piece = pt[kk * 8:(kk + 1) * 8]
                        grp[g] = piece if grp[g] is None else jnp.where(
                            lane >= h * L - t * 128, piece, grp[g])
                rs.append(jnp.concatenate(grp, axis=0).T)
            rr = jnp.concatenate(rs, axis=0)
            pcs = []
            for t in range(NT_):
                pc = None
                for h in tile_heads[t]:
                    piece = rr[h * L:(h + 1) * L]
                    pc = piece if pc is None else jnp.where(
                        lane_l >= h * L - t * 128, piece, pc)
                pcs.append(pc.astype(BF16))
            return _dot(jnp.concatenate(pcs, axis=1), zs[w][...])[:, 0:DM].astype(BF16)

        def out_copy(base):
            return pltpu.make_async_copy(
                stage_s.at[pl.ds(base, 2 * SEG)], out_hbm.at[pl.ds(base, 2 * SEG)], osem)

        def pair(j, mem):
            base = pl.multiple_of(j * 2 * SEG, 2 * SEG)
            x0 = ax_s[pl.ds(base, SEG), :]
            x1 = ax_s[pl.ds(base + SEG, SEG), :]
            lhs1 = jnp.concatenate([x0, x1[0:8], mem], axis=0)
            out1 = seg(lhs1, jnp.concatenate([x0, mem], axis=0),
                       [(0, 32, 0, 0), (32, 8, 1, 0), (40, 8, 0, 32)], 0)
            stage_s[pl.ds(base, SEG), 0:DM] = out1[0:SEG]
            lhs2 = jnp.concatenate([x1[16:32], out1[SEG:L], x1[8:16]], axis=0)
            out2 = seg(lhs2, jnp.concatenate([x1, out1[SEG:L]], axis=0),
                       [(0, 16, 1, 16), (16, 8, 1, 32), (24, 8, 1, 8)], 1)
            stage_s[pl.ds(base + SEG, SEG), 0:DM] = out2[0:SEG]
            out_copy(base).start()
            return out2[SEG:L]

        lax.fori_loop(0, N_PAIR_ITERS, pair, mem0_s[...])
        for j in range(N_PAIR_ITERS):
            out_copy(j * 2 * SEG).wait()

    pl.run_scoped(
        main,
        pltpu.VMEM((2, H, 512, DH), BF16), pltpu.VMEM((H, DM, DH), BF16),
        pltpu.VMEM((H, DH, 512), BF16),
        pltpu.VMEM((H // 2, DM, 2 * DM), BF16), pltpu.VMEM((H // 2, DM, 2 * DM), BF16),
        pltpu.VMEM((S, DM), BF16),
        pltpu.VMEM((S, DH), BF16), pltpu.VMEM((S, DH), BF16),
        pltpu.VMEM((S, 2 * DM), BF16), pltpu.VMEM((2, DM, 128), F32),
        pltpu.VMEM((H * L, 512), BF16), pltpu.VMEM((H * L, 512), BF16),
        pltpu.VMEM((H * L, 512), BF16), pltpu.VMEM((H * L, 512), BF16),
    )


@functools.partial(jax.jit, static_argnames=("A_seg_len",))
def pallas_concat_heads__memory_aug_recurrent_mem_tr__compressed_kv_cla__prompt_kernel(
    A_x: jax.Array,
    A_mem0: jax.Array,
    A_Wq: jax.Array,
    A_Wk: jax.Array,
    A_Wv: jax.Array,
    A_Wo: jax.Array,
    A_seg_len: int,
    B_x: jax.Array,
    B_c_kv: jax.Array,
    B_w_q: jax.Array,
    B_w_uk: jax.Array,
    B_w_uv: jax.Array,
    B_w_o: jax.Array,
):
    assert A_seg_len == SEG
    assert A_x.shape == (1, S, DM) and A_mem0.shape == (1, MEM, DM)
    assert A_Wq.shape == (DM, H, DH) and A_Wo.shape == (H, DH, DM)
    assert B_x.shape == (1, S, DM) and B_c_kv.shape == (1, S, DC)
    assert B_w_q.shape == (DM, H, DH) and B_w_uk.shape == (DC, H, DH)
    assert B_w_o.shape == (H, DH, DM)

    axt = jnp.swapaxes(A_x, 1, 2).reshape(DM, S)
    bxt = jnp.swapaxes(B_x, 1, 2).reshape(DM, S)
    awot = jnp.swapaxes(A_Wo, 1, 2)
    bwot = jnp.swapaxes(B_w_o, 1, 2)

    any_spec = pl.BlockSpec(memory_space=pl.ANY)
    out = pl.pallas_call(
        _kernel,
        out_shape=jax.ShapeDtypeStruct((S, 2 * DM), BF16),
        in_specs=[any_spec] * 12,
        out_specs=any_spec,
        scratch_shapes=[
            pltpu.VMEM((H, DC, DH), BF16),
            pltpu.VMEM((H, DC, DH), BF16),
            pltpu.VMEM((S, DC), BF16),
            pltpu.VMEM((H, DM, DH), BF16),
            pltpu.VMEM((H, S, DH), BF16),
            pltpu.VMEM((3, DM + 1, H, DH), BF16),
            pltpu.VMEM((H + 1, DM, DH), BF16),
            pltpu.VMEM((S // 128 + 1, DM, 128), BF16),
            pltpu.VMEM((MEM, DM), BF16),
            pltpu.SemaphoreType.DMA((18,)),
            pltpu.SemaphoreType.DMA,
        ],
        compiler_params=pltpu.CompilerParams(vmem_limit_bytes=120 * 1024 * 1024),
    )(axt, A_mem0.reshape(MEM, DM), A_Wq, A_Wk, A_Wv, awot,
      bxt, B_c_kv.reshape(S, DC), B_w_q, B_w_uk, B_w_uv, bwot)
    return out.reshape(1, S, 2 * DM)
```

```python
import functools

import jax
import jax.numpy as jnp
from jax import lax
import jax.experimental.pallas as pl
import jax.experimental.pallas.tpu as pltpu

F32 = jnp.float32
BF16 = jnp.bfloat16
NT = (((1,), (1,)), ((), ()))
NEG = -1000000000.0

S = 2048
DM = 448
H = 16
DH = 256
HD = H * DH
DC = 1024
MEM = 8
SEG = 32
L = SEG + MEM
NPAIR = S // (2 * SEG)

BQ = 256
HB = BQ // 2
NQ = S // BQ
PB = 512
QB = 128
KB = 128
N_OPROJ_ITERS = S // 128
N_HEAD_ITERS = H
N_PAIR_ITERS = NPAIR
TAILPOS = 4
GRC = 2
GTAIL = 2


def _dot(a, b):
    return jnp.dot(a, b, preferred_element_type=F32)


def _dot_nt(a, b):
    return lax.dot_general(a, b, NT, preferred_element_type=F32)


def _recip(l):
    r = pl.reciprocal(l, approx=True)
    return r * (2.0 - l * r)


def _kernel(axt_hbm, mem0_hbm, awq_hbm, awk_hbm, awv_hbm, awot_hbm,
            bxt_hbm, ckv_hbm, bwq_hbm, bwk_hbm, bwv_hbm, bwot_hbm,
            out_hbm,
            wk_s, wv_s, ckv_s, bwot_s, q_s, rawa_s, awot_s, axt_s, mem0_s,
            sems, osem):
    scale = DH ** -0.5

    def cp(src, dst, i):
        return pltpu.make_async_copy(src, dst, sems.at[i])

    cp_ckv = cp(ckv_hbm, ckv_s, 6)
    cp_bwot = cp(bwot_hbm, bwot_s, 7)
    cp_awot = cp(awot_hbm, awot_s, 8)
    cp_axt = [cp(axt_hbm.at[:, pl.ds(j * 128, 128)], axt_s.at[j], 9)
              for j in range(S // 128)]
    cp_aw = [cp(w, rawa_s.at[t, pl.ds(0, DM)], 10 + t)
             for t, w in enumerate((awq_hbm, awk_hbm, awv_hbm))]

    cp_mem0 = cp(mem0_hbm, mem0_s, 13)

    def prologue(bxt_s, bx_s, rawq_s, wq_s, rawk_s, rawv_s):
        cp_bxt = [cp(bxt_hbm.at[:, pl.ds(j * 128, 128)], bxt_s.at[j], 0 if j < 4 else 1)
                  for j in range(S // 128)]
        RQ = DM // 4
        cp_bwq_lo = [cp(bwq_hbm.at[pl.ds(c * RQ, RQ), pl.ds(0, 8), :],
                        rawq_s.at[0, pl.ds(c * RQ, RQ)], 14 + c) for c in range(4)]
        cp_bwq_hi = cp(bwq_hbm.at[:, pl.ds(8, 8), :], rawq_s.at[1], 3)
        cp_bwk = cp(bwk_hbm, rawk_s, 4)
        cp_bwv = cp(bwv_hbm, rawv_s, 5)
        for c in (cp_bxt[:4] + cp_bwq_lo + cp_bxt[4:]
                  + [cp_bwq_hi, cp_bwk, cp_bwv, cp_ckv, cp_bwot, cp_awot] + cp_axt
                  + cp_aw + [cp_mem0]):
            c.start()

        def relayout(src, dst, h0, r0, n):
            w = jnp.swapaxes(src[pl.ds(r0, n)], 0, 1)
            for h in range(w.shape[0]):
                dst[h0 + h, pl.ds(r0, n), :] = w[h]

        def xpose(j):
            r0 = j * 128 if isinstance(j, int) else pl.multiple_of(j * 128, 128)
            bx_s[pl.ds(r0, 128), :] = bxt_s[j].T

        def blk(h0, nh, r_lo, r_hi, side):
            def body(i, c):
                h = h0 + i
                for r in range(r_lo, r_hi):
                    rows = slice(r * QB, (r + 1) * QB)
                    q_s[h, rows, :] = (_dot(bx_s[rows, :], wq_s[h]) * scale).astype(BF16)
                    side(i, r - r_lo)
                return c
            lax.fori_loop(0, nh, body, 0)

        def side_xpose(i, r):
            if r < 3:
                xpose(4 + i * 3 + r)

        def side_wq(i, r):
            if r < 4:
                r0 = jnp.minimum(i, DM // 64 - 1) * 64 + r * 16
                relayout(rawq_s.at[1], wq_s, 8, pl.multiple_of(r0, 16), 16)

        def side_relayout(src, dst):
            def side(i, r):
                relayout(src, dst, 0, pl.multiple_of(i * 256 + r * 16, 16), 16)
            return side

        for c in cp_bxt[:4]:
            c.wait()
        for j in range(4):
            xpose(j)
        for c in range(4):
            cp_bwq_lo[c].wait()
            relayout(rawq_s.at[0], wq_s, 0, c * RQ, RQ)
        blk(0, 4, 0, 4, lambda i, r: None)
        for c in cp_bxt[4:]:
            c.wait()
        blk(4, 4, 0, 4, side_xpose)
        cp_bwq_hi.wait()
        blk(0, 8, 4, 16, side_wq)
        cp_bwk.wait()
        blk(8, 4, 0, 16, side_relayout(rawk_s, wk_s))
        cp_bwv.wait()
        blk(12, 4, 0, 16, side_relayout(rawv_s, wv_s))

    pl.run_scoped(
        prologue,
        pltpu.VMEM((S // 128, DM, 128), BF16), pltpu.VMEM((S, DM), BF16),
        pltpu.VMEM((2, DM, 8, DH), BF16), pltpu.VMEM((H, DM, DH), BF16),
        pltpu.VMEM((DC, H, DH), BF16), pltpu.VMEM((DC, H, DH), BF16),
    )

    def main(wqk_s, awv_s, wz_s, wg_s, ax_s, k_s, v_s, stage_s, ot_s,
             ts0, ts1, zs0, zs1):
        cp_ckv.wait()

        tri = (lax.broadcasted_iota(jnp.int32, (HB, HB), 1)
               <= lax.broadcasted_iota(jnp.int32, (HB, HB), 0))
        tri2 = (lax.broadcasted_iota(jnp.int32, (BQ, HB), 1)
                <= lax.broadcasted_iota(jnp.int32, (BQ, HB), 0))

        def kvproj(w_ref, dst, h, pb, lo, hi):
            for r0 in range(lo, hi, pb):
                dst[r0:r0 + pb, :] = _dot(ckv_s[r0:r0 + pb, :], w_ref[h]).astype(BF16)

        def qk(h, i):
            d0 = i * BQ
            q = q_s[h, d0:d0 + BQ, :]
            so = _dot_nt(q, k_s[0:d0, :]) if i > 0 else None
            s1 = _dot_nt(q, k_s[d0:d0 + HB, :])
            s2 = _dot_nt(q[HB:], k_s[d0 + HB:d0 + BQ, :])
            return so, s1, s2

        def soft_pv_out(h, i, ss):
            so, s1, s2 = ss
            d0 = i * BQ
            s1 = jnp.where(tri2, s1, NEG)
            s2 = jnp.where(tri, s2, NEG)
            m = jnp.max(s1, axis=1, keepdims=True)
            if so is not None:
                m = jnp.maximum(m, jnp.max(so, axis=1, keepdims=True))
            mb = jnp.maximum(m[HB:], jnp.max(s2, axis=1, keepdims=True))
            m = jnp.concatenate([m[:HB], mb], axis=0)
            p1 = jnp.exp(s1 - m)
            p2 = jnp.exp(s2 - mb)
            l = jnp.sum(p1, axis=1, keepdims=True)
            acc = _dot(p1.astype(BF16), v_s[d0:d0 + HB, :])
            if so is not None:
                po = jnp.exp(so - m)
                l = l + jnp.sum(po, axis=1, keepdims=True)
                acc = acc + _dot(po.astype(BF16), v_s[0:d0, :])
            l2 = l[HB:] + jnp.sum(p2, axis=1, keepdims=True)
            acc2 = acc[HB:] + _dot(p2.astype(BF16), v_s[d0 + HB:d0 + BQ, :])
            ctx = jnp.concatenate(
                [acc[:HB] * _recip(l[:HB]), acc2 * _recip(l2)], axis=0).astype(BF16)
            q_s[h, d0:d0 + BQ, :] = ctx

        def head(h, c):
            kvproj(wk_s, k_s, h, KB, 0, S)
            order = list(range(NQ - 1, -1, -1))
            ss = qk(h, order[0])
            kvproj(wv_s, v_s, h, PB, 0, S)
            for n, i in enumerate(order):
                nxt = qk(h, order[n + 1]) if n + 1 < NQ else None
                soft_pv_out(h, i, ss)
                ss = nxt
            return c

        lax.fori_loop(0, N_HEAD_ITERS, head, 0)

        cp_bwot.wait()
        cp_awot.wait()
        for c in cp_axt + cp_aw + [cp_mem0]:
            c.wait()
        ot_s[0] = jnp.zeros((DM, 128), F32)

        def flush(r0):
            stage_s[pl.ds(r0, 128), DM:2 * DM] = ot_s[0].T.astype(BF16)

        def oproj(j, c):
            r0 = pl.multiple_of(j * 128, 128)
            w0 = jnp.minimum(j, DM // 32 - 1) * 32
            pin_w = jnp.maximum(j, DM)
            pin_h = jnp.maximum(j, H)
            pin_o = jnp.where(j >= 0, 1, 0)
            acc = None
            for h in range(H):
                r = _dot_nt(bwot_s[h], q_s[h, pl.ds(r0, 128), :])
                acc = r if acc is None else acc + r
                if h == 0:
                    ot_s[pin_o, 0:8, :] = r[0:8]
                    flush(pl.multiple_of(jnp.maximum(j - 1, 0) * 128, 128))
                elif h in (3, 6, 9, 12):
                    half, g = divmod(h // 3 - 1, 2)
                    rr = pl.multiple_of(w0 + half * 16, 16)
                    rawa_s[2, pin_w, :, 0:128] = r[0:16].astype(BF16)
                    w = jnp.swapaxes(rawa_s[2, pl.ds(rr, 16), g * 8:(g + 1) * 8, :], 0, 1)
                    for u in range(8):
                        awv_s[g * 8 + u, pl.ds(rr, 16), :] = w[u]
                elif h == 14:
                    axt_s[pin_h, 0:16, :] = r[0:16].astype(BF16)
                    ax_s[pl.ds(r0, 128), :] = axt_s[j].T
            ot_s[0] = acc
            return c

        lax.fori_loop(0, N_OPROJ_ITERS, oproj, 0)
        flush(S - 128)

        RC = DM // 4

        def tails(i, a_of, b_of, dst, mul):
            t = [_dot_nt(b_of(2 * i + u)[384:DM, :], a_of(2 * i + u)[...]) for u in range(2)]
            dst[i, :, 384:512] = (jnp.concatenate(t, axis=0) * mul).astype(BF16).T

        def wzprep(i, c):
            for n in range(8):
                if n == TAILPOS:
                    tails(i, lambda h: awv_s.at[h], lambda h: awot_s.at[h], wz_s, 1.0)
                rc, u = divmod(n, 2)
                rows = slice(rc * RC, (rc + 1) * RC)
                w = _dot_nt(awv_s[2 * i + u, rows, :], awot_s[2 * i + u, 0:384, :])
                wz_s[i, rows, u * 512:u * 512 + 384] = w.astype(BF16)
                if n < 7:
                    piece = i * 7 + n
                    t = jnp.where(piece >= DM // 16, 1, 0)
                    rr = pl.multiple_of((piece - t * (DM // 16)) * 16, 16)
                    wr = jnp.swapaxes(rawa_s[t, pl.ds(rr, 16)], 0, 1)
                    for h in range(H):
                        wqk_s[t, h, pl.ds(rr, 16), :] = wr[h]
            return c

        lax.fori_loop(0, H // 2, wzprep, 0)

        def gprep(i, c):
            for n in range(2 * GRC):
                if n == GTAIL:
                    tails(i, lambda h: wqk_s.at[0, h], lambda h: wqk_s.at[1, h], wg_s, scale)
                rc, u = divmod(n, 2)
                rows = slice(rc * (DM // GRC), (rc + 1) * (DM // GRC))
                w = _dot_nt(wqk_s[0, 2 * i + u, rows, :], wqk_s[1, 2 * i + u, 0:384, :])
                wg_s[i, rows, u * 512:u * 512 + 384] = (w * scale).astype(BF16)
            return c

        lax.fori_loop(0, H // 2, gprep, 0)

        key = lax.broadcasted_iota(jnp.int32, (L, H * L), 0)
        qry = lax.broadcasted_iota(jnp.int32, (L, H * L), 1) % L
        mask = (qry >= SEG) | (key >= SEG) | (key <= qry)
        lane = lax.broadcasted_iota(jnp.int32, (8, 128), 1)
        lane_l = lax.broadcasted_iota(jnp.int32, (L, 128), 1)
        NT_ = H * L // 128
        tile_heads = [[h for h in range(H) if h * L < (t + 1) * 128 and (h + 1) * L > t * 128]
                      for t in range(NT_)]

        def proj(lhs, w_ref, dests):
            for i in range(H // 2):
                r = _dot(lhs, w_ref[i])
                mid = r[:, 384:512]
                parts = [(r[:, 0:384].astype(BF16), mid.astype(BF16)),
                         (r[:, 512:896].astype(BF16), pltpu.roll(mid, 64, 1).astype(BF16))]
                for u in range(2):
                    for (a, n, d, b) in dests:
                        r0 = (2 * i + u) * L + b
                        d[r0:r0 + n, 0:384] = parts[u][0][a:a + n]
                        d[r0:r0 + n, 384:512] = parts[u][1][a:a + n]

        def seg(lhs, keys, sel, w):
            def dests(refs):
                return [(a, n, refs[v], b) for (a, n, v, b) in sel]
            ts, zs = (ts0, ts1), (zs0, zs1)
            proj(lhs, wg_s, dests(ts))
            sc = _dot_nt(keys, ts[w][:, 0:DM])
            proj(lhs, wz_s, dests(zs))
            sc = jnp.where(mask, sc, NEG)
            e = jnp.exp(sc - jnp.max(sc, axis=0, keepdims=True))
            p = e * _recip(jnp.sum(e, axis=0, keepdims=True))
            rs = []
            for t in range(NT_):
                pt = p[:, t * 128:(t + 1) * 128]
                grp = [None] * 16
                for h in tile_heads[t]:
                    for kk in range(L // 8):
                        g = (h * (L // 8) + kk) % 16
                        piece = pt[kk * 8:(kk + 1) * 8]
                        grp[g] = piece if grp[g] is None else jnp.where(
                            lane >= h * L - t * 128, piece, grp[g])
                rs.append(jnp.concatenate(grp, axis=0).T)
            rr = jnp.concatenate(rs, axis=0)
            pcs = []
            for t in range(NT_):
                pc = None
                for h in tile_heads[t]:
                    piece = rr[h * L:(h + 1) * L]
                    pc = piece if pc is None else jnp.where(
                        lane_l >= h * L - t * 128, piece, pc)
                pcs.append(pc.astype(BF16))
            return _dot(jnp.concatenate(pcs, axis=1), zs[w][...])[:, 0:DM].astype(BF16)

        def out_copy(base):
            return pltpu.make_async_copy(
                stage_s.at[pl.ds(base, 2 * SEG)], out_hbm.at[pl.ds(base, 2 * SEG)], osem)

        def pair(j, mem):
            base = pl.multiple_of(j * 2 * SEG, 2 * SEG)
            x0 = ax_s[pl.ds(base, SEG), :]
            x1 = ax_s[pl.ds(base + SEG, SEG), :]
            lhs1 = jnp.concatenate([x0, x1[0:8], mem], axis=0)
            out1 = seg(lhs1, jnp.concatenate([x0, mem], axis=0),
                       [(0, 32, 0, 0), (32, 8, 1, 0), (40, 8, 0, 32)], 0)
            stage_s[pl.ds(base, SEG), 0:DM] = out1[0:SEG]
            lhs2 = jnp.concatenate([x1[16:32], out1[SEG:L], x1[8:16]], axis=0)
            out2 = seg(lhs2, jnp.concatenate([x1, out1[SEG:L]], axis=0),
                       [(0, 16, 1, 16), (16, 8, 1, 32), (24, 8, 1, 8)], 1)
            stage_s[pl.ds(base + SEG, SEG), 0:DM] = out2[0:SEG]
            out_copy(base).start()
            return out2[SEG:L]

        lax.fori_loop(0, N_PAIR_ITERS, pair, mem0_s[...])
        for j in range(N_PAIR_ITERS):
            out_copy(j * 2 * SEG).wait()

    pl.run_scoped(
        main,
        pltpu.VMEM((2, H, DM, DH), BF16), pltpu.VMEM((H, DM, DH), BF16),
        pltpu.VMEM((H // 2, DM, 2 * DM), BF16), pltpu.VMEM((H // 2, DM, 2 * DM), BF16),
        pltpu.VMEM((S, DM), BF16),
        pltpu.VMEM((S, DH), BF16), pltpu.VMEM((S, DH), BF16),
        pltpu.VMEM((S, 2 * DM), BF16), pltpu.VMEM((2, DM, 128), F32),
        pltpu.VMEM((H * L, 512), BF16), pltpu.VMEM((H * L, 512), BF16),
        pltpu.VMEM((H * L, 512), BF16), pltpu.VMEM((H * L, 512), BF16),
    )


@functools.partial(jax.jit, static_argnames=("A_seg_len",))
def pallas_concat_heads__memory_aug_recurrent_mem_tr__compressed_kv_cla__prompt_kernel(
    A_x: jax.Array,
    A_mem0: jax.Array,
    A_Wq: jax.Array,
    A_Wk: jax.Array,
    A_Wv: jax.Array,
    A_Wo: jax.Array,
    A_seg_len: int,
    B_x: jax.Array,
    B_c_kv: jax.Array,
    B_w_q: jax.Array,
    B_w_uk: jax.Array,
    B_w_uv: jax.Array,
    B_w_o: jax.Array,
):
    assert A_seg_len == SEG
    assert A_x.shape == (1, S, DM) and A_mem0.shape == (1, MEM, DM)
    assert A_Wq.shape == (DM, H, DH) and A_Wo.shape == (H, DH, DM)
    assert B_x.shape == (1, S, DM) and B_c_kv.shape == (1, S, DC)
    assert B_w_q.shape == (DM, H, DH) and B_w_uk.shape == (DC, H, DH)
    assert B_w_o.shape == (H, DH, DM)

    axt = jnp.swapaxes(A_x, 1, 2).reshape(DM, S)
    bxt = jnp.swapaxes(B_x, 1, 2).reshape(DM, S)
    awot = jnp.swapaxes(A_Wo, 1, 2)
    bwot = jnp.swapaxes(B_w_o, 1, 2)

    any_spec = pl.BlockSpec(memory_space=pl.ANY)
    out = pl.pallas_call(
        _kernel,
        out_shape=jax.ShapeDtypeStruct((S, 2 * DM), BF16),
        in_specs=[any_spec] * 12,
        out_specs=any_spec,
        scratch_shapes=[
            pltpu.VMEM((H, DC, DH), BF16),
            pltpu.VMEM((H, DC, DH), BF16),
            pltpu.VMEM((S, DC), BF16),
            pltpu.VMEM((H, DM, DH), BF16),
            pltpu.VMEM((H, S, DH), BF16),
            pltpu.VMEM((3, DM + 1, H, DH), BF16),
            pltpu.VMEM((H, DM, DH), BF16),
            pltpu.VMEM((S // 128 + 1, DM, 128), BF16),
            pltpu.VMEM((MEM, DM), BF16),
            pltpu.SemaphoreType.DMA((18,)),
            pltpu.SemaphoreType.DMA,
        ],
        compiler_params=pltpu.CompilerParams(vmem_limit_bytes=120 * 1024 * 1024),
    )(axt, A_mem0.reshape(MEM, DM), A_Wq, A_Wk, A_Wv, awot,
      bxt, B_c_kv.reshape(S, DC), B_w_q, B_w_uk, B_w_uv, bwot)
    return out.reshape(1, S, 2 * DM)
```

```python
import functools

import jax
import jax.numpy as jnp
from jax import lax
import jax.experimental.pallas as pl
import jax.experimental.pallas.tpu as pltpu

F32 = jnp.float32
BF16 = jnp.bfloat16
NT = (((1,), (1,)), ((), ()))
NEG = -1000000000.0

S = 2048
DM = 448
H = 16
DH = 256
HD = H * DH
DC = 1024
MEM = 8
SEG = 32
L = SEG + MEM
NPAIR = S // (2 * SEG)

BQ = 256
HB = BQ // 2
NQ = S // BQ
PB = 512
QB = 128
KB = 128
N_OPROJ_ITERS = S // 128
N_HEAD_ITERS = H
N_PAIR_ITERS = NPAIR
TAILPOS = 4
GRC = 2
GTAIL = 2
GTAIL2 = 1
ORDER = 'U T01 st T234567 x1 sc Z01 sm Z23 x2 Z4567'


def _dot(a, b):
    return jnp.dot(a, b, preferred_element_type=F32)


def _dot_nt(a, b):
    return lax.dot_general(a, b, NT, preferred_element_type=F32)


def _recip(l):
    r = pl.reciprocal(l, approx=True)
    return r * (2.0 - l * r)


def _kernel(axt_hbm, mem0_hbm, awq_hbm, awk_hbm, awv_hbm, awot_hbm,
            bxt_hbm, ckv_hbm, bwq_hbm, bwk_hbm, bwv_hbm, bwot_hbm,
            out_hbm,
            wk_s, wv_s, ckv_s, bwot_s, q_s, rawa_s, awot_s, axt_s, mem0_s,
            sems, osem):
    scale = DH ** -0.5

    def cp(src, dst, i):
        return pltpu.make_async_copy(src, dst, sems.at[i])

    cp_ckv = cp(ckv_hbm, ckv_s, 6)
    cp_bwot = cp(bwot_hbm, bwot_s, 7)
    cp_awot = cp(awot_hbm, awot_s, 8)
    cp_axt = [cp(axt_hbm.at[:, pl.ds(j * 128, 128)], axt_s.at[j], 9)
              for j in range(S // 128)]
    cp_aw = [cp(w, rawa_s.at[t, pl.ds(0, DM)], 10 + t)
             for t, w in enumerate((awq_hbm, awk_hbm, awv_hbm))]

    cp_mem0 = cp(mem0_hbm, mem0_s, 13)

    def prologue(bxt_s, bx_s, rawq_s, wq_s, rawk_s, rawv_s):
        cp_bxt = [cp(bxt_hbm.at[:, pl.ds(j * 128, 128)], bxt_s.at[j], 0 if j < 4 else 1)
                  for j in range(S // 128)]
        RQ = DM // 4
        cp_bwq_lo = [cp(bwq_hbm.at[pl.ds(c * RQ, RQ), pl.ds(0, 8), :],
                        rawq_s.at[0, pl.ds(c * RQ, RQ)], 14 + c) for c in range(4)]
        cp_bwq_hi = cp(bwq_hbm.at[:, pl.ds(8, 8), :], rawq_s.at[1], 3)
        cp_bwk = cp(bwk_hbm, rawk_s, 4)
        cp_bwv = cp(bwv_hbm, rawv_s, 5)
        for c in (cp_bxt[:4] + cp_bwq_lo + cp_bxt[4:]
                  + [cp_bwq_hi, cp_bwk, cp_bwv, cp_ckv, cp_bwot, cp_awot] + cp_axt
                  + cp_aw + [cp_mem0]):
            c.start()

        def relayout(src, dst, h0, r0, n):
            w = jnp.swapaxes(src[pl.ds(r0, n)], 0, 1)
            for h in range(w.shape[0]):
                dst[h0 + h, pl.ds(r0, n), :] = w[h]

        def xpose(j):
            r0 = j * 128 if isinstance(j, int) else pl.multiple_of(j * 128, 128)
            bx_s[pl.ds(r0, 128), :] = bxt_s[j].T

        def blk(h0, nh, r_lo, r_hi, side):
            def body(i, c):
                h = h0 + i
                for r in range(r_lo, r_hi):
                    rows = slice(r * QB, (r + 1) * QB)
                    q_s[h, rows, :] = (_dot(bx_s[rows, :], wq_s[h]) * scale).astype(BF16)
                    side(i, r - r_lo)
                return c
            lax.fori_loop(0, nh, body, 0)

        def side_xpose(i, r):
            if r < 3:
                xpose(4 + i * 3 + r)

        def side_wq(i, r):
            if r < 4:
                r0 = jnp.minimum(i, DM // 64 - 1) * 64 + r * 16
                relayout(rawq_s.at[1], wq_s, 8, pl.multiple_of(r0, 16), 16)

        def side_relayout(src, dst):
            def side(i, r):
                relayout(src, dst, 0, pl.multiple_of(i * 256 + r * 16, 16), 16)
            return side

        for c in cp_bxt[:4]:
            c.wait()
        for j in range(4):
            xpose(j)
        for c in range(4):
            cp_bwq_lo[c].wait()
            relayout(rawq_s.at[0], wq_s, 0, c * RQ, RQ)
        blk(0, 4, 0, 4, lambda i, r: None)
        for c in cp_bxt[4:]:
            c.wait()
        blk(4, 4, 0, 4, side_xpose)
        cp_bwq_hi.wait()
        blk(0, 8, 4, 16, side_wq)
        cp_bwk.wait()
        blk(8, 4, 0, 16, side_relayout(rawk_s, wk_s))
        cp_bwv.wait()
        blk(12, 4, 0, 16, side_relayout(rawv_s, wv_s))

    pl.run_scoped(
        prologue,
        pltpu.VMEM((S // 128, DM, 128), BF16), pltpu.VMEM((S, DM), BF16),
        pltpu.VMEM((2, DM, 8, DH), BF16), pltpu.VMEM((H, DM, DH), BF16),
        pltpu.VMEM((DC, H, DH), BF16), pltpu.VMEM((DC, H, DH), BF16),
    )

    def main(wqk_s, awv_s, wz_s, wg_s, wu_s, ax_s, k_s, v_s, stage_s, ot_s,
             ts0, ts1, zs0, zs1, us0, us1):
        cp_ckv.wait()

        tri = (lax.broadcasted_iota(jnp.int32, (HB, HB), 1)
               <= lax.broadcasted_iota(jnp.int32, (HB, HB), 0))
        tri2 = (lax.broadcasted_iota(jnp.int32, (BQ, HB), 1)
                <= lax.broadcasted_iota(jnp.int32, (BQ, HB), 0))

        def kvproj(w_ref, dst, h, pb, lo, hi):
            for r0 in range(lo, hi, pb):
                dst[r0:r0 + pb, :] = _dot(ckv_s[r0:r0 + pb, :], w_ref[h]).astype(BF16)

        def qk(h, i):
            d0 = i * BQ
            q = q_s[h, d0:d0 + BQ, :]
            so = _dot_nt(q, k_s[0:d0, :]) if i > 0 else None
            s1 = _dot_nt(q, k_s[d0:d0 + HB, :])
            s2 = _dot_nt(q[HB:], k_s[d0 + HB:d0 + BQ, :])
            return so, s1, s2

        def soft_pv_out(h, i, ss):
            so, s1, s2 = ss
            d0 = i * BQ
            s1 = jnp.where(tri2, s1, NEG)
            s2 = jnp.where(tri, s2, NEG)
            m = jnp.max(s1, axis=1, keepdims=True)
            if so is not None:
                m = jnp.maximum(m, jnp.max(so, axis=1, keepdims=True))
            mb = jnp.maximum(m[HB:], jnp.max(s2, axis=1, keepdims=True))
            m = jnp.concatenate([m[:HB], mb], axis=0)
            p1 = jnp.exp(s1 - m)
            p2 = jnp.exp(s2 - mb)
            l = jnp.sum(p1, axis=1, keepdims=True)
            acc = _dot(p1.astype(BF16), v_s[d0:d0 + HB, :])
            if so is not None:
                po = jnp.exp(so - m)
                l = l + jnp.sum(po, axis=1, keepdims=True)
                acc = acc + _dot(po.astype(BF16), v_s[0:d0, :])
            l2 = l[HB:] + jnp.sum(p2, axis=1, keepdims=True)
            acc2 = acc[HB:] + _dot(p2.astype(BF16), v_s[d0 + HB:d0 + BQ, :])
            ctx = jnp.concatenate(
                [acc[:HB] * _recip(l[:HB]), acc2 * _recip(l2)], axis=0).astype(BF16)
            q_s[h, d0:d0 + BQ, :] = ctx

        def head(h, c):
            kvproj(wk_s, k_s, h, KB, 0, S)
            order = list(range(NQ - 1, -1, -1))
            ss = qk(h, order[0])
            kvproj(wv_s, v_s, h, PB, 0, S)
            for n, i in enumerate(order):
                nxt = qk(h, order[n + 1]) if n + 1 < NQ else None
                soft_pv_out(h, i, ss)
                ss = nxt
            return c

        lax.fori_loop(0, N_HEAD_ITERS, head, 0)

        cp_bwot.wait()
        cp_awot.wait()
        for c in cp_axt + cp_aw + [cp_mem0]:
            c.wait()
        ot_s[0] = jnp.zeros((DM, 128), F32)

        def flush(r0):
            stage_s[pl.ds(r0, 128), DM:2 * DM] = ot_s[0].T.astype(BF16)

        def oproj(j, c):
            r0 = pl.multiple_of(j * 128, 128)
            w0 = jnp.minimum(j, DM // 32 - 1) * 32
            pin_w = jnp.maximum(j, DM)
            pin_h = jnp.maximum(j, H)
            pin_o = jnp.where(j >= 0, 1, 0)
            acc = None
            for h in range(H):
                r = _dot_nt(bwot_s[h], q_s[h, pl.ds(r0, 128), :])
                acc = r if acc is None else acc + r
                if h == 0:
                    ot_s[pin_o, 0:8, :] = r[0:8]
                    flush(pl.multiple_of(jnp.maximum(j - 1, 0) * 128, 128))
                elif h in (3, 6, 9, 12):
                    half, g = divmod(h // 3 - 1, 2)
                    rr = pl.multiple_of(w0 + half * 16, 16)
                    rawa_s[2, pin_w, :, 0:128] = r[0:16].astype(BF16)
                    w = jnp.swapaxes(rawa_s[2, pl.ds(rr, 16), g * 8:(g + 1) * 8, :], 0, 1)
                    for u in range(8):
                        awv_s[g * 8 + u, pl.ds(rr, 16), :] = w[u]
                elif h == 14:
                    axt_s[pin_h, 0:16, :] = r[0:16].astype(BF16)
                    ax_s[pl.ds(r0, 128), :] = axt_s[j].T
            ot_s[0] = acc
            return c

        lax.fori_loop(0, N_OPROJ_ITERS, oproj, 0)
        flush(S - 128)

        RC = DM // 4

        def tails(a, b, mul):
            t = [_dot_nt(b[u], a[u]) for u in range(2)]
            return (jnp.concatenate(t, axis=0) * mul).astype(BF16).T

        def wzprep(i, c):
            for n in range(8):
                if n == TAILPOS:
                    wz_s[i, :, 384:512] = tails(
                        [awv_s[2 * i + u] for u in range(2)],
                        [awot_s[2 * i + u, 384:DM, :] for u in range(2)], 1.0)
                rc, u = divmod(n, 2)
                rows = slice(rc * RC, (rc + 1) * RC)
                w = _dot_nt(awv_s[2 * i + u, rows, :], awot_s[2 * i + u, 0:384, :])
                wz_s[i, rows, u * 512:u * 512 + 384] = w.astype(BF16)
                if n < 7:
                    piece = i * 7 + n
                    t = jnp.where(piece >= DM // 16, 1, 0)
                    rr = pl.multiple_of((piece - t * (DM // 16)) * 16, 16)
                    wr = jnp.swapaxes(rawa_s[t, pl.ds(rr, 16)], 0, 1)
                    for h in range(H):
                        wqk_s[t, h, pl.ds(rr, 16), :] = wr[h]
            return c

        lax.fori_loop(0, H // 2, wzprep, 0)

        def gprep(i, c):
            for n in range(2 * GRC):
                if n == GTAIL:
                    wg_s[i, :, 384:512] = tails(
                        [wqk_s[0, 2 * i + u, 0:384, :] for u in range(2)],
                        [wqk_s[1, 2 * i + u, 384:DM, :] for u in range(2)], scale)
                if n == GTAIL2:
                    wu_s[i] = tails(
                        [wqk_s[1, 2 * i + u] for u in range(2)],
                        [wqk_s[0, 2 * i + u, 384:DM, :] for u in range(2)], scale)
                rc, u = divmod(n, 2)
                rows = slice(rc * (384 // GRC), (rc + 1) * (384 // GRC))
                w = _dot_nt(wqk_s[0, 2 * i + u, rows, :], wqk_s[1, 2 * i + u, 0:384, :])
                wg_s[i, rows, u * 512:u * 512 + 384] = (w * scale).astype(BF16)
            return c

        lax.fori_loop(0, H // 2, gprep, 0)

        key = lax.broadcasted_iota(jnp.int32, (L, H * L), 0)
        qry = lax.broadcasted_iota(jnp.int32, (L, H * L), 1) % L
        mask = (qry >= SEG) | (key >= SEG) | (key <= qry)
        lane = lax.broadcasted_iota(jnp.int32, (8, 128), 1)
        lane_l = lax.broadcasted_iota(jnp.int32, (L, 128), 1)
        NT_ = H * L // 128
        tile_heads = [[h for h in range(H) if h * L < (t + 1) * 128 and (h + 1) * L > t * 128]
                      for t in range(NT_)]

        def proj(lhs, w_ref, dests, chunks):
            for i in chunks:
                r = _dot(lhs, w_ref[i])
                mid = r[:, 384:512]
                parts = [(r[:, 0:384].astype(BF16), mid.astype(BF16)),
                         (r[:, 512:896].astype(BF16), pltpu.roll(mid, 64, 1).astype(BF16))]
                for u in range(2):
                    for (a, n, d, b) in dests:
                        r0 = (2 * i + u) * L + b
                        d[r0:r0 + n, 0:384] = parts[u][0][a:a + n]
                        d[r0:r0 + n, 384:512] = parts[u][1][a:a + n]

        def proj_u(lhs, dests):
            for i in range(H // 2):
                r = _dot(lhs, wu_s[i])
                parts = [r.astype(BF16), pltpu.roll(r, 64, 1).astype(BF16)]
                for u in range(2):
                    for (a, n, d, b) in dests:
                        r0 = (2 * i + u) * L + b
                        d[r0:r0 + n, :] = parts[u][a:a + n]

        def head_t(p):
            rs = []
            for t in range(NT_):
                pt = p[:, t * 128:(t + 1) * 128]
                grp = [None] * 16
                for h in tile_heads[t]:
                    for kk in range(L // 8):
                        g = (h * (L // 8) + kk) % 16
                        piece = pt[kk * 8:(kk + 1) * 8]
                        grp[g] = piece if grp[g] is None else jnp.where(
                            lane >= h * L - t * 128, piece, grp[g])
                rs.append(jnp.concatenate(grp, axis=0).T)
            rr = jnp.concatenate(rs, axis=0)
            pcs = []
            for t in range(NT_):
                pc = None
                for h in tile_heads[t]:
                    piece = rr[h * L:(h + 1) * L]
                    pc = piece if pc is None else jnp.where(
                        lane_l >= h * L - t * 128, piece, pc)
                pcs.append(pc)
            return jnp.concatenate(pcs, axis=1)

        def seg(lhs, hs, sel, w):
            def dests(refs):
                return [(a, n, refs[v], b) for (a, n, v, b) in sel]
            ts, zs, us = (ts0, ts1), (zs0, zs1), (us0, us1)
            v = {}
            for step in ORDER.split():
                if step == "U":
                    proj_u(lhs, dests(us))
                elif step[0] == "T":
                    proj(lhs[:, 0:384], wg_s, dests(ts), [int(c) for c in step[1:]])
                elif step[0] == "Z":
                    proj(lhs, wz_s, dests(zs), [int(c) for c in step[1:]])
                elif step == "st":
                    v["st"] = _dot_nt(hs[:, 384:DM], us[w][:, 0:64])
                elif step == "sc":
                    v["sc"] = _dot_nt(hs, ts[w][:, 0:DM])
                elif step == "x1":
                    v["st"] = head_t(v["st"])
                elif step == "sm":
                    sc = jnp.where(mask, v["sc"] + v["st"], NEG)
                    e = jnp.exp(sc - jnp.max(sc, axis=0, keepdims=True))
                    v["p"] = e * _recip(jnp.sum(e, axis=0, keepdims=True))
                elif step == "x2":
                    v["p"] = head_t(v["p"]).astype(BF16)
            return _dot(v["p"], zs[w][...])[:, 0:DM].astype(BF16)

        def out_copy(base):
            return pltpu.make_async_copy(
                stage_s.at[pl.ds(base, 2 * SEG)], out_hbm.at[pl.ds(base, 2 * SEG)], osem)

        def pair(j, mem):
            base = pl.multiple_of(j * 2 * SEG, 2 * SEG)
            x0 = ax_s[pl.ds(base, SEG), :]
            x1 = ax_s[pl.ds(base + SEG, SEG), :]
            lhs1 = jnp.concatenate([x0, x1[0:8], mem], axis=0)
            out1 = seg(lhs1, jnp.concatenate([x0, mem], axis=0),
                       [(0, 32, 0, 0), (32, 8, 1, 0), (40, 8, 0, 32)], 0)
            stage_s[pl.ds(base, SEG), 0:DM] = out1[0:SEG]
            lhs2 = jnp.concatenate([x1[16:32], out1[SEG:L], x1[8:16]], axis=0)
            out2 = seg(lhs2, jnp.concatenate([x1, out1[SEG:L]], axis=0),
                       [(0, 16, 1, 16), (16, 8, 1, 32), (24, 8, 1, 8)], 1)
            stage_s[pl.ds(base + SEG, SEG), 0:DM] = out2[0:SEG]
            out_copy(base).start()
            return out2[SEG:L]

        lax.fori_loop(0, N_PAIR_ITERS, pair, mem0_s[...])
        for j in range(N_PAIR_ITERS):
            out_copy(j * 2 * SEG).wait()

    pl.run_scoped(
        main,
        pltpu.VMEM((2, H, DM, DH), BF16), pltpu.VMEM((H, DM, DH), BF16),
        pltpu.VMEM((H // 2, DM, 2 * DM), BF16), pltpu.VMEM((H // 2, 384, 2 * DM), BF16),
        pltpu.VMEM((H // 2, DM, 128), BF16),
        pltpu.VMEM((S, DM), BF16),
        pltpu.VMEM((S, DH), BF16), pltpu.VMEM((S, DH), BF16),
        pltpu.VMEM((S, 2 * DM), BF16), pltpu.VMEM((2, DM, 128), F32),
        pltpu.VMEM((H * L, 512), BF16), pltpu.VMEM((H * L, 512), BF16),
        pltpu.VMEM((H * L, 512), BF16), pltpu.VMEM((H * L, 512), BF16),
        pltpu.VMEM((H * L, 128), BF16), pltpu.VMEM((H * L, 128), BF16),
    )


@functools.partial(jax.jit, static_argnames=("A_seg_len",))
def pallas_concat_heads__memory_aug_recurrent_mem_tr__compressed_kv_cla__prompt_kernel(
    A_x: jax.Array,
    A_mem0: jax.Array,
    A_Wq: jax.Array,
    A_Wk: jax.Array,
    A_Wv: jax.Array,
    A_Wo: jax.Array,
    A_seg_len: int,
    B_x: jax.Array,
    B_c_kv: jax.Array,
    B_w_q: jax.Array,
    B_w_uk: jax.Array,
    B_w_uv: jax.Array,
    B_w_o: jax.Array,
):
    assert A_seg_len == SEG
    assert A_x.shape == (1, S, DM) and A_mem0.shape == (1, MEM, DM)
    assert A_Wq.shape == (DM, H, DH) and A_Wo.shape == (H, DH, DM)
    assert B_x.shape == (1, S, DM) and B_c_kv.shape == (1, S, DC)
    assert B_w_q.shape == (DM, H, DH) and B_w_uk.shape == (DC, H, DH)
    assert B_w_o.shape == (H, DH, DM)

    axt = jnp.swapaxes(A_x, 1, 2).reshape(DM, S)
    bxt = jnp.swapaxes(B_x, 1, 2).reshape(DM, S)
    awot = jnp.swapaxes(A_Wo, 1, 2)
    bwot = jnp.swapaxes(B_w_o, 1, 2)

    any_spec = pl.BlockSpec(memory_space=pl.ANY)
    out = pl.pallas_call(
        _kernel,
        out_shape=jax.ShapeDtypeStruct((S, 2 * DM), BF16),
        in_specs=[any_spec] * 12,
        out_specs=any_spec,
        scratch_shapes=[
            pltpu.VMEM((H, DC, DH), BF16),
            pltpu.VMEM((H, DC, DH), BF16),
            pltpu.VMEM((S, DC), BF16),
            pltpu.VMEM((H, DM, DH), BF16),
            pltpu.VMEM((H, S, DH), BF16),
            pltpu.VMEM((3, DM + 1, H, DH), BF16),
            pltpu.VMEM((H, DM, DH), BF16),
            pltpu.VMEM((S // 128 + 1, DM, 128), BF16),
            pltpu.VMEM((MEM, DM), BF16),
            pltpu.SemaphoreType.DMA((18,)),
            pltpu.SemaphoreType.DMA,
        ],
        compiler_params=pltpu.CompilerParams(vmem_limit_bytes=120 * 1024 * 1024),
    )(axt, A_mem0.reshape(MEM, DM), A_Wq, A_Wk, A_Wv, awot,
      bxt, B_c_kv.reshape(S, DC), B_w_q, B_w_uk, B_w_uv, bwot)
    return out.reshape(1, S, 2 * DM)
```

```python
import functools

import jax
import jax.numpy as jnp
from jax import lax
import jax.experimental.pallas as pl
import jax.experimental.pallas.tpu as pltpu

F32 = jnp.float32
BF16 = jnp.bfloat16
NT = (((1,), (1,)), ((), ()))
TN = (((0,), (0,)), ((), ()))
NEG = -1000000000.0

S = 2048
DM = 448
H = 16
DH = 256
HD = H * DH
DC = 1024
MEM = 8
SEG = 32
L = SEG + MEM
NPAIR = S // (2 * SEG)

BQ = 256
HB = BQ // 2
NQ = S // BQ
PB = 512
QB = 128
KB = 128
N_OPROJ_ITERS = S // 128
N_HEAD_ITERS = H
N_PAIR_ITERS = NPAIR
TAILPOS = 4
TAILPOS2 = 2
GRC = 2
GTAIL = 2
GTAIL2 = 1
ORDER = 'U T01 st T234567 x1 sc Z01 sm Z2 ut x2 Z34 x3 Z567 F PV'


def _dot(a, b):
    return jnp.dot(a, b, preferred_element_type=F32)


def _dot_nt(a, b):
    return lax.dot_general(a, b, NT, preferred_element_type=F32)


def _recip(l):
    r = pl.reciprocal(l, approx=True)
    return r * (2.0 - l * r)


def _kernel(axt_hbm, mem0_hbm, awq_hbm, awk_hbm, awv_hbm, awot_hbm,
            bxt_hbm, ckv_hbm, bwq_hbm, bwk_hbm, bwv_hbm, bwot_hbm,
            out_hbm,
            wk_s, wv_s, ckv_s, bwot_s, q_s, rawa_s, awot_s, axt_s, mem0_s,
            sems, osem):
    scale = DH ** -0.5

    def cp(src, dst, i):
        return pltpu.make_async_copy(src, dst, sems.at[i])

    cp_ckv = cp(ckv_hbm, ckv_s, 6)
    cp_bwot = cp(bwot_hbm, bwot_s, 7)
    cp_awot = cp(awot_hbm, awot_s, 8)
    cp_axt = [cp(axt_hbm.at[:, pl.ds(j * 128, 128)], axt_s.at[j], 9)
              for j in range(S // 128)]
    cp_aw = [cp(w, rawa_s.at[t, pl.ds(0, DM)], 10 + t)
             for t, w in enumerate((awq_hbm, awk_hbm, awv_hbm))]

    cp_mem0 = cp(mem0_hbm, mem0_s, 13)

    def prologue(bxt_s, bx_s, rawq_s, wq_s, rawk_s, rawv_s):
        cp_bxt = [cp(bxt_hbm.at[:, pl.ds(j * 128, 128)], bxt_s.at[j], 0 if j < 4 else 1)
                  for j in range(S // 128)]
        RQ = DM // 4
        cp_bwq_lo = [cp(bwq_hbm.at[pl.ds(c * RQ, RQ), pl.ds(0, 8), :],
                        rawq_s.at[0, pl.ds(c * RQ, RQ)], 14 + c) for c in range(4)]
        cp_bwq_hi = cp(bwq_hbm.at[:, pl.ds(8, 8), :], rawq_s.at[1], 3)
        cp_bwk = cp(bwk_hbm, rawk_s, 4)
        cp_bwv = cp(bwv_hbm, rawv_s, 5)
        for c in (cp_bxt[:4] + cp_bwq_lo + cp_bxt[4:]
                  + [cp_bwq_hi, cp_bwk, cp_bwv, cp_ckv, cp_bwot, cp_awot] + cp_axt
                  + cp_aw + [cp_mem0]):
            c.start()

        def relayout(src, dst, h0, r0, n):
            w = jnp.swapaxes(src[pl.ds(r0, n)], 0, 1)
            for h in range(w.shape[0]):
                dst[h0 + h, pl.ds(r0, n), :] = w[h]

        def xpose(j):
            r0 = j * 128 if isinstance(j, int) else pl.multiple_of(j * 128, 128)
            bx_s[pl.ds(r0, 128), :] = bxt_s[j].T

        def blk(h0, nh, r_lo, r_hi, side):
            def body(i, c):
                h = h0 + i
                for r in range(r_lo, r_hi):
                    rows = slice(r * QB, (r + 1) * QB)
                    q_s[h, rows, :] = (_dot(bx_s[rows, :], wq_s[h]) * scale).astype(BF16)
                    side(i, r - r_lo)
                return c
            lax.fori_loop(0, nh, body, 0)

        def side_xpose(i, r):
            if r < 3:
                xpose(4 + i * 3 + r)

        def side_wq(i, r):
            if r < 4:
                r0 = jnp.minimum(i, DM // 64 - 1) * 64 + r * 16
                relayout(rawq_s.at[1], wq_s, 8, pl.multiple_of(r0, 16), 16)

        def side_relayout(src, dst):
            def side(i, r):
                relayout(src, dst, 0, pl.multiple_of(i * 256 + r * 16, 16), 16)
            return side

        for c in cp_bxt[:4]:
            c.wait()
        for j in range(4):
            xpose(j)
        for c in range(4):
            cp_bwq_lo[c].wait()
            relayout(rawq_s.at[0], wq_s, 0, c * RQ, RQ)
        blk(0, 4, 0, 4, lambda i, r: None)
        for c in cp_bxt[4:]:
            c.wait()
        blk(4, 4, 0, 4, side_xpose)
        cp_bwq_hi.wait()
        blk(0, 8, 4, 16, side_wq)
        cp_bwk.wait()
        blk(8, 4, 0, 16, side_relayout(rawk_s, wk_s))
        cp_bwv.wait()
        blk(12, 4, 0, 16, side_relayout(rawv_s, wv_s))

    pl.run_scoped(
        prologue,
        pltpu.VMEM((S // 128, DM, 128), BF16), pltpu.VMEM((S, DM), BF16),
        pltpu.VMEM((2, DM, 8, DH), BF16), pltpu.VMEM((H, DM, DH), BF16),
        pltpu.VMEM((DC, H, DH), BF16), pltpu.VMEM((DC, H, DH), BF16),
    )

    def main(wqk_s, awv_s, wz_s, wg_s, wu_s, wt_s, ax_s, k_s, v_s, stage_s, ot_s,
             ts0, ts1, zs0, zs1, us0, us1):
        cp_ckv.wait()

        tri = (lax.broadcasted_iota(jnp.int32, (HB, HB), 1)
               <= lax.broadcasted_iota(jnp.int32, (HB, HB), 0))
        tri2 = (lax.broadcasted_iota(jnp.int32, (BQ, HB), 1)
                <= lax.broadcasted_iota(jnp.int32, (BQ, HB), 0))

        def kvproj(w_ref, dst, h, pb, lo, hi):
            for r0 in range(lo, hi, pb):
                dst[r0:r0 + pb, :] = _dot(ckv_s[r0:r0 + pb, :], w_ref[h]).astype(BF16)

        def qk(h, i):
            d0 = i * BQ
            q = q_s[h, d0:d0 + BQ, :]
            so = _dot_nt(q, k_s[0:d0, :]) if i > 0 else None
            s1 = _dot_nt(q, k_s[d0:d0 + HB, :])
            s2 = _dot_nt(q[HB:], k_s[d0 + HB:d0 + BQ, :])
            return so, s1, s2

        def soft_pv_out(h, i, ss):
            so, s1, s2 = ss
            d0 = i * BQ
            s1 = jnp.where(tri2, s1, NEG)
            s2 = jnp.where(tri, s2, NEG)
            m = jnp.max(s1, axis=1, keepdims=True)
            if so is not None:
                m = jnp.maximum(m, jnp.max(so, axis=1, keepdims=True))
            mb = jnp.maximum(m[HB:], jnp.max(s2, axis=1, keepdims=True))
            m = jnp.concatenate([m[:HB], mb], axis=0)
            p1 = jnp.exp(s1 - m)
            p2 = jnp.exp(s2 - mb)
            l = jnp.sum(p1, axis=1, keepdims=True)
            acc = _dot(p1.astype(BF16), v_s[d0:d0 + HB, :])
            if so is not None:
                po = jnp.exp(so - m)
                l = l + jnp.sum(po, axis=1, keepdims=True)
                acc = acc + _dot(po.astype(BF16), v_s[0:d0, :])
            l2 = l[HB:] + jnp.sum(p2, axis=1, keepdims=True)
            acc2 = acc[HB:] + _dot(p2.astype(BF16), v_s[d0 + HB:d0 + BQ, :])
            ctx = jnp.concatenate(
                [acc[:HB] * _recip(l[:HB]), acc2 * _recip(l2)], axis=0).astype(BF16)
            q_s[h, d0:d0 + BQ, :] = ctx

        def head(h, c):
            kvproj(wk_s, k_s, h, KB, 0, S)
            order = list(range(NQ - 1, -1, -1))
            ss = qk(h, order[0])
            kvproj(wv_s, v_s, h, PB, 0, S)
            for n, i in enumerate(order):
                nxt = qk(h, order[n + 1]) if n + 1 < NQ else None
                soft_pv_out(h, i, ss)
                ss = nxt
            return c

        lax.fori_loop(0, N_HEAD_ITERS, head, 0)

        cp_bwot.wait()
        cp_awot.wait()
        for c in cp_axt + cp_aw + [cp_mem0]:
            c.wait()
        ot_s[0] = jnp.zeros((DM, 128), F32)

        def flush(r0):
            stage_s[pl.ds(r0, 128), DM:2 * DM] = ot_s[0].T.astype(BF16)

        def oproj(j, c):
            r0 = pl.multiple_of(j * 128, 128)
            w0 = jnp.minimum(j, DM // 32 - 1) * 32
            pin_w = jnp.maximum(j, DM)
            pin_h = jnp.maximum(j, H)
            pin_o = jnp.where(j >= 0, 1, 0)
            acc = None
            for h in range(H):
                r = _dot_nt(bwot_s[h], q_s[h, pl.ds(r0, 128), :])
                acc = r if acc is None else acc + r
                if h == 0:
                    ot_s[pin_o, 0:8, :] = r[0:8]
                    flush(pl.multiple_of(jnp.maximum(j - 1, 0) * 128, 128))
                elif h in (3, 6, 9, 12):
                    half, g = divmod(h // 3 - 1, 2)
                    rr = pl.multiple_of(w0 + half * 16, 16)
                    rawa_s[2, pin_w, :, 0:128] = r[0:16].astype(BF16)
                    w = jnp.swapaxes(rawa_s[2, pl.ds(rr, 16), g * 8:(g + 1) * 8, :], 0, 1)
                    for u in range(8):
                        awv_s[g * 8 + u, pl.ds(rr, 16), :] = w[u]
                elif h == 14:
                    axt_s[pin_h, 0:16, :] = r[0:16].astype(BF16)
                    ax_s[pl.ds(r0, 128), :] = axt_s[j].T
            ot_s[0] = acc
            return c

        lax.fori_loop(0, N_OPROJ_ITERS, oproj, 0)
        flush(S - 128)

        RC = 384 // 4

        def tails(a, b, mul):
            t = [_dot_nt(b[u], a[u]) for u in range(2)]
            return (jnp.concatenate(t, axis=0) * mul).astype(BF16).T

        def wzprep(i, c):
            for n in range(8):
                if n == TAILPOS:
                    wz_s[i, :, 384:512] = tails(
                        [awv_s[2 * i + u, 0:384, :] for u in range(2)],
                        [awot_s[2 * i + u, 384:DM, :] for u in range(2)], 1.0)
                if n == TAILPOS2:
                    for u in range(2):
                        wt_s[i, u * 64:(u + 1) * 64, :] = _dot_nt(
                            awv_s[2 * i + u, 384:DM, :], awot_s[2 * i + u]).astype(BF16)
                rc, u = divmod(n, 2)
                rows = slice(rc * RC, (rc + 1) * RC)
                w = _dot_nt(awv_s[2 * i + u, rows, :], awot_s[2 * i + u, 0:384, :])
                wz_s[i, rows, u * 512:u * 512 + 384] = w.astype(BF16)
                if n < 7:
                    piece = i * 7 + n
                    t = jnp.where(piece >= DM // 16, 1, 0)
                    rr = pl.multiple_of((piece - t * (DM // 16)) * 16, 16)
                    wr = jnp.swapaxes(rawa_s[t, pl.ds(rr, 16)], 0, 1)
                    for h in range(H):
                        wqk_s[t, h, pl.ds(rr, 16), :] = wr[h]
            return c

        lax.fori_loop(0, H // 2, wzprep, 0)

        def gprep(i, c):
            for n in range(2 * GRC):
                if n == GTAIL:
                    wg_s[i, :, 384:512] = tails(
                        [wqk_s[0, 2 * i + u, 0:384, :] for u in range(2)],
                        [wqk_s[1, 2 * i + u, 384:DM, :] for u in range(2)], scale)
                if n == GTAIL2:
                    wu_s[i] = tails(
                        [wqk_s[1, 2 * i + u] for u in range(2)],
                        [wqk_s[0, 2 * i + u, 384:DM, :] for u in range(2)], scale)
                rc, u = divmod(n, 2)
                rows = slice(rc * (384 // GRC), (rc + 1) * (384 // GRC))
                w = _dot_nt(wqk_s[0, 2 * i + u, rows, :], wqk_s[1, 2 * i + u, 0:384, :])
                wg_s[i, rows, u * 512:u * 512 + 384] = (w * scale).astype(BF16)
            return c

        lax.fori_loop(0, H // 2, gprep, 0)

        key = lax.broadcasted_iota(jnp.int32, (L, H * L), 0)
        qry = lax.broadcasted_iota(jnp.int32, (L, H * L), 1) % L
        mask = (qry >= SEG) | (key >= SEG) | (key <= qry)
        lane = lax.broadcasted_iota(jnp.int32, (8, 128), 1)
        lane_l = lax.broadcasted_iota(jnp.int32, (L, 128), 1)
        NT_ = H * L // 128
        tile_heads = [[h for h in range(H) if h * L < (t + 1) * 128 and (h + 1) * L > t * 128]
                      for t in range(NT_)]

        def proj(lhs, w_ref, dests, chunks):
            for i in chunks:
                r = _dot(lhs, w_ref[i])
                mid = r[:, 384:512]
                parts = [(r[:, 0:384].astype(BF16), mid.astype(BF16)),
                         (r[:, 512:896].astype(BF16), pltpu.roll(mid, 64, 1).astype(BF16))]
                for u in range(2):
                    for (a, n, d, b) in dests:
                        r0 = (2 * i + u) * L + b
                        d[r0:r0 + n, 0:384] = parts[u][0][a:a + n]
                        d[r0:r0 + n, 384:512] = parts[u][1][a:a + n]

        def proj_u(lhs, dests):
            for i in range(H // 2):
                r = _dot(lhs, wu_s[i])
                parts = [r.astype(BF16), pltpu.roll(r, 64, 1).astype(BF16)]
                for u in range(2):
                    for (a, n, d, b) in dests:
                        r0 = (2 * i + u) * L + b
                        d[r0:r0 + n, :] = parts[u][a:a + n]

        def head_t(p):
            rs = []
            for t in range(NT_):
                pt = p[:, t * 128:(t + 1) * 128]
                grp = [None] * 16
                for h in tile_heads[t]:
                    for kk in range(L // 8):
                        g = (h * (L // 8) + kk) % 16
                        piece = pt[kk * 8:(kk + 1) * 8]
                        grp[g] = piece if grp[g] is None else jnp.where(
                            lane >= h * L - t * 128, piece, grp[g])
                rs.append(jnp.concatenate(grp, axis=0).T)
            rr = jnp.concatenate(rs, axis=0)
            pcs = []
            for t in range(NT_):
                pc = None
                for h in tile_heads[t]:
                    piece = rr[h * L:(h + 1) * L]
                    pc = piece if pc is None else jnp.where(
                        lane_l >= h * L - t * 128, piece, pc)
                pcs.append(pc)
            return jnp.concatenate(pcs, axis=1)

        def seg(lhs, hs, sel, w, left):
            def dests(refs):
                return [(a, n, refs[v], b) for (a, n, v, b) in sel]
            ts, zs, us = (ts0, ts1), (zs0, zs1), (us0, us1)
            v = {}
            for step in ORDER.split():
                if step == "U":
                    proj_u(lhs, dests(us))
                elif step[0] == "T":
                    proj(lhs[:, 0:384], wg_s, dests(ts), [int(c) for c in step[1:]])
                elif step[0] == "Z":
                    proj(lhs[:, 0:384], wz_s, dests(zs), [int(c) for c in step[1:]])
                elif step == "st":
                    v["st"] = _dot_nt(hs[:, 384:DM], us[w][:, 0:64])
                elif step == "sc":
                    v["sc"] = _dot_nt(hs, ts[w][:, 0:DM])
                elif step == "x1":
                    v["st"] = head_t(v["st"])
                elif step == "sm":
                    sc = jnp.where(mask, v["sc"] + v["st"], NEG)
                    e = jnp.exp(sc - jnp.max(sc, axis=0, keepdims=True))
                    v["p"] = e * _recip(jnp.sum(e, axis=0, keepdims=True))
                elif step == "x2":
                    v["pc"] = head_t(v["p"]).astype(BF16)
                elif step == "ut":
                    v["u"] = lax.dot_general(hs[:, 384:DM], v["p"].astype(BF16), TN,
                                             preferred_element_type=F32)
                elif step == "x3":
                    ut = jnp.concatenate([v["u"], v["u"]], axis=0)
                    rr = jnp.concatenate(
                        [ut[:, t * 128:(t + 1) * 128].T for t in range(NT_)], axis=0)
                    v["u"] = jnp.concatenate(
                        [jnp.where(lane_l < 64, rr[2 * i * L:(2 * i + 1) * L],
                                   rr[(2 * i + 1) * L:(2 * i + 2) * L])
                         for i in range(H // 2)], axis=1)
                elif step == "F":
                    rows = v["u"][8:L] if left is None else jnp.concatenate(
                        [v["u"], left], axis=0)
                    v["f"] = _dot(rows.astype(BF16), wt_s[...].reshape(H * 64, DM))
                elif step == "PV":
                    v["o"] = _dot(v["pc"], zs[w][...])[:, 0:DM]
            return v["o"], v["f"], v["u"][0:8]

        def out_copy(base):
            return pltpu.make_async_copy(
                stage_s.at[pl.ds(base, 2 * SEG)], out_hbm.at[pl.ds(base, 2 * SEG)], osem)

        def pair(j, mem):
            base = pl.multiple_of(j * 2 * SEG, 2 * SEG)
            x0 = ax_s[pl.ds(base, SEG), :]
            x1 = ax_s[pl.ds(base + SEG, SEG), :]
            lhs1 = jnp.concatenate([x0, x1[0:8], mem], axis=0)
            o1, f1, left = seg(lhs1, jnp.concatenate([x0, mem], axis=0),
                               [(0, 32, 0, 0), (32, 8, 1, 0), (40, 8, 0, 32)], 0, None)
            mem1 = (o1[SEG:L] + f1[SEG - 8:SEG]).astype(BF16)
            lhs2 = jnp.concatenate([x1[16:32], mem1, x1[8:16]], axis=0)
            o2, f2, _ = seg(lhs2, jnp.concatenate([x1, mem1], axis=0),
                            [(0, 16, 1, 16), (16, 8, 1, 32), (24, 8, 1, 8)], 1, left)
            f1 = jnp.concatenate([f2[L:L + 8], f1[0:SEG - 8]], axis=0)
            stage_s[pl.ds(base, SEG), 0:DM] = (o1[0:SEG] + f1).astype(BF16)
            out2 = (o2 + f2[0:L]).astype(BF16)
            stage_s[pl.ds(base + SEG, SEG), 0:DM] = out2[0:SEG]
            out_copy(base).start()
            return out2[SEG:L]

        lax.fori_loop(0, N_PAIR_ITERS, pair, mem0_s[...])
        for j in range(N_PAIR_ITERS):
            out_copy(j * 2 * SEG).wait()

    pl.run_scoped(
        main,
        pltpu.VMEM((2, H, DM, DH), BF16), pltpu.VMEM((H, DM, DH), BF16),
        pltpu.VMEM((H // 2, 384, 2 * DM), BF16), pltpu.VMEM((H // 2, 384, 2 * DM), BF16),
        pltpu.VMEM((H // 2, DM, 128), BF16), pltpu.VMEM((H // 2, 128, DM), BF16),
        pltpu.VMEM((S, DM), BF16),
        pltpu.VMEM((S, DH), BF16), pltpu.VMEM((S, DH), BF16),
        pltpu.VMEM((S, 2 * DM), BF16), pltpu.VMEM((2, DM, 128), F32),
        pltpu.VMEM((H * L, 512), BF16), pltpu.VMEM((H * L, 512), BF16),
        pltpu.VMEM((H * L, 512), BF16), pltpu.VMEM((H * L, 512), BF16),
        pltpu.VMEM((H * L, 128), BF16), pltpu.VMEM((H * L, 128), BF16),
    )


@functools.partial(jax.jit, static_argnames=("A_seg_len",))
def pallas_concat_heads__memory_aug_recurrent_mem_tr__compressed_kv_cla__prompt_kernel(
    A_x: jax.Array,
    A_mem0: jax.Array,
    A_Wq: jax.Array,
    A_Wk: jax.Array,
    A_Wv: jax.Array,
    A_Wo: jax.Array,
    A_seg_len: int,
    B_x: jax.Array,
    B_c_kv: jax.Array,
    B_w_q: jax.Array,
    B_w_uk: jax.Array,
    B_w_uv: jax.Array,
    B_w_o: jax.Array,
):
    assert A_seg_len == SEG
    assert A_x.shape == (1, S, DM) and A_mem0.shape == (1, MEM, DM)
    assert A_Wq.shape == (DM, H, DH) and A_Wo.shape == (H, DH, DM)
    assert B_x.shape == (1, S, DM) and B_c_kv.shape == (1, S, DC)
    assert B_w_q.shape == (DM, H, DH) and B_w_uk.shape == (DC, H, DH)
    assert B_w_o.shape == (H, DH, DM)

    axt = jnp.swapaxes(A_x, 1, 2).reshape(DM, S)
    bxt = jnp.swapaxes(B_x, 1, 2).reshape(DM, S)
    awot = jnp.swapaxes(A_Wo, 1, 2)
    bwot = jnp.swapaxes(B_w_o, 1, 2)

    any_spec = pl.BlockSpec(memory_space=pl.ANY)
    out = pl.pallas_call(
        _kernel,
        out_shape=jax.ShapeDtypeStruct((S, 2 * DM), BF16),
        in_specs=[any_spec] * 12,
        out_specs=any_spec,
        scratch_shapes=[
            pltpu.VMEM((H, DC, DH), BF16),
            pltpu.VMEM((H, DC, DH), BF16),
            pltpu.VMEM((S, DC), BF16),
            pltpu.VMEM((H, DM, DH), BF16),
            pltpu.VMEM((H, S, DH), BF16),
            pltpu.VMEM((3, DM + 1, H, DH), BF16),
            pltpu.VMEM((H, DM, DH), BF16),
            pltpu.VMEM((S // 128 + 1, DM, 128), BF16),
            pltpu.VMEM((MEM, DM), BF16),
            pltpu.SemaphoreType.DMA((18,)),
            pltpu.SemaphoreType.DMA,
        ],
        compiler_params=pltpu.CompilerParams(vmem_limit_bytes=120 * 1024 * 1024),
    )(axt, A_mem0.reshape(MEM, DM), A_Wq, A_Wk, A_Wv, awot,
      bxt, B_c_kv.reshape(S, DC), B_w_q, B_w_uk, B_w_uv, bwot)
    return out.reshape(1, S, 2 * DM)
```

```python
import functools

import jax
import jax.numpy as jnp
from jax import lax
import jax.experimental.pallas as pl
import jax.experimental.pallas.tpu as pltpu

F32 = jnp.float32
BF16 = jnp.bfloat16
NT = (((1,), (1,)), ((), ()))
TN = (((0,), (0,)), ((), ()))
NEG = -1000000000.0

S = 2048
DM = 448
H = 16
DH = 256
HD = H * DH
DC = 1024
MEM = 8
SEG = 32
L = SEG + MEM
NPAIR = S // (2 * SEG)

BQ = 256
HB = BQ // 2
NQ = S // BQ
PB = 512
QB = 128
KB = 128
N_OPROJ_ITERS = S // 128
N_HEAD_ITERS = H
N_PAIR_ITERS = NPAIR
TAILPOS = 4
TAILPOS2 = 2
PVS = (0,)
GRC = 2
GTAIL = 2
GTAIL2 = 1
ORDER = 'U T01 st T234567 x1 sc Z01 sm Z2 ut x2 Z34 x3 Z567 F PV'


def _dot(a, b):
    return jnp.dot(a, b, preferred_element_type=F32)


def _dot_nt(a, b):
    return lax.dot_general(a, b, NT, preferred_element_type=F32)


def _recip(l):
    r = pl.reciprocal(l, approx=True)
    return r * (2.0 - l * r)


def _kernel(axt_hbm, mem0_hbm, awq_hbm, awk_hbm, awv_hbm, awot_hbm,
            bxt_hbm, ckv_hbm, bwq_hbm, bwk_hbm, bwv_hbm, bwot_hbm,
            out_hbm,
            wk_s, wv_s, ckv_s, bwot_s, q_s, rawa_s, awot_s, axt_s, mem0_s,
            sems, osem):
    scale = DH ** -0.5

    def cp(src, dst, i):
        return pltpu.make_async_copy(src, dst, sems.at[i])

    cp_ckv = cp(ckv_hbm, ckv_s, 6)
    cp_bwot = cp(bwot_hbm, bwot_s, 7)
    cp_awot = cp(awot_hbm, awot_s, 8)
    cp_axt = [cp(axt_hbm.at[:, pl.ds(j * 128, 128)], axt_s.at[j], 9)
              for j in range(S // 128)]
    cp_aw = [cp(w, rawa_s.at[t, pl.ds(0, DM)], 10 + t)
             for t, w in enumerate((awq_hbm, awk_hbm, awv_hbm))]

    cp_mem0 = cp(mem0_hbm, mem0_s, 13)

    def prologue(bxt_s, bx_s, rawq_s, wq_s, rawk_s, rawv_s):
        cp_bxt = [cp(bxt_hbm.at[:, pl.ds(j * 128, 128)], bxt_s.at[j], 0 if j < 4 else 1)
                  for j in range(S // 128)]
        RQ = DM // 4
        cp_bwq_lo = [cp(bwq_hbm.at[pl.ds(c * RQ, RQ), pl.ds(0, 8), :],
                        rawq_s.at[0, pl.ds(c * RQ, RQ)], 14 + c) for c in range(4)]
        cp_bwq_hi = cp(bwq_hbm.at[:, pl.ds(8, 8), :], rawq_s.at[1], 3)
        cp_bwk = cp(bwk_hbm, rawk_s, 4)
        cp_bwv = cp(bwv_hbm, rawv_s, 5)
        for c in (cp_bxt[:4] + cp_bwq_lo + cp_bxt[4:]
                  + [cp_bwq_hi, cp_bwk, cp_bwv, cp_ckv, cp_bwot, cp_awot] + cp_axt
                  + cp_aw + [cp_mem0]):
            c.start()

        def relayout(src, dst, h0, r0, n):
            w = jnp.swapaxes(src[pl.ds(r0, n)], 0, 1)
            for h in range(w.shape[0]):
                dst[h0 + h, pl.ds(r0, n), :] = w[h]

        def xpose(j):
            r0 = j * 128 if isinstance(j, int) else pl.multiple_of(j * 128, 128)
            bx_s[pl.ds(r0, 128), :] = bxt_s[j].T

        def blk(h0, nh, r_lo, r_hi, side):
            def body(i, c):
                h = h0 + i
                for r in range(r_lo, r_hi):
                    rows = slice(r * QB, (r + 1) * QB)
                    q_s[h, rows, :] = (_dot(bx_s[rows, :], wq_s[h]) * scale).astype(BF16)
                    side(i, r - r_lo)
                return c
            lax.fori_loop(0, nh, body, 0)

        def side_xpose(i, r):
            if r < 3:
                xpose(4 + i * 3 + r)

        def side_wq(i, r):
            if r < 4:
                r0 = jnp.minimum(i, DM // 64 - 1) * 64 + r * 16
                relayout(rawq_s.at[1], wq_s, 8, pl.multiple_of(r0, 16), 16)

        def side_relayout(src, dst):
            def side(i, r):
                relayout(src, dst, 0, pl.multiple_of(i * 256 + r * 16, 16), 16)
            return side

        for c in cp_bxt[:4]:
            c.wait()
        for j in range(4):
            xpose(j)
        for c in range(4):
            cp_bwq_lo[c].wait()
            relayout(rawq_s.at[0], wq_s, 0, c * RQ, RQ)
        blk(0, 4, 0, 4, lambda i, r: None)
        for c in cp_bxt[4:]:
            c.wait()
        blk(4, 4, 0, 4, side_xpose)
        cp_bwq_hi.wait()
        blk(0, 8, 4, 16, side_wq)
        cp_bwk.wait()
        blk(8, 4, 0, 16, side_relayout(rawk_s, wk_s))
        cp_bwv.wait()
        blk(12, 4, 0, 16, side_relayout(rawv_s, wv_s))

    pl.run_scoped(
        prologue,
        pltpu.VMEM((S // 128, DM, 128), BF16), pltpu.VMEM((S, DM), BF16),
        pltpu.VMEM((2, DM, 8, DH), BF16), pltpu.VMEM((H, DM, DH), BF16),
        pltpu.VMEM((DC, H, DH), BF16), pltpu.VMEM((DC, H, DH), BF16),
    )

    def main(wqk_s, awv_s, wz_s, wg_s, wu_s, wt_s, ax_s, k_s, v_s, stage_s, ot_s,
             ts0, ts1, zs0, zs1, us0, us1):
        cp_ckv.wait()

        tri = (lax.broadcasted_iota(jnp.int32, (HB, HB), 1)
               <= lax.broadcasted_iota(jnp.int32, (HB, HB), 0))
        tri2 = (lax.broadcasted_iota(jnp.int32, (BQ, HB), 1)
                <= lax.broadcasted_iota(jnp.int32, (BQ, HB), 0))

        def kvproj(w_ref, dst, h, pb, lo, hi):
            for r0 in range(lo, hi, pb):
                dst[r0:r0 + pb, :] = _dot(ckv_s[r0:r0 + pb, :], w_ref[h]).astype(BF16)

        def qk(h, i):
            d0 = i * BQ
            q = q_s[h, d0:d0 + BQ, :]
            so = _dot_nt(q, k_s[0:d0, :]) if i > 0 else None
            s1 = _dot_nt(q, k_s[d0:d0 + HB, :])
            s2 = _dot_nt(q[HB:], k_s[d0 + HB:d0 + BQ, :])
            return so, s1, s2

        def soft_pv_out(h, i, ss):
            so, s1, s2 = ss
            d0 = i * BQ
            s1 = jnp.where(tri2, s1, NEG)
            s2 = jnp.where(tri, s2, NEG)
            m = jnp.max(s1, axis=1, keepdims=True)
            if so is not None:
                m = jnp.maximum(m, jnp.max(so, axis=1, keepdims=True))
            mb = jnp.maximum(m[HB:], jnp.max(s2, axis=1, keepdims=True))
            m = jnp.concatenate([m[:HB], mb], axis=0)
            p1 = jnp.exp(s1 - m)
            p2 = jnp.exp(s2 - mb)
            l = jnp.sum(p1, axis=1, keepdims=True)
            acc = _dot(p1.astype(BF16), v_s[d0:d0 + HB, :])
            if so is not None:
                po = jnp.exp(so - m)
                l = l + jnp.sum(po, axis=1, keepdims=True)
                acc = acc + _dot(po.astype(BF16), v_s[0:d0, :])
            l2 = l[HB:] + jnp.sum(p2, axis=1, keepdims=True)
            acc2 = acc[HB:] + _dot(p2.astype(BF16), v_s[d0 + HB:d0 + BQ, :])
            ctx = jnp.concatenate(
                [acc[:HB] * _recip(l[:HB]), acc2 * _recip(l2)], axis=0).astype(BF16)
            q_s[h, d0:d0 + BQ, :] = ctx

        def head(h, c):
            kvproj(wk_s, k_s, h, KB, 0, S)
            order = list(range(NQ - 1, -1, -1))
            ss = qk(h, order[0])
            kvproj(wv_s, v_s, h, PB, 0, S)
            for n, i in enumerate(order):
                nxt = qk(h, order[n + 1]) if n + 1 < NQ else None
                soft_pv_out(h, i, ss)
                ss = nxt
            return c

        lax.fori_loop(0, N_HEAD_ITERS, head, 0)

        cp_bwot.wait()
        cp_awot.wait()
        for c in cp_axt + cp_aw + [cp_mem0]:
            c.wait()
        ot_s[0] = jnp.zeros((DM, 128), F32)

        def flush(r0):
            stage_s[pl.ds(r0, 128), DM:2 * DM] = ot_s[0].T.astype(BF16)

        def oproj(j, c):
            r0 = pl.multiple_of(j * 128, 128)
            w0 = jnp.minimum(j, DM // 32 - 1) * 32
            pin_w = jnp.maximum(j, DM)
            pin_h = jnp.maximum(j, H)
            pin_o = jnp.where(j >= 0, 1, 0)
            acc = None
            for h in range(H):
                r = _dot_nt(bwot_s[h], q_s[h, pl.ds(r0, 128), :])
                acc = r if acc is None else acc + r
                if h == 0:
                    ot_s[pin_o, 0:8, :] = r[0:8]
                    flush(pl.multiple_of(jnp.maximum(j - 1, 0) * 128, 128))
                elif h in (3, 6, 9, 12):
                    half, g = divmod(h // 3 - 1, 2)
                    rr = pl.multiple_of(w0 + half * 16, 16)
                    rawa_s[2, pin_w, :, 0:128] = r[0:16].astype(BF16)
                    w = jnp.swapaxes(rawa_s[2, pl.ds(rr, 16), g * 8:(g + 1) * 8, :], 0, 1)
                    for u in range(8):
                        awv_s[g * 8 + u, pl.ds(rr, 16), :] = w[u]
                elif h == 14:
                    axt_s[pin_h, 0:16, :] = r[0:16].astype(BF16)
                    ax_s[pl.ds(r0, 128), :] = axt_s[j].T
            ot_s[0] = acc
            return c

        lax.fori_loop(0, N_OPROJ_ITERS, oproj, 0)
        flush(S - 128)

        RC = 384 // 4

        def tails(a, b, mul):
            t = [_dot_nt(b[u], a[u]) for u in range(2)]
            return (jnp.concatenate(t, axis=0) * mul).astype(BF16).T

        def wzprep(i, c):
            for n in range(8):
                if n == TAILPOS:
                    wz_s[i, :, 384:512] = tails(
                        [awv_s[2 * i + u, 0:384, :] for u in range(2)],
                        [awot_s[2 * i + u, 384:DM, :] for u in range(2)], 1.0)
                if n == TAILPOS2:
                    for u in range(2):
                        wt_s[i, u * 64:(u + 1) * 64, :] = _dot_nt(
                            awv_s[2 * i + u, 384:DM, :], awot_s[2 * i + u]).astype(BF16)
                rc, u = divmod(n, 2)
                rows = slice(rc * RC, (rc + 1) * RC)
                w = _dot_nt(awv_s[2 * i + u, rows, :], awot_s[2 * i + u, 0:384, :])
                wz_s[i, rows, u * 512:u * 512 + 384] = w.astype(BF16)
                if n < 7:
                    piece = i * 7 + n
                    t = jnp.where(piece >= DM // 16, 1, 0)
                    rr = pl.multiple_of((piece - t * (DM // 16)) * 16, 16)
                    wr = jnp.swapaxes(rawa_s[t, pl.ds(rr, 16)], 0, 1)
                    for h in range(H):
                        wqk_s[t, h, pl.ds(rr, 16), :] = wr[h]
            return c

        lax.fori_loop(0, H // 2, wzprep, 0)

        def gprep(i, c):
            for n in range(2 * GRC):
                if n == GTAIL:
                    wg_s[i, :, 384:512] = tails(
                        [wqk_s[0, 2 * i + u, 0:384, :] for u in range(2)],
                        [wqk_s[1, 2 * i + u, 384:DM, :] for u in range(2)], scale)
                if n == GTAIL2:
                    wu_s[i] = tails(
                        [wqk_s[1, 2 * i + u] for u in range(2)],
                        [wqk_s[0, 2 * i + u, 384:DM, :] for u in range(2)], scale)
                rc, u = divmod(n, 2)
                rows = slice(rc * (384 // GRC), (rc + 1) * (384 // GRC))
                w = _dot_nt(wqk_s[0, 2 * i + u, rows, :], wqk_s[1, 2 * i + u, 0:384, :])
                wg_s[i, rows, u * 512:u * 512 + 384] = (w * scale).astype(BF16)
            return c

        lax.fori_loop(0, H // 2, gprep, 0)

        key = lax.broadcasted_iota(jnp.int32, (L, H * L), 0)
        qry = lax.broadcasted_iota(jnp.int32, (L, H * L), 1) % L
        mask = (qry >= SEG) | (key >= SEG) | (key <= qry)
        lane = lax.broadcasted_iota(jnp.int32, (8, 128), 1)
        lane_l = lax.broadcasted_iota(jnp.int32, (L, 128), 1)
        NT_ = H * L // 128
        tile_heads = [[h for h in range(H) if h * L < (t + 1) * 128 and (h + 1) * L > t * 128]
                      for t in range(NT_)]

        def proj(lhs, w_ref, dests, chunks):
            for i in chunks:
                r = _dot(lhs, w_ref[i])
                mid = r[:, 384:512]
                parts = [(r[:, 0:384].astype(BF16), mid.astype(BF16)),
                         (r[:, 512:896].astype(BF16), pltpu.roll(mid, 64, 1).astype(BF16))]
                for u in range(2):
                    for (a, n, d, b) in dests:
                        r0 = (2 * i + u) * L + b
                        d[r0:r0 + n, 0:384] = parts[u][0][a:a + n]
                        d[r0:r0 + n, 384:512] = parts[u][1][a:a + n]

        def proj_u(lhs, dests):
            for i in range(H // 2):
                r = _dot(lhs, wu_s[i])
                parts = [r.astype(BF16), pltpu.roll(r, 64, 1).astype(BF16)]
                for u in range(2):
                    for (a, n, d, b) in dests:
                        r0 = (2 * i + u) * L + b
                        d[r0:r0 + n, :] = parts[u][a:a + n]

        def head_t(p):
            rs = []
            for t in range(NT_):
                pt = p[:, t * 128:(t + 1) * 128]
                grp = [None] * 16
                for h in tile_heads[t]:
                    for kk in range(L // 8):
                        g = (h * (L // 8) + kk) % 16
                        piece = pt[kk * 8:(kk + 1) * 8]
                        grp[g] = piece if grp[g] is None else jnp.where(
                            lane >= h * L - t * 128, piece, grp[g])
                rs.append(jnp.concatenate(grp, axis=0).T)
            rr = jnp.concatenate(rs, axis=0)
            pcs = []
            for t in range(NT_):
                pc = None
                for h in tile_heads[t]:
                    piece = rr[h * L:(h + 1) * L]
                    pc = piece if pc is None else jnp.where(
                        lane_l >= h * L - t * 128, piece, pc)
                pcs.append(pc)
            return jnp.concatenate(pcs, axis=1)

        def seg(lhs, hs, sel, w, left):
            def dests(refs):
                return [(a, n, refs[v], b) for (a, n, v, b) in sel]
            ts, zs, us = (ts0, ts1), (zs0, zs1), (us0, us1)
            v = {}
            for step in ORDER.split():
                if step == "U":
                    proj_u(lhs, dests(us))
                elif step[0] == "T":
                    proj(lhs[:, 0:384], wg_s, dests(ts), [int(c) for c in step[1:]])
                elif step[0] == "Z":
                    proj(lhs[:, 0:384], wz_s, dests(zs), [int(c) for c in step[1:]])
                elif step == "st":
                    v["st"] = _dot_nt(hs[:, 384:DM], us[w][:, 0:64])
                elif step == "sc":
                    v["sc"] = _dot_nt(hs, ts[w][:, 0:DM])
                elif step == "x1":
                    v["st"] = head_t(v["st"])
                elif step == "sm":
                    sc = jnp.where(mask, v["sc"] + v["st"], NEG)
                    e = jnp.exp(sc - jnp.max(sc, axis=0, keepdims=True))
                    v["p"] = e * _recip(jnp.sum(e, axis=0, keepdims=True))
                elif step == "x2":
                    v["pf"] = head_t(v["p"])
                    v["pc"] = v["pf"].astype(BF16)
                elif step == "ut":
                    v["u"] = lax.dot_general(hs[:, 384:DM], v["p"].astype(BF16), TN,
                                             preferred_element_type=F32)
                elif step == "x3":
                    ut = jnp.concatenate([v["u"], v["u"]], axis=0)
                    rr = jnp.concatenate(
                        [ut[:, t * 128:(t + 1) * 128].T for t in range(NT_)], axis=0)
                    v["u"] = jnp.concatenate(
                        [jnp.where(lane_l < 64, rr[2 * i * L:(2 * i + 1) * L],
                                   rr[(2 * i + 1) * L:(2 * i + 2) * L])
                         for i in range(H // 2)], axis=1)
                elif step == "F":
                    rows = v["u"][8:L] if left is None else jnp.concatenate(
                        [v["u"], left], axis=0)
                    v["f"] = _dot(rows.astype(BF16), wt_s[...].reshape(H * 64, DM))
                elif step == "PV":
                    if w in PVS:
                        o1 = _dot(v["pf"][24:L].astype(BF16), zs[w][...])[:, 0:DM]
                        o2 = _dot(v["pf"][0:24].astype(BF16), zs[w][...])[:, 0:DM]
                        v["o"] = jnp.concatenate([o2, o1], axis=0)
                    else:
                        v["o"] = _dot(v["pc"], zs[w][...])[:, 0:DM]
            return v["o"], v["f"], v["u"][0:8]

        def out_copy(base):
            return pltpu.make_async_copy(
                stage_s.at[pl.ds(base, 2 * SEG)], out_hbm.at[pl.ds(base, 2 * SEG)], osem)

        def pair(j, mem):
            base = pl.multiple_of(j * 2 * SEG, 2 * SEG)
            x0 = ax_s[pl.ds(base, SEG), :]
            x1 = ax_s[pl.ds(base + SEG, SEG), :]
            lhs1 = jnp.concatenate([x0, x1[0:8], mem], axis=0)
            o1, f1, left = seg(lhs1, jnp.concatenate([x0, mem], axis=0),
                               [(0, 32, 0, 0), (32, 8, 1, 0), (40, 8, 0, 32)], 0, None)
            mem1 = (o1[SEG:L] + f1[SEG - 8:SEG]).astype(BF16)
            lhs2 = jnp.concatenate([x1[16:32], mem1, x1[8:16]], axis=0)
            o2, f2, _ = seg(lhs2, jnp.concatenate([x1, mem1], axis=0),
                            [(0, 16, 1, 16), (16, 8, 1, 32), (24, 8, 1, 8)], 1, left)
            f1 = jnp.concatenate([f2[L:L + 8], f1[0:SEG - 8]], axis=0)
            stage_s[pl.ds(base, SEG), 0:DM] = (o1[0:SEG] + f1).astype(BF16)
            out2 = (o2 + f2[0:L]).astype(BF16)
            stage_s[pl.ds(base + SEG, SEG), 0:DM] = out2[0:SEG]
            out_copy(base).start()
            return out2[SEG:L]

        lax.fori_loop(0, N_PAIR_ITERS, pair, mem0_s[...])
        for j in range(N_PAIR_ITERS):
            out_copy(j * 2 * SEG).wait()

    pl.run_scoped(
        main,
        pltpu.VMEM((2, H, DM, DH), BF16), pltpu.VMEM((H, DM, DH), BF16),
        pltpu.VMEM((H // 2, 384, 2 * DM), BF16), pltpu.VMEM((H // 2, 384, 2 * DM), BF16),
        pltpu.VMEM((H // 2, DM, 128), BF16), pltpu.VMEM((H // 2, 128, DM), BF16),
        pltpu.VMEM((S, DM), BF16),
        pltpu.VMEM((S, DH), BF16), pltpu.VMEM((S, DH), BF16),
        pltpu.VMEM((S, 2 * DM), BF16), pltpu.VMEM((2, DM, 128), F32),
        pltpu.VMEM((H * L, 512), BF16), pltpu.VMEM((H * L, 512), BF16),
        pltpu.VMEM((H * L, 512), BF16), pltpu.VMEM((H * L, 512), BF16),
        pltpu.VMEM((H * L, 128), BF16), pltpu.VMEM((H * L, 128), BF16),
    )


@functools.partial(jax.jit, static_argnames=("A_seg_len",))
def pallas_concat_heads__memory_aug_recurrent_mem_tr__compressed_kv_cla__prompt_kernel(
    A_x: jax.Array,
    A_mem0: jax.Array,
    A_Wq: jax.Array,
    A_Wk: jax.Array,
    A_Wv: jax.Array,
    A_Wo: jax.Array,
    A_seg_len: int,
    B_x: jax.Array,
    B_c_kv: jax.Array,
    B_w_q: jax.Array,
    B_w_uk: jax.Array,
    B_w_uv: jax.Array,
    B_w_o: jax.Array,
):
    assert A_seg_len == SEG
    assert A_x.shape == (1, S, DM) and A_mem0.shape == (1, MEM, DM)
    assert A_Wq.shape == (DM, H, DH) and A_Wo.shape == (H, DH, DM)
    assert B_x.shape == (1, S, DM) and B_c_kv.shape == (1, S, DC)
    assert B_w_q.shape == (DM, H, DH) and B_w_uk.shape == (DC, H, DH)
    assert B_w_o.shape == (H, DH, DM)

    axt = jnp.swapaxes(A_x, 1, 2).reshape(DM, S)
    bxt = jnp.swapaxes(B_x, 1, 2).reshape(DM, S)
    awot = jnp.swapaxes(A_Wo, 1, 2)
    bwot = jnp.swapaxes(B_w_o, 1, 2)

    any_spec = pl.BlockSpec(memory_space=pl.ANY)
    out = pl.pallas_call(
        _kernel,
        out_shape=jax.ShapeDtypeStruct((S, 2 * DM), BF16),
        in_specs=[any_spec] * 12,
        out_specs=any_spec,
        scratch_shapes=[
            pltpu.VMEM((H, DC, DH), BF16),
            pltpu.VMEM((H, DC, DH), BF16),
            pltpu.VMEM((S, DC), BF16),
            pltpu.VMEM((H, DM, DH), BF16),
            pltpu.VMEM((H, S, DH), BF16),
            pltpu.VMEM((3, DM + 1, H, DH), BF16),
            pltpu.VMEM((H, DM, DH), BF16),
            pltpu.VMEM((S // 128 + 1, DM, 128), BF16),
            pltpu.VMEM((MEM, DM), BF16),
            pltpu.SemaphoreType.DMA((18,)),
            pltpu.SemaphoreType.DMA,
        ],
        compiler_params=pltpu.CompilerParams(vmem_limit_bytes=120 * 1024 * 1024),
    )(axt, A_mem0.reshape(MEM, DM), A_Wq, A_Wk, A_Wv, awot,
      bxt, B_c_kv.reshape(S, DC), B_w_q, B_w_uk, B_w_uv, bwot)
    return out.reshape(1, S, 2 * DM)
```

```python
import functools

import jax
import jax.numpy as jnp
from jax import lax
import jax.experimental.pallas as pl
import jax.experimental.pallas.tpu as pltpu

F32 = jnp.float32
BF16 = jnp.bfloat16
NT = (((1,), (1,)), ((), ()))
TN = (((0,), (0,)), ((), ()))
NEG = -1000000000.0

S = 2048
DM = 448
H = 16
DH = 256
HD = H * DH
DC = 1024
MEM = 8
SEG = 32
L = SEG + MEM
NPAIR = S // (2 * SEG)

BQ = 256
HB = BQ // 2
NQ = S // BQ
PB = 512
QB = 128
KB = 128
N_OPROJ_ITERS = S // 128
N_HEAD_ITERS = H
N_PAIR_ITERS = NPAIR
TAILPOS = 4
TAILPOS2 = 2
PVS = (0,)
AVPOS = (5, 7, 9, 11)
GRC = 2
GTAIL = 2
GTAIL2 = 1
ORDER = 'U T01 st T234567 x1 sc Z01 sm Z2 ut x2 Z34 x3 Z567 F PV'


def _dot(a, b):
    return jnp.dot(a, b, preferred_element_type=F32)


def _dot_nt(a, b):
    return lax.dot_general(a, b, NT, preferred_element_type=F32)


def _recip(l):
    r = pl.reciprocal(l, approx=True)
    return r * (2.0 - l * r)


def _kernel(axt_hbm, mem0_hbm, awq_hbm, awk_hbm, awv_hbm, awot_hbm,
            bxt_hbm, ckv_hbm, bwq_hbm, bwk_hbm, bwv_hbm, bwot_hbm,
            out_hbm,
            wk_s, wv_s, ckv_s, bwot_s, q_s, rawa_s, awot_s, awv_s, axt_s, mem0_s,
            sems, osem):
    scale = DH ** -0.5

    def cp(src, dst, i):
        return pltpu.make_async_copy(src, dst, sems.at[i])

    cp_ckv = cp(ckv_hbm, ckv_s, 6)
    cp_bwot = cp(bwot_hbm, bwot_s, 7)
    cp_awot = cp(awot_hbm, awot_s, 8)
    cp_axt = [cp(axt_hbm.at[:, pl.ds(j * 128, 128)], axt_s.at[j], 9)
              for j in range(S // 128)]
    cp_aw = [cp(w, rawa_s.at[t, pl.ds(0, DM)], 10 + t)
             for t, w in enumerate((awq_hbm, awk_hbm))]

    def cp_awv(i):
        lo = min if isinstance(i, int) else jnp.minimum
        return cp(awv_hbm.at[pl.ds(lo(i, DM // 64 - 1) * 64, 64)],
                  rawa_s.at[2, pl.ds(i * 64, 64)], 18 + i)

    cp_mem0 = cp(mem0_hbm, mem0_s, 13)

    def prologue(bxt_s, bx_s, rawq_s, wq_s, rawk_s, rawv_s):
        cp_bxt = [cp(bxt_hbm.at[:, pl.ds(j * 128, 128)], bxt_s.at[j], 0 if j < 4 else 1)
                  for j in range(S // 128)]
        RQ = DM // 4
        cp_bwq_lo = [cp(bwq_hbm.at[pl.ds(c * RQ, RQ), pl.ds(0, 8), :],
                        rawq_s.at[0, pl.ds(c * RQ, RQ)], 14 + c) for c in range(4)]
        cp_bwq_hi = cp(bwq_hbm.at[:, pl.ds(8, 8), :], rawq_s.at[1], 3)
        cp_bwk = cp(bwk_hbm, rawk_s, 4)
        cp_bwv = cp(bwv_hbm, rawv_s, 5)
        for c in (cp_bxt[:4] + cp_bwq_lo + cp_bxt[4:]
                  + [cp_bwq_hi] + [cp_awv(i) for i in range(9)]
                  + [cp_bwk, cp_bwv, cp_ckv, cp_bwot, cp_awot] + cp_axt + cp_aw + [cp_mem0]):
            c.start()

        def relayout(src, dst, h0, r0, n):
            w = jnp.swapaxes(src[pl.ds(r0, n)], 0, 1)
            for h in range(w.shape[0]):
                dst[h0 + h, pl.ds(r0, n), :] = w[h]

        def xpose(j):
            r0 = j * 128 if isinstance(j, int) else pl.multiple_of(j * 128, 128)
            bx_s[pl.ds(r0, 128), :] = bxt_s[j].T

        def blk(h0, nh, r_lo, r_hi, side, post=None):
            def body(i, c):
                h = h0 + i
                for r in range(r_lo, r_hi):
                    rows = slice(r * QB, (r + 1) * QB)
                    q_s[h, rows, :] = (_dot(bx_s[rows, :], wq_s[h]) * scale).astype(BF16)
                    side(i, r - r_lo)
                if post is not None:
                    post(i)
                return c
            lax.fori_loop(0, nh, body, 0)

        def side_xpose(i, r):
            if r < 3:
                xpose(4 + i * 3 + r)

        def side_wq(i, r):
            if r < 4:
                r0 = jnp.minimum(i, DM // 64 - 1) * 64 + r * 16
                relayout(rawq_s.at[1], wq_s, 8, pl.multiple_of(r0, 16), 16)
            if r in AVPOS:
                r0 = i * 64 + AVPOS.index(r) * 16
                relayout(rawa_s.at[2], awv_s, 0, pl.multiple_of(r0, 16), 16)

        def side_relayout(src, dst):
            def side(i, r):
                relayout(src, dst, 0, pl.multiple_of(i * 256 + r * 16, 16), 16)
            return side

        for c in cp_bxt[:4]:
            c.wait()
        for j in range(4):
            xpose(j)
        for c in range(4):
            cp_bwq_lo[c].wait()
            relayout(rawq_s.at[0], wq_s, 0, c * RQ, RQ)
        blk(0, 4, 0, 4, lambda i, r: None)
        for c in cp_bxt[4:]:
            c.wait()
        blk(4, 4, 0, 4, side_xpose)
        cp_bwq_hi.wait()
        cp_awv(0).wait()
        blk(0, 8, 4, 16, side_wq, lambda i: cp_awv(i + 1).wait())
        cp_bwk.wait()
        blk(8, 4, 0, 16, side_relayout(rawk_s, wk_s))
        cp_bwv.wait()
        blk(12, 4, 0, 16, side_relayout(rawv_s, wv_s))

    pl.run_scoped(
        prologue,
        pltpu.VMEM((S // 128, DM, 128), BF16), pltpu.VMEM((S, DM), BF16),
        pltpu.VMEM((2, DM, 8, DH), BF16), pltpu.VMEM((H, DM, DH), BF16),
        pltpu.VMEM((DC, H, DH), BF16), pltpu.VMEM((DC, H, DH), BF16),
    )

    def main(wqk_s, wz_s, wg_s, wu_s, wt_s, ax_s, k_s, v_s, stage_s, ot_s,
             ts0, ts1, zs0, zs1, us0, us1):
        cp_ckv.wait()

        tri = (lax.broadcasted_iota(jnp.int32, (HB, HB), 1)
               <= lax.broadcasted_iota(jnp.int32, (HB, HB), 0))
        tri2 = (lax.broadcasted_iota(jnp.int32, (BQ, HB), 1)
                <= lax.broadcasted_iota(jnp.int32, (BQ, HB), 0))

        def kvproj(w_ref, dst, h, pb, lo, hi):
            for r0 in range(lo, hi, pb):
                dst[r0:r0 + pb, :] = _dot(ckv_s[r0:r0 + pb, :], w_ref[h]).astype(BF16)

        def qk(h, i):
            d0 = i * BQ
            q = q_s[h, d0:d0 + BQ, :]
            so = _dot_nt(q, k_s[0:d0, :]) if i > 0 else None
            s1 = _dot_nt(q, k_s[d0:d0 + HB, :])
            s2 = _dot_nt(q[HB:], k_s[d0 + HB:d0 + BQ, :])
            return so, s1, s2

        def soft_pv_out(h, i, ss):
            so, s1, s2 = ss
            d0 = i * BQ
            s1 = jnp.where(tri2, s1, NEG)
            s2 = jnp.where(tri, s2, NEG)
            m = jnp.max(s1, axis=1, keepdims=True)
            if so is not None:
                m = jnp.maximum(m, jnp.max(so, axis=1, keepdims=True))
            mb = jnp.maximum(m[HB:], jnp.max(s2, axis=1, keepdims=True))
            m = jnp.concatenate([m[:HB], mb], axis=0)
            p1 = jnp.exp(s1 - m)
            p2 = jnp.exp(s2 - mb)
            l = jnp.sum(p1, axis=1, keepdims=True)
            acc = _dot(p1.astype(BF16), v_s[d0:d0 + HB, :])
            if so is not None:
                po = jnp.exp(so - m)
                l = l + jnp.sum(po, axis=1, keepdims=True)
                acc = acc + _dot(po.astype(BF16), v_s[0:d0, :])
            l2 = l[HB:] + jnp.sum(p2, axis=1, keepdims=True)
            acc2 = acc[HB:] + _dot(p2.astype(BF16), v_s[d0 + HB:d0 + BQ, :])
            ctx = jnp.concatenate(
                [acc[:HB] * _recip(l[:HB]), acc2 * _recip(l2)], axis=0).astype(BF16)
            q_s[h, d0:d0 + BQ, :] = ctx

        def head(h, c):
            kvproj(wk_s, k_s, h, KB, 0, S)
            order = list(range(NQ - 1, -1, -1))
            ss = qk(h, order[0])
            kvproj(wv_s, v_s, h, PB, 0, S)
            for n, i in enumerate(order):
                nxt = qk(h, order[n + 1]) if n + 1 < NQ else None
                soft_pv_out(h, i, ss)
                ss = nxt
            return c

        lax.fori_loop(0, N_HEAD_ITERS, head, 0)

        cp_bwot.wait()
        cp_awot.wait()
        for c in cp_axt + cp_aw + [cp_mem0]:
            c.wait()
        ot_s[0] = jnp.zeros((DM, 128), F32)

        def flush(r0):
            stage_s[pl.ds(r0, 128), DM:2 * DM] = ot_s[0].T.astype(BF16)

        def oproj(j, c):
            r0 = pl.multiple_of(j * 128, 128)
            pin_h = jnp.maximum(j, H)
            pin_o = jnp.where(j >= 0, 1, 0)
            acc = None
            for h in range(H):
                r = _dot_nt(bwot_s[h], q_s[h, pl.ds(r0, 128), :])
                acc = r if acc is None else acc + r
                if h == 0:
                    ot_s[pin_o, 0:8, :] = r[0:8]
                    flush(pl.multiple_of(jnp.maximum(j - 1, 0) * 128, 128))
                elif h == 14:
                    axt_s[pin_h, 0:16, :] = r[0:16].astype(BF16)
                    ax_s[pl.ds(r0, 128), :] = axt_s[j].T
            ot_s[0] = acc
            return c

        lax.fori_loop(0, N_OPROJ_ITERS, oproj, 0)
        flush(S - 128)

        RC = 384 // 4

        def tails(a, b, mul):
            t = [_dot_nt(b[u], a[u]) for u in range(2)]
            return (jnp.concatenate(t, axis=0) * mul).astype(BF16).T

        def wzprep(i, c):
            for n in range(8):
                if n == TAILPOS:
                    wz_s[i, :, 384:512] = tails(
                        [awv_s[2 * i + u, 0:384, :] for u in range(2)],
                        [awot_s[2 * i + u, 384:DM, :] for u in range(2)], 1.0)
                if n == TAILPOS2:
                    for u in range(2):
                        wt_s[i, u * 64:(u + 1) * 64, :] = _dot_nt(
                            awv_s[2 * i + u, 384:DM, :], awot_s[2 * i + u]).astype(BF16)
                rc, u = divmod(n, 2)
                rows = slice(rc * RC, (rc + 1) * RC)
                w = _dot_nt(awv_s[2 * i + u, rows, :], awot_s[2 * i + u, 0:384, :])
                wz_s[i, rows, u * 512:u * 512 + 384] = w.astype(BF16)
                if n < 7:
                    piece = i * 7 + n
                    t = jnp.where(piece >= DM // 16, 1, 0)
                    rr = pl.multiple_of((piece - t * (DM // 16)) * 16, 16)
                    wr = jnp.swapaxes(rawa_s[t, pl.ds(rr, 16)], 0, 1)
                    for h in range(H):
                        wqk_s[t, h, pl.ds(rr, 16), :] = wr[h]
            return c

        lax.fori_loop(0, H // 2, wzprep, 0)

        def gprep(i, c):
            for n in range(2 * GRC):
                if n == GTAIL:
                    wg_s[i, :, 384:512] = tails(
                        [wqk_s[0, 2 * i + u, 0:384, :] for u in range(2)],
                        [wqk_s[1, 2 * i + u, 384:DM, :] for u in range(2)], scale)
                if n == GTAIL2:
                    wu_s[i] = tails(
                        [wqk_s[1, 2 * i + u] for u in range(2)],
                        [wqk_s[0, 2 * i + u, 384:DM, :] for u in range(2)], scale)
                rc, u = divmod(n, 2)
                rows = slice(rc * (384 // GRC), (rc + 1) * (384 // GRC))
                w = _dot_nt(wqk_s[0, 2 * i + u, rows, :], wqk_s[1, 2 * i + u, 0:384, :])
                wg_s[i, rows, u * 512:u * 512 + 384] = (w * scale).astype(BF16)
            return c

        lax.fori_loop(0, H // 2, gprep, 0)

        key = lax.broadcasted_iota(jnp.int32, (L, H * L), 0)
        qry = lax.broadcasted_iota(jnp.int32, (L, H * L), 1) % L
        mask = (qry >= SEG) | (key >= SEG) | (key <= qry)
        lane = lax.broadcasted_iota(jnp.int32, (8, 128), 1)
        lane_l = lax.broadcasted_iota(jnp.int32, (L, 128), 1)
        NT_ = H * L // 128
        tile_heads = [[h for h in range(H) if h * L < (t + 1) * 128 and (h + 1) * L > t * 128]
                      for t in range(NT_)]

        def proj(lhs, w_ref, dests, chunks):
            for i in chunks:
                r = _dot(lhs, w_ref[i])
                mid = r[:, 384:512]
                parts = [(r[:, 0:384].astype(BF16), mid.astype(BF16)),
                         (r[:, 512:896].astype(BF16), pltpu.roll(mid, 64, 1).astype(BF16))]
                for u in range(2):
                    for (a, n, d, b) in dests:
                        r0 = (2 * i + u) * L + b
                        d[r0:r0 + n, 0:384] = parts[u][0][a:a + n]
                        d[r0:r0 + n, 384:512] = parts[u][1][a:a + n]

        def proj_u(lhs, dests):
            for i in range(H // 2):
                r = _dot(lhs, wu_s[i])
                parts = [r.astype(BF16), pltpu.roll(r, 64, 1).astype(BF16)]
                for u in range(2):
                    for (a, n, d, b) in dests:
                        r0 = (2 * i + u) * L + b
                        d[r0:r0 + n, :] = parts[u][a:a + n]

        def head_t(p):
            rs = []
            for t in range(NT_):
                pt = p[:, t * 128:(t + 1) * 128]
                grp = [None] * 16
                for h in tile_heads[t]:
                    for kk in range(L // 8):
                        g = (h * (L // 8) + kk) % 16
                        piece = pt[kk * 8:(kk + 1) * 8]
                        grp[g] = piece if grp[g] is None else jnp.where(
                            lane >= h * L - t * 128, piece, grp[g])
                rs.append(jnp.concatenate(grp, axis=0).T)
            rr = jnp.concatenate(rs, axis=0)
            pcs = []
            for t in range(NT_):
                pc = None
                for h in tile_heads[t]:
                    piece = rr[h * L:(h + 1) * L]
                    pc = piece if pc is None else jnp.where(
                        lane_l >= h * L - t * 128, piece, pc)
                pcs.append(pc)
            return jnp.concatenate(pcs, axis=1)

        def seg(lhs, hs, sel, w, left):
            def dests(refs):
                return [(a, n, refs[v], b) for (a, n, v, b) in sel]
            ts, zs, us = (ts0, ts1), (zs0, zs1), (us0, us1)
            v = {}
            for step in ORDER.split():
                if step == "U":
                    proj_u(lhs, dests(us))
                elif step[0] == "T":
                    proj(lhs[:, 0:384], wg_s, dests(ts), [int(c) for c in step[1:]])
                elif step[0] == "Z":
                    proj(lhs[:, 0:384], wz_s, dests(zs), [int(c) for c in step[1:]])
                elif step == "st":
                    v["st"] = _dot_nt(hs[:, 384:DM], us[w][:, 0:64])
                elif step == "sc":
                    v["sc"] = _dot_nt(hs, ts[w][:, 0:DM])
                elif step == "x1":
                    v["st"] = head_t(v["st"])
                elif step == "sm":
                    sc = jnp.where(mask, v["sc"] + v["st"], NEG)
                    e = jnp.exp(sc - jnp.max(sc, axis=0, keepdims=True))
                    v["p"] = e * _recip(jnp.sum(e, axis=0, keepdims=True))
                elif step == "x2":
                    v["pf"] = head_t(v["p"])
                    v["pc"] = v["pf"].astype(BF16)
                elif step == "ut":
                    v["u"] = lax.dot_general(hs[:, 384:DM], v["p"].astype(BF16), TN,
                                             preferred_element_type=F32)
                elif step == "x3":
                    ut = jnp.concatenate([v["u"], v["u"]], axis=0)
                    rr = jnp.concatenate(
                        [ut[:, t * 128:(t + 1) * 128].T for t in range(NT_)], axis=0)
                    v["u"] = jnp.concatenate(
                        [jnp.where(lane_l < 64, rr[2 * i * L:(2 * i + 1) * L],
                                   rr[(2 * i + 1) * L:(2 * i + 2) * L])
                         for i in range(H // 2)], axis=1)
                elif step == "F":
                    rows = v["u"][8:L] if left is None else jnp.concatenate(
                        [v["u"], left], axis=0)
                    v["f"] = _dot(rows.astype(BF16), wt_s[...].reshape(H * 64, DM))
                elif step == "PV":
                    if w in PVS:
                        o1 = _dot(v["pf"][24:L].astype(BF16), zs[w][...])[:, 0:DM]
                        o2 = _dot(v["pf"][0:24].astype(BF16), zs[w][...])[:, 0:DM]
                        v["o"] = jnp.concatenate([o2, o1], axis=0)
                    else:
                        v["o"] = _dot(v["pc"], zs[w][...])[:, 0:DM]
            return v["o"], v["f"], v["u"][0:8]

        def out_copy(base):
            return pltpu.make_async_copy(
                stage_s.at[pl.ds(base, 2 * SEG)], out_hbm.at[pl.ds(base, 2 * SEG)], osem)

        def pair(j, mem):
            base = pl.multiple_of(j * 2 * SEG, 2 * SEG)
            x0 = ax_s[pl.ds(base, SEG), :]
            x1 = ax_s[pl.ds(base + SEG, SEG), :]
            lhs1 = jnp.concatenate([x0, x1[0:8], mem], axis=0)
            o1, f1, left = seg(lhs1, jnp.concatenate([x0, mem], axis=0),
                               [(0, 32, 0, 0), (32, 8, 1, 0), (40, 8, 0, 32)], 0, None)
            mem1 = (o1[SEG:L] + f1[SEG - 8:SEG]).astype(BF16)
            lhs2 = jnp.concatenate([x1[16:32], mem1, x1[8:16]], axis=0)
            o2, f2, _ = seg(lhs2, jnp.concatenate([x1, mem1], axis=0),
                            [(0, 16, 1, 16), (16, 8, 1, 32), (24, 8, 1, 8)], 1, left)
            f1 = jnp.concatenate([f2[L:L + 8], f1[0:SEG - 8]], axis=0)
            stage_s[pl.ds(base, SEG), 0:DM] = (o1[0:SEG] + f1).astype(BF16)
            out2 = (o2 + f2[0:L]).astype(BF16)
            stage_s[pl.ds(base + SEG, SEG), 0:DM] = out2[0:SEG]
            out_copy(base).start()
            return out2[SEG:L]

        lax.fori_loop(0, N_PAIR_ITERS, pair, mem0_s[...])
        for j in range(N_PAIR_ITERS):
            out_copy(j * 2 * SEG).wait()

    pl.run_scoped(
        main,
        pltpu.VMEM((2, H, DM, DH), BF16),
        pltpu.VMEM((H // 2, 384, 2 * DM), BF16), pltpu.VMEM((H // 2, 384, 2 * DM), BF16),
        pltpu.VMEM((H // 2, DM, 128), BF16), pltpu.VMEM((H // 2, 128, DM), BF16),
        pltpu.VMEM((S, DM), BF16),
        pltpu.VMEM((S, DH), BF16), pltpu.VMEM((S, DH), BF16),
        pltpu.VMEM((S, 2 * DM), BF16), pltpu.VMEM((2, DM, 128), F32),
        pltpu.VMEM((H * L, 512), BF16), pltpu.VMEM((H * L, 512), BF16),
        pltpu.VMEM((H * L, 512), BF16), pltpu.VMEM((H * L, 512), BF16),
        pltpu.VMEM((H * L, 128), BF16), pltpu.VMEM((H * L, 128), BF16),
    )


@functools.partial(jax.jit, static_argnames=("A_seg_len",))
def pallas_concat_heads__memory_aug_recurrent_mem_tr__compressed_kv_cla__prompt_kernel(
    A_x: jax.Array,
    A_mem0: jax.Array,
    A_Wq: jax.Array,
    A_Wk: jax.Array,
    A_Wv: jax.Array,
    A_Wo: jax.Array,
    A_seg_len: int,
    B_x: jax.Array,
    B_c_kv: jax.Array,
    B_w_q: jax.Array,
    B_w_uk: jax.Array,
    B_w_uv: jax.Array,
    B_w_o: jax.Array,
):
    assert A_seg_len == SEG
    assert A_x.shape == (1, S, DM) and A_mem0.shape == (1, MEM, DM)
    assert A_Wq.shape == (DM, H, DH) and A_Wo.shape == (H, DH, DM)
    assert B_x.shape == (1, S, DM) and B_c_kv.shape == (1, S, DC)
    assert B_w_q.shape == (DM, H, DH) and B_w_uk.shape == (DC, H, DH)
    assert B_w_o.shape == (H, DH, DM)

    axt = jnp.swapaxes(A_x, 1, 2).reshape(DM, S)
    bxt = jnp.swapaxes(B_x, 1, 2).reshape(DM, S)
    awot = jnp.swapaxes(A_Wo, 1, 2)
    bwot = jnp.swapaxes(B_w_o, 1, 2)

    any_spec = pl.BlockSpec(memory_space=pl.ANY)
    out = pl.pallas_call(
        _kernel,
        out_shape=jax.ShapeDtypeStruct((S, 2 * DM), BF16),
        in_specs=[any_spec] * 12,
        out_specs=any_spec,
        scratch_shapes=[
            pltpu.VMEM((H, DC, DH), BF16),
            pltpu.VMEM((H, DC, DH), BF16),
            pltpu.VMEM((S, DC), BF16),
            pltpu.VMEM((H, DM, DH), BF16),
            pltpu.VMEM((H, S, DH), BF16),
            pltpu.VMEM((3, DM + 128, H, DH), BF16),
            pltpu.VMEM((H, DM, DH), BF16),
            pltpu.VMEM((H, DM + 64, DH), BF16),
            pltpu.VMEM((S // 128 + 1, DM, 128), BF16),
            pltpu.VMEM((MEM, DM), BF16),
            pltpu.SemaphoreType.DMA((27,)),
            pltpu.SemaphoreType.DMA,
        ],
        compiler_params=pltpu.CompilerParams(vmem_limit_bytes=120 * 1024 * 1024),
    )(axt, A_mem0.reshape(MEM, DM), A_Wq, A_Wk, A_Wv, awot,
      bxt, B_c_kv.reshape(S, DC), B_w_q, B_w_uk, B_w_uv, bwot)
    return out.reshape(1, S, 2 * DM)
```

```python
import functools

import jax
import jax.numpy as jnp
from jax import lax
import jax.experimental.pallas as pl
import jax.experimental.pallas.tpu as pltpu

F32 = jnp.float32
BF16 = jnp.bfloat16
NT = (((1,), (1,)), ((), ()))
TN = (((0,), (0,)), ((), ()))
NEG = -1000000000.0

S = 2048
DM = 448
H = 16
DH = 256
HD = H * DH
DC = 1024
MEM = 8
SEG = 32
L = SEG + MEM
NPAIR = S // (2 * SEG)

BQ = 256
HB = BQ // 2
NQ = S // BQ
PB = 512
QB = 128
KB = 128
N_OPROJ_ITERS = S // 128
N_HEAD_ITERS = H
N_PAIR_ITERS = NPAIR
TAILPOS = 4
TAILPOS2 = 2
PVS = (0,)
OU = 2
WU = 1
GU = 2
B1U = 1
B2U = 1
AVPOS = (5, 7, 9, 11)
GRC = 2
GTAIL = 2
GTAIL2 = 1
ORDER = 'U T01 st T234567 x1 sc Z01 sm Z2 ut x2 Z34 x3 Z567 F PV'


def _dot(a, b):
    return jnp.dot(a, b, preferred_element_type=F32)


def _dot_nt(a, b):
    return lax.dot_general(a, b, NT, preferred_element_type=F32)


def _recip(l):
    r = pl.reciprocal(l, approx=True)
    return r * (2.0 - l * r)


def _kernel(axt_hbm, mem0_hbm, awq_hbm, awk_hbm, awv_hbm, awot_hbm,
            bxt_hbm, ckv_hbm, bwq_hbm, bwk_hbm, bwv_hbm, bwot_hbm,
            out_hbm,
            wkv_s, ckv_s, bwot_s, q_s, rawa_s, awot_s, awv_s, axt_s, mem0_s,
            sems, osem):
    scale = DH ** -0.5

    def cp(src, dst, i):
        return pltpu.make_async_copy(src, dst, sems.at[i])

    cp_ckv = cp(ckv_hbm, ckv_s, 6)
    cp_bwot = cp(bwot_hbm, bwot_s, 7)
    cp_awot = cp(awot_hbm, awot_s, 8)
    cp_axt = [cp(axt_hbm.at[:, pl.ds(j * 128, 128)], axt_s.at[j], 9)
              for j in range(S // 128)]
    cp_aw = [cp(w, rawa_s.at[t, pl.ds(0, DM)], 10 + t)
             for t, w in enumerate((awq_hbm, awk_hbm))]

    def cp_awv(i):
        lo = min if isinstance(i, int) else jnp.minimum
        return cp(awv_hbm.at[pl.ds(lo(i, DM // 64 - 1) * 64, 64)],
                  rawa_s.at[2, pl.ds(i * 64, 64)], 18 + i)

    cp_mem0 = cp(mem0_hbm, mem0_s, 13)

    def prologue(bxt_s, bx_s, rawq_s, wq_s, rawkv_s):
        cp_bxt = [cp(bxt_hbm.at[:, pl.ds(j * 128, 128)], bxt_s.at[j], 0 if j < 4 else 1)
                  for j in range(S // 128)]
        RQ = DM // 4
        cp_bwq_lo = [cp(bwq_hbm.at[pl.ds(c * RQ, RQ), pl.ds(0, 8), :],
                        rawq_s.at[0, pl.ds(c * RQ, RQ)], 14 + c) for c in range(4)]
        cp_bwq_hi = cp(bwq_hbm.at[:, pl.ds(8, 8), :], rawq_s.at[1], 3)

        def cp_kv(i):
            src = bwk_hbm if i < 4 else bwv_hbm
            return cp(src.at[pl.ds(min(i % 4 + i // 8 * 3, 3) * 256, 256)],
                      rawkv_s.at[pl.ds(i * 256, 256)], 27 + i)

        def wait_kv(i):
            dst = rawkv_s.at[pl.ds(i * 256, 256)]
            cp(dst, dst, 27 + i).wait()

        for c in (cp_bxt[:4] + cp_bwq_lo + cp_bxt[4:]
                  + [cp_bwq_hi] + [cp_awv(i) for i in range(9)]
                  + [cp_kv(i) for i in range(9)]
                  + [cp_ckv, cp_bwot, cp_awot] + cp_axt + cp_aw + [cp_mem0]):
            c.start()

        def relayout(src, dst, h0, r0, n):
            w = jnp.swapaxes(src[pl.ds(r0, n)], 0, 1)
            for h in range(w.shape[0]):
                dst[h0 + h, pl.ds(r0, n), :] = w[h]

        def xpose(j):
            r0 = j * 128 if isinstance(j, int) else pl.multiple_of(j * 128, 128)
            bx_s[pl.ds(r0, 128), :] = bxt_s[j].T

        def blk(h0, nh, r_lo, r_hi, side, post=None, unroll=1):
            def body(i, c):
                h = h0 + i
                for r in range(r_lo, r_hi):
                    rows = slice(r * QB, (r + 1) * QB)
                    q_s[h, rows, :] = (_dot(bx_s[rows, :], wq_s[h]) * scale).astype(BF16)
                    side(i, r - r_lo)
                if post is not None:
                    post(i)
                return c
            lax.fori_loop(0, nh, body, 0, unroll=unroll)

        def side_xpose(i, r):
            if r < 3:
                xpose(4 + i * 3 + r)

        def side_wq(i, r):
            if r < 4:
                r0 = jnp.minimum(i, DM // 64 - 1) * 64 + r * 16
                relayout(rawq_s.at[1], wq_s, 8, pl.multiple_of(r0, 16), 16)
            if r in AVPOS:
                r0 = i * 64 + AVPOS.index(r) * 16
                relayout(rawa_s.at[2], awv_s, 0, pl.multiple_of(r0, 16), 16)

        def side_kv(i, r):
            w = jnp.swapaxes(rawkv_s[pl.ds(pl.multiple_of(i * 256 + r * 16, 16), 16)], 0, 1)
            r0 = pl.multiple_of((i % 4) * 256 + r * 16, 16)
            for h in range(H):
                wkv_s[(i // 4) * H + h, pl.ds(r0, 16), :] = w[h]

        for c in cp_bxt[:4]:
            c.wait()
        for j in range(4):
            xpose(j)
        for c in range(4):
            cp_bwq_lo[c].wait()
            relayout(rawq_s.at[0], wq_s, 0, c * RQ, RQ)
        blk(0, 4, 0, 4, lambda i, r: None, unroll=B1U)
        for c in cp_bxt[4:]:
            c.wait()
        blk(4, 4, 0, 4, side_xpose, unroll=B2U)
        cp_bwq_hi.wait()
        cp_awv(0).wait()
        blk(0, 8, 4, 16, side_wq, lambda i: cp_awv(i + 1).wait())
        wait_kv(0)
        blk(8, 8, 0, 16, side_kv, lambda i: wait_kv(i + 1))

    pl.run_scoped(
        prologue,
        pltpu.VMEM((S // 128, DM, 128), BF16), pltpu.VMEM((S, DM), BF16),
        pltpu.VMEM((2, DM, 8, DH), BF16), pltpu.VMEM((H, DM, DH), BF16),
        pltpu.VMEM((2 * DC + 256, H, DH), BF16),
    )

    def main(wqk_s, wz_s, wg_s, wu_s, wt_s, ax_s, k_s, v_s, stage_s, ot_s,
             ts0, ts1, zs0, zs1, us0, us1):
        cp_ckv.wait()

        tri = (lax.broadcasted_iota(jnp.int32, (HB, HB), 1)
               <= lax.broadcasted_iota(jnp.int32, (HB, HB), 0))
        tri2 = (lax.broadcasted_iota(jnp.int32, (BQ, HB), 1)
                <= lax.broadcasted_iota(jnp.int32, (BQ, HB), 0))

        def kvproj(dst, h, pb, lo, hi):
            for r0 in range(lo, hi, pb):
                dst[r0:r0 + pb, :] = _dot(ckv_s[r0:r0 + pb, :], wkv_s[h]).astype(BF16)

        def qk(h, i):
            d0 = i * BQ
            q = q_s[h, d0:d0 + BQ, :]
            so = _dot_nt(q, k_s[0:d0, :]) if i > 0 else None
            s1 = _dot_nt(q, k_s[d0:d0 + HB, :])
            s2 = _dot_nt(q[HB:], k_s[d0 + HB:d0 + BQ, :])
            return so, s1, s2

        def soft_pv_out(h, i, ss):
            so, s1, s2 = ss
            d0 = i * BQ
            s1 = jnp.where(tri2, s1, NEG)
            s2 = jnp.where(tri, s2, NEG)
            m = jnp.max(s1, axis=1, keepdims=True)
            if so is not None:
                m = jnp.maximum(m, jnp.max(so, axis=1, keepdims=True))
            mb = jnp.maximum(m[HB:], jnp.max(s2, axis=1, keepdims=True))
            m = jnp.concatenate([m[:HB], mb], axis=0)
            p1 = jnp.exp(s1 - m)
            p2 = jnp.exp(s2 - mb)
            l = jnp.sum(p1, axis=1, keepdims=True)
            acc = _dot(p1.astype(BF16), v_s[d0:d0 + HB, :])
            if so is not None:
                po = jnp.exp(so - m)
                l = l + jnp.sum(po, axis=1, keepdims=True)
                acc = acc + _dot(po.astype(BF16), v_s[0:d0, :])
            l2 = l[HB:] + jnp.sum(p2, axis=1, keepdims=True)
            acc2 = acc[HB:] + _dot(p2.astype(BF16), v_s[d0 + HB:d0 + BQ, :])
            ctx = jnp.concatenate(
                [acc[:HB] * _recip(l[:HB]), acc2 * _recip(l2)], axis=0).astype(BF16)
            q_s[h, d0:d0 + BQ, :] = ctx

        def head(h, c):
            kvproj(k_s, h, KB, 0, S)
            order = list(range(NQ - 1, -1, -1))
            ss = qk(h, order[0])
            kvproj(v_s, H + h, PB, 0, S)
            for n, i in enumerate(order):
                nxt = qk(h, order[n + 1]) if n + 1 < NQ else None
                soft_pv_out(h, i, ss)
                ss = nxt
            return c

        lax.fori_loop(0, N_HEAD_ITERS, head, 0)

        cp_bwot.wait()
        cp_awot.wait()
        for c in cp_axt + cp_aw + [cp_mem0]:
            c.wait()
        ot_s[0] = jnp.zeros((DM, 128), F32)

        def flush(r0):
            stage_s[pl.ds(r0, 128), DM:2 * DM] = ot_s[0].T.astype(BF16)

        def oproj(j, c):
            r0 = pl.multiple_of(j * 128, 128)
            pin_h = jnp.maximum(j, H)
            pin_o = jnp.where(j >= 0, 1, 0)
            acc = None
            for h in range(H):
                r = _dot_nt(bwot_s[h], q_s[h, pl.ds(r0, 128), :])
                acc = r if acc is None else acc + r
                if h == 0:
                    ot_s[pin_o, 0:8, :] = r[0:8]
                    flush(pl.multiple_of(jnp.maximum(j - 1, 0) * 128, 128))
                elif h == 14:
                    axt_s[pin_h, 0:16, :] = r[0:16].astype(BF16)
                    ax_s[pl.ds(r0, 128), :] = axt_s[j].T
            ot_s[0] = acc
            return c

        lax.fori_loop(0, N_OPROJ_ITERS, oproj, 0, unroll=OU)
        flush(S - 128)

        RC = 384 // 4

        def tails(a, b, mul):
            t = [_dot_nt(b[u], a[u]) for u in range(2)]
            return (jnp.concatenate(t, axis=0) * mul).astype(BF16).T

        def wzprep(i, c):
            for n in range(8):
                if n == TAILPOS:
                    wz_s[i, :, 384:512] = tails(
                        [awv_s[2 * i + u, 0:384, :] for u in range(2)],
                        [awot_s[2 * i + u, 384:DM, :] for u in range(2)], 1.0)
                if n == TAILPOS2:
                    for u in range(2):
                        wt_s[i, u * 64:(u + 1) * 64, :] = _dot_nt(
                            awv_s[2 * i + u, 384:DM, :], awot_s[2 * i + u]).astype(BF16)
                rc, u = divmod(n, 2)
                rows = slice(rc * RC, (rc + 1) * RC)
                w = _dot_nt(awv_s[2 * i + u, rows, :], awot_s[2 * i + u, 0:384, :])
                wz_s[i, rows, u * 512:u * 512 + 384] = w.astype(BF16)
                if n < 7:
                    piece = i * 7 + n
                    t = jnp.where(piece >= DM // 16, 1, 0)
                    rr = pl.multiple_of((piece - t * (DM // 16)) * 16, 16)
                    wr = jnp.swapaxes(rawa_s[t, pl.ds(rr, 16)], 0, 1)
                    for h in range(H):
                        wqk_s[t, h, pl.ds(rr, 16), :] = wr[h]
            return c

        lax.fori_loop(0, H // 2, wzprep, 0, unroll=WU)

        def gprep(i, c):
            for n in range(2 * GRC):
                if n == GTAIL:
                    wg_s[i, :, 384:512] = tails(
                        [wqk_s[0, 2 * i + u, 0:384, :] for u in range(2)],
                        [wqk_s[1, 2 * i + u, 384:DM, :] for u in range(2)], scale)
                if n == GTAIL2:
                    wu_s[i] = tails(
                        [wqk_s[1, 2 * i + u] for u in range(2)],
                        [wqk_s[0, 2 * i + u, 384:DM, :] for u in range(2)], scale)
                rc, u = divmod(n, 2)
                rows = slice(rc * (384 // GRC), (rc + 1) * (384 // GRC))
                w = _dot_nt(wqk_s[0, 2 * i + u, rows, :], wqk_s[1, 2 * i + u, 0:384, :])
                wg_s[i, rows, u * 512:u * 512 + 384] = (w * scale).astype(BF16)
            return c

        lax.fori_loop(0, H // 2, gprep, 0, unroll=GU)

        key = lax.broadcasted_iota(jnp.int32, (L, H * L), 0)
        qry = lax.broadcasted_iota(jnp.int32, (L, H * L), 1) % L
        mask = (qry >= SEG) | (key >= SEG) | (key <= qry)
        lane = lax.broadcasted_iota(jnp.int32, (8, 128), 1)
        lane_l = lax.broadcasted_iota(jnp.int32, (L, 128), 1)
        NT_ = H * L // 128
        tile_heads = [[h for h in range(H) if h * L < (t + 1) * 128 and (h + 1) * L > t * 128]
                      for t in range(NT_)]

        def proj(lhs, w_ref, dests, chunks):
            for i in chunks:
                r = _dot(lhs, w_ref[i])
                mid = r[:, 384:512]
                parts = [(r[:, 0:384].astype(BF16), mid.astype(BF16)),
                         (r[:, 512:896].astype(BF16), pltpu.roll(mid, 64, 1).astype(BF16))]
                for u in range(2):
                    for (a, n, d, b) in dests:
                        r0 = (2 * i + u) * L + b
                        d[r0:r0 + n, 0:384] = parts[u][0][a:a + n]
                        d[r0:r0 + n, 384:512] = parts[u][1][a:a + n]

        def proj_u(lhs, dests):
            for i in range(H // 2):
                r = _dot(lhs, wu_s[i])
                parts = [r.astype(BF16), pltpu.roll(r, 64, 1).astype(BF16)]
                for u in range(2):
                    for (a, n, d, b) in dests:
                        r0 = (2 * i + u) * L + b
                        d[r0:r0 + n, :] = parts[u][a:a + n]

        def head_t(p):
            rs = []
            for t in range(NT_):
                pt = p[:, t * 128:(t + 1) * 128]
                grp = [None] * 16
                for h in tile_heads[t]:
                    for kk in range(L // 8):
                        g = (h * (L // 8) + kk) % 16
                        piece = pt[kk * 8:(kk + 1) * 8]
                        grp[g] = piece if grp[g] is None else jnp.where(
                            lane >= h * L - t * 128, piece, grp[g])
                rs.append(jnp.concatenate(grp, axis=0).T)
            rr = jnp.concatenate(rs, axis=0)
            pcs = []
            for t in range(NT_):
                pc = None
                for h in tile_heads[t]:
                    piece = rr[h * L:(h + 1) * L]
                    pc = piece if pc is None else jnp.where(
                        lane_l >= h * L - t * 128, piece, pc)
                pcs.append(pc)
            return jnp.concatenate(pcs, axis=1)

        def seg(lhs, hs, sel, w, left):
            def dests(refs):
                return [(a, n, refs[v], b) for (a, n, v, b) in sel]
            ts, zs, us = (ts0, ts1), (zs0, zs1), (us0, us1)
            v = {}
            for step in ORDER.split():
                if step == "U":
                    proj_u(lhs, dests(us))
                elif step[0] == "T":
                    proj(lhs[:, 0:384], wg_s, dests(ts), [int(c) for c in step[1:]])
                elif step[0] == "Z":
                    proj(lhs[:, 0:384], wz_s, dests(zs), [int(c) for c in step[1:]])
                elif step == "st":
                    v["st"] = _dot_nt(hs[:, 384:DM], us[w][:, 0:64])
                elif step == "sc":
                    v["sc"] = _dot_nt(hs, ts[w][:, 0:DM])
                elif step == "x1":
                    v["st"] = head_t(v["st"])
                elif step == "sm":
                    sc = jnp.where(mask, v["sc"] + v["st"], NEG)
                    e = jnp.exp(sc - jnp.max(sc, axis=0, keepdims=True))
                    v["p"] = e * _recip(jnp.sum(e, axis=0, keepdims=True))
                elif step == "x2":
                    v["pf"] = head_t(v["p"])
                    v["pc"] = v["pf"].astype(BF16)
                elif step == "ut":
                    v["u"] = lax.dot_general(hs[:, 384:DM], v["p"].astype(BF16), TN,
                                             preferred_element_type=F32)
                elif step == "x3":
                    ut = jnp.concatenate([v["u"], v["u"]], axis=0)
                    rr = jnp.concatenate(
                        [ut[:, t * 128:(t + 1) * 128].T for t in range(NT_)], axis=0)
                    v["u"] = jnp.concatenate(
                        [jnp.where(lane_l < 64, rr[2 * i * L:(2 * i + 1) * L],
                                   rr[(2 * i + 1) * L:(2 * i + 2) * L])
                         for i in range(H // 2)], axis=1)
                elif step == "F":
                    rows = v["u"][8:L] if left is None else jnp.concatenate(
                        [v["u"], left], axis=0)
                    v["f"] = _dot(rows.astype(BF16), wt_s[...].reshape(H * 64, DM))
                elif step == "PV":
                    if w in PVS:
                        o1 = _dot(v["pf"][24:L].astype(BF16), zs[w][...])[:, 0:DM]
                        o2 = _dot(v["pf"][0:24].astype(BF16), zs[w][...])[:, 0:DM]
                        v["o"] = jnp.concatenate([o2, o1], axis=0)
                    else:
                        v["o"] = _dot(v["pc"], zs[w][...])[:, 0:DM]
            return v["o"], v["f"], v["u"][0:8]

        def out_copy(base):
            return pltpu.make_async_copy(
                stage_s.at[pl.ds(base, 2 * SEG)], out_hbm.at[pl.ds(base, 2 * SEG)], osem)

        def pair(j, mem):
            base = pl.multiple_of(j * 2 * SEG, 2 * SEG)
            x0 = ax_s[pl.ds(base, SEG), :]
            x1 = ax_s[pl.ds(base + SEG, SEG), :]
            lhs1 = jnp.concatenate([x0, x1[0:8], mem], axis=0)
            o1, f1, left = seg(lhs1, jnp.concatenate([x0, mem], axis=0),
                               [(0, 32, 0, 0), (32, 8, 1, 0), (40, 8, 0, 32)], 0, None)
            mem1 = (o1[SEG:L] + f1[SEG - 8:SEG]).astype(BF16)
            lhs2 = jnp.concatenate([x1[16:32], mem1, x1[8:16]], axis=0)
            o2, f2, _ = seg(lhs2, jnp.concatenate([x1, mem1], axis=0),
                            [(0, 16, 1, 16), (16, 8, 1, 32), (24, 8, 1, 8)], 1, left)
            f1 = jnp.concatenate([f2[L:L + 8], f1[0:SEG - 8]], axis=0)
            stage_s[pl.ds(base, SEG), 0:DM] = (o1[0:SEG] + f1).astype(BF16)
            out2 = (o2 + f2[0:L]).astype(BF16)
            stage_s[pl.ds(base + SEG, SEG), 0:DM] = out2[0:SEG]
            out_copy(base).start()
            return out2[SEG:L]

        lax.fori_loop(0, N_PAIR_ITERS, pair, mem0_s[...])
        for j in range(N_PAIR_ITERS):
            out_copy(j * 2 * SEG).wait()

    pl.run_scoped(
        main,
        pltpu.VMEM((2, H, DM, DH), BF16),
        pltpu.VMEM((H // 2, 384, 2 * DM), BF16), pltpu.VMEM((H // 2, 384, 2 * DM), BF16),
        pltpu.VMEM((H // 2, DM, 128), BF16), pltpu.VMEM((H // 2, 128, DM), BF16),
        pltpu.VMEM((S, DM), BF16),
        pltpu.VMEM((S, DH), BF16), pltpu.VMEM((S, DH), BF16),
        pltpu.VMEM((S, 2 * DM), BF16), pltpu.VMEM((2, DM, 128), F32),
        pltpu.VMEM((H * L, 512), BF16), pltpu.VMEM((H * L, 512), BF16),
        pltpu.VMEM((H * L, 512), BF16), pltpu.VMEM((H * L, 512), BF16),
        pltpu.VMEM((H * L, 128), BF16), pltpu.VMEM((H * L, 128), BF16),
    )


@functools.partial(jax.jit, static_argnames=("A_seg_len",))
def pallas_concat_heads__memory_aug_recurrent_mem_tr__compressed_kv_cla__prompt_kernel(
    A_x: jax.Array,
    A_mem0: jax.Array,
    A_Wq: jax.Array,
    A_Wk: jax.Array,
    A_Wv: jax.Array,
    A_Wo: jax.Array,
    A_seg_len: int,
    B_x: jax.Array,
    B_c_kv: jax.Array,
    B_w_q: jax.Array,
    B_w_uk: jax.Array,
    B_w_uv: jax.Array,
    B_w_o: jax.Array,
):
    assert A_seg_len == SEG
    assert A_x.shape == (1, S, DM) and A_mem0.shape == (1, MEM, DM)
    assert A_Wq.shape == (DM, H, DH) and A_Wo.shape == (H, DH, DM)
    assert B_x.shape == (1, S, DM) and B_c_kv.shape == (1, S, DC)
    assert B_w_q.shape == (DM, H, DH) and B_w_uk.shape == (DC, H, DH)
    assert B_w_o.shape == (H, DH, DM)

    axt = jnp.swapaxes(A_x, 1, 2).reshape(DM, S)
    bxt = jnp.swapaxes(B_x, 1, 2).reshape(DM, S)
    awot = jnp.swapaxes(A_Wo, 1, 2)
    bwot = jnp.swapaxes(B_w_o, 1, 2)

    any_spec = pl.BlockSpec(memory_space=pl.ANY)
    out = pl.pallas_call(
        _kernel,
        out_shape=jax.ShapeDtypeStruct((S, 2 * DM), BF16),
        in_specs=[any_spec] * 12,
        out_specs=any_spec,
        scratch_shapes=[
            pltpu.VMEM((2 * H, DC, DH), BF16),
            pltpu.VMEM((S, DC), BF16),
            pltpu.VMEM((H, DM, DH), BF16),
            pltpu.VMEM((H, S, DH), BF16),
            pltpu.VMEM((3, DM + 128, H, DH), BF16),
            pltpu.VMEM((H, DM, DH), BF16),
            pltpu.VMEM((H, DM + 64, DH), BF16),
            pltpu.VMEM((S // 128 + 1, DM, 128), BF16),
            pltpu.VMEM((MEM, DM), BF16),
            pltpu.SemaphoreType.DMA((36,)),
            pltpu.SemaphoreType.DMA,
        ],
        compiler_params=pltpu.CompilerParams(vmem_limit_bytes=120 * 1024 * 1024),
    )(axt, A_mem0.reshape(MEM, DM), A_Wq, A_Wk, A_Wv, awot,
      bxt, B_c_kv.reshape(S, DC), B_w_q, B_w_uk, B_w_uv, bwot)
    return out.reshape(1, S, 2 * DM)
```

```python
import functools

import jax
import jax.numpy as jnp
from jax import lax
import jax.experimental.pallas as pl
import jax.experimental.pallas.tpu as pltpu

F32 = jnp.float32
BF16 = jnp.bfloat16
NT = (((1,), (1,)), ((), ()))
TN = (((0,), (0,)), ((), ()))
NEG = -1000000000.0

S = 2048
DM = 448
H = 16
DH = 256
HD = H * DH
DC = 1024
MEM = 8
SEG = 32
L = SEG + MEM
NPAIR = S // (2 * SEG)

BQ = 256
HB = BQ // 2
NQ = S // BQ
PB = 512
QB = 128
KB = 128
N_OPROJ_ITERS = S // 128
N_HEAD_ITERS = H
N_PAIR_ITERS = NPAIR
TAILPOS = 4
TAILPOS2 = 2
PVS = (0,)
QDEF = 8
OU = 2
WU = 1
GU = 2
B1U = 1
B2U = 1
AVPOS = (5, 7, 9, 11)
GRC = 2
GTAIL = 2
GTAIL2 = 1
ORDER = 'U T01 st T234567 x1 sc Z01 sm Z2 ut x2 Z34 x3 Z567 F PV'


def _dot(a, b):
    return jnp.dot(a, b, preferred_element_type=F32)


def _dot_nt(a, b):
    return lax.dot_general(a, b, NT, preferred_element_type=F32)


def _recip(l):
    r = pl.reciprocal(l, approx=True)
    return r * (2.0 - l * r)


def _kernel(axt_hbm, mem0_hbm, awq_hbm, awk_hbm, awv_hbm, awot_hbm,
            bxt_hbm, ckv_hbm, bwq_hbm, bwk_hbm, bwv_hbm, bwot_hbm,
            out_hbm,
            wkv_s, ckv_s, bwot_s, q_s, rawa_s, awot_s, awv_s, axt_s, mem0_s, bx_s, wq_s,
            sems, osem):
    scale = DH ** -0.5

    def cp(src, dst, i):
        return pltpu.make_async_copy(src, dst, sems.at[i])

    cp_ckv = cp(ckv_hbm, ckv_s, 6)
    cp_bwot = cp(bwot_hbm, bwot_s, 7)
    cp_awot = cp(awot_hbm, awot_s, 8)
    cp_axt = [cp(axt_hbm.at[:, pl.ds(j * 128, 128)], axt_s.at[j], 9)
              for j in range(S // 128)]
    cp_aw = [cp(w, rawa_s.at[t, pl.ds(0, DM)], 10 + t)
             for t, w in enumerate((awq_hbm, awk_hbm))]

    def cp_awv(i):
        lo = min if isinstance(i, int) else jnp.minimum
        return cp(awv_hbm.at[pl.ds(lo(i, DM // 64 - 1) * 64, 64)],
                  rawa_s.at[2, pl.ds(i * 64, 64)], 18 + i)

    cp_mem0 = cp(mem0_hbm, mem0_s, 13)

    def qproj(h, hw, r):
        rows = slice(r * QB, (r + 1) * QB)
        q_s[h, rows, :] = (_dot(bx_s[rows, :], wq_s[hw]) * scale).astype(BF16)

    def prologue(bxt_s, rawq_s, rawkv_s):
        cp_bxt = [cp(bxt_hbm.at[:, pl.ds(j * 128, 128)], bxt_s.at[j], 0 if j < 4 else 1)
                  for j in range(S // 128)]
        RQ = DM // 4
        cp_bwq_lo = [cp(bwq_hbm.at[pl.ds(c * RQ, RQ), pl.ds(0, 8), :],
                        rawq_s.at[0, pl.ds(c * RQ, RQ)], 14 + c) for c in range(4)]
        cp_bwq_hi = cp(bwq_hbm.at[:, pl.ds(8, 8), :], rawq_s.at[1], 3)

        def cp_kv(i):
            src = bwk_hbm if i < 4 else bwv_hbm
            return cp(src.at[pl.ds(min(i % 4 + i // 8 * 3, 3) * 256, 256)],
                      rawkv_s.at[pl.ds(i * 256, 256)], 27 + i)

        def wait_kv(i):
            dst = rawkv_s.at[pl.ds(i * 256, 256)]
            cp(dst, dst, 27 + i).wait()

        for c in (cp_bxt[:4] + cp_bwq_lo + cp_bxt[4:]
                  + [cp_bwq_hi] + [cp_awv(i) for i in range(9)]
                  + [cp_kv(i) for i in range(9)]
                  + [cp_ckv, cp_bwot, cp_awot] + cp_axt + cp_aw + [cp_mem0]):
            c.start()

        def relayout(src, dst, h0, r0, n):
            w = jnp.swapaxes(src[pl.ds(r0, n)], 0, 1)
            for h in range(w.shape[0]):
                dst[h0 + h, pl.ds(r0, n), :] = w[h]

        def xpose(j):
            r0 = j * 128 if isinstance(j, int) else pl.multiple_of(j * 128, 128)
            bx_s[pl.ds(r0, 128), :] = bxt_s[j].T

        def blk(h0, nh, r_lo, r_hi, side, post=None, unroll=1):
            def body(i, c):
                h = h0 + i
                for r in range(r_lo, r_hi):
                    if r != QDEF:
                        qproj(h, h, r)
                    side(i, r - r_lo)
                if post is not None:
                    post(i)
                return c
            lax.fori_loop(0, nh, body, 0, unroll=unroll)

        def side_xpose(i, r):
            if r < 3:
                xpose(4 + i * 3 + r)

        def side_wq(i, r):
            if r < 4:
                r0 = jnp.minimum(i, DM // 64 - 1) * 64 + r * 16
                relayout(rawq_s.at[1], wq_s, 8, pl.multiple_of(r0, 16), 16)
            if r in AVPOS:
                r0 = i * 64 + AVPOS.index(r) * 16
                relayout(rawa_s.at[2], awv_s, 0, pl.multiple_of(r0, 16), 16)

        def side_kv(i, r):
            w = jnp.swapaxes(rawkv_s[pl.ds(pl.multiple_of(i * 256 + r * 16, 16), 16)], 0, 1)
            r0 = pl.multiple_of((i % 4) * 256 + r * 16, 16)
            for h in range(H):
                wkv_s[(i // 4) * H + h, pl.ds(r0, 16), :] = w[h]

        for c in cp_bxt[:4]:
            c.wait()
        for j in range(4):
            xpose(j)
        for c in range(4):
            cp_bwq_lo[c].wait()
            relayout(rawq_s.at[0], wq_s, 0, c * RQ, RQ)
        blk(0, 4, 0, 4, lambda i, r: None, unroll=B1U)
        for c in cp_bxt[4:]:
            c.wait()
        blk(4, 4, 0, 4, side_xpose, unroll=B2U)
        qproj(0, 0, QDEF)
        cp_bwq_hi.wait()
        cp_awv(0).wait()
        blk(0, 8, 4, 16, side_wq, lambda i: cp_awv(i + 1).wait())
        wait_kv(0)
        blk(8, 8, 0, 16, side_kv, lambda i: wait_kv(i + 1))

    pl.run_scoped(
        prologue,
        pltpu.VMEM((S // 128, DM, 128), BF16),
        pltpu.VMEM((2, DM, 8, DH), BF16),
        pltpu.VMEM((2 * DC + 256, H, DH), BF16),
    )

    def main(wqk_s, wz_s, wg_s, wu_s, wt_s, ax_s, k_s, v_s, stage_s, ot_s,
             ts0, ts1, zs0, zs1, us0, us1):
        cp_ckv.wait()

        tri = (lax.broadcasted_iota(jnp.int32, (HB, HB), 1)
               <= lax.broadcasted_iota(jnp.int32, (HB, HB), 0))
        tri2 = (lax.broadcasted_iota(jnp.int32, (BQ, HB), 1)
                <= lax.broadcasted_iota(jnp.int32, (BQ, HB), 0))

        def kvproj(dst, h, pb, lo, hi):
            for r0 in range(lo, hi, pb):
                dst[r0:r0 + pb, :] = _dot(ckv_s[r0:r0 + pb, :], wkv_s[h]).astype(BF16)

        def qk(h, i):
            d0 = i * BQ
            q = q_s[h, d0:d0 + BQ, :]
            so = _dot_nt(q, k_s[0:d0, :]) if i > 0 else None
            s1 = _dot_nt(q, k_s[d0:d0 + HB, :])
            s2 = _dot_nt(q[HB:], k_s[d0 + HB:d0 + BQ, :])
            return so, s1, s2

        def soft_pv_out(h, i, ss):
            so, s1, s2 = ss
            d0 = i * BQ
            s1 = jnp.where(tri2, s1, NEG)
            s2 = jnp.where(tri, s2, NEG)
            m = jnp.max(s1, axis=1, keepdims=True)
            if so is not None:
                m = jnp.maximum(m, jnp.max(so, axis=1, keepdims=True))
            mb = jnp.maximum(m[HB:], jnp.max(s2, axis=1, keepdims=True))
            m = jnp.concatenate([m[:HB], mb], axis=0)
            p1 = jnp.exp(s1 - m)
            p2 = jnp.exp(s2 - mb)
            l = jnp.sum(p1, axis=1, keepdims=True)
            acc = _dot(p1.astype(BF16), v_s[d0:d0 + HB, :])
            if so is not None:
                po = jnp.exp(so - m)
                l = l + jnp.sum(po, axis=1, keepdims=True)
                acc = acc + _dot(po.astype(BF16), v_s[0:d0, :])
            l2 = l[HB:] + jnp.sum(p2, axis=1, keepdims=True)
            acc2 = acc[HB:] + _dot(p2.astype(BF16), v_s[d0 + HB:d0 + BQ, :])
            ctx = jnp.concatenate(
                [acc[:HB] * _recip(l[:HB]), acc2 * _recip(l2)], axis=0).astype(BF16)
            q_s[h, d0:d0 + BQ, :] = ctx

        def head(h, c):
            kvproj(k_s, h, KB, 0, S)
            order = list(range(NQ - 1, -1, -1))
            ss = qk(h, order[0])
            kvproj(v_s, H + h, PB, 0, S)
            for n, i in enumerate(order):
                nxt = qk(h, order[n + 1]) if n + 1 < NQ else None
                if n == NQ - 2:
                    qproj(h + 1, jnp.minimum(h + 1, H - 1), QDEF)
                soft_pv_out(h, i, ss)
                ss = nxt
            return c

        lax.fori_loop(0, N_HEAD_ITERS, head, 0)

        cp_bwot.wait()
        cp_awot.wait()
        for c in cp_axt + cp_aw + [cp_mem0]:
            c.wait()
        ot_s[0] = jnp.zeros((DM, 128), F32)

        def flush(r0):
            stage_s[pl.ds(r0, 128), DM:2 * DM] = ot_s[0].T.astype(BF16)

        def oproj(j, c):
            r0 = pl.multiple_of(j * 128, 128)
            pin_h = jnp.maximum(j, H)
            pin_o = jnp.where(j >= 0, 1, 0)
            acc = None
            for h in range(H):
                r = _dot_nt(bwot_s[h], q_s[h, pl.ds(r0, 128), :])
                acc = r if acc is None else acc + r
                if h == 0:
                    ot_s[pin_o, 0:8, :] = r[0:8]
                    flush(pl.multiple_of(jnp.maximum(j - 1, 0) * 128, 128))
                elif h == 14:
                    axt_s[pin_h, 0:16, :] = r[0:16].astype(BF16)
                    ax_s[pl.ds(r0, 128), :] = axt_s[j].T
            ot_s[0] = acc
            return c

        lax.fori_loop(0, N_OPROJ_ITERS, oproj, 0, unroll=OU)
        flush(S - 128)

        RC = 384 // 4

        def tails(a, b, mul):
            t = [_dot_nt(b[u], a[u]) for u in range(2)]
            return (jnp.concatenate(t, axis=0) * mul).astype(BF16).T

        def wzprep(i, c):
            for n in range(8):
                if n == TAILPOS:
                    wz_s[i, :, 384:512] = tails(
                        [awv_s[2 * i + u, 0:384, :] for u in range(2)],
                        [awot_s[2 * i + u, 384:DM, :] for u in range(2)], 1.0)
                if n == TAILPOS2:
                    for u in range(2):
                        wt_s[i, u * 64:(u + 1) * 64, :] = _dot_nt(
                            awv_s[2 * i + u, 384:DM, :], awot_s[2 * i + u]).astype(BF16)
                rc, u = divmod(n, 2)
                rows = slice(rc * RC, (rc + 1) * RC)
                w = _dot_nt(awv_s[2 * i + u, rows, :], awot_s[2 * i + u, 0:384, :])
                wz_s[i, rows, u * 512:u * 512 + 384] = w.astype(BF16)
                if n < 7:
                    piece = i * 7 + n
                    t = jnp.where(piece >= DM // 16, 1, 0)
                    rr = pl.multiple_of((piece - t * (DM // 16)) * 16, 16)
                    wr = jnp.swapaxes(rawa_s[t, pl.ds(rr, 16)], 0, 1)
                    for h in range(H):
                        wqk_s[t, h, pl.ds(rr, 16), :] = wr[h]
            return c

        lax.fori_loop(0, H // 2, wzprep, 0, unroll=WU)

        def gprep(i, c):
            for n in range(2 * GRC):
                if n == GTAIL:
                    wg_s[i, :, 384:512] = tails(
                        [wqk_s[0, 2 * i + u, 0:384, :] for u in range(2)],
                        [wqk_s[1, 2 * i + u, 384:DM, :] for u in range(2)], scale)
                if n == GTAIL2:
                    wu_s[i] = tails(
                        [wqk_s[1, 2 * i + u] for u in range(2)],
                        [wqk_s[0, 2 * i + u, 384:DM, :] for u in range(2)], scale)
                rc, u = divmod(n, 2)
                rows = slice(rc * (384 // GRC), (rc + 1) * (384 // GRC))
                w = _dot_nt(wqk_s[0, 2 * i + u, rows, :], wqk_s[1, 2 * i + u, 0:384, :])
                wg_s[i, rows, u * 512:u * 512 + 384] = (w * scale).astype(BF16)
            return c

        lax.fori_loop(0, H // 2, gprep, 0, unroll=GU)

        key = lax.broadcasted_iota(jnp.int32, (L, H * L), 0)
        qry = lax.broadcasted_iota(jnp.int32, (L, H * L), 1) % L
        mask = (qry >= SEG) | (key >= SEG) | (key <= qry)
        lane = lax.broadcasted_iota(jnp.int32, (8, 128), 1)
        lane_l = lax.broadcasted_iota(jnp.int32, (L, 128), 1)
        NT_ = H * L // 128
        tile_heads = [[h for h in range(H) if h * L < (t + 1) * 128 and (h + 1) * L > t * 128]
                      for t in range(NT_)]

        def proj(lhs, w_ref, dests, chunks):
            for i in chunks:
                r = _dot(lhs, w_ref[i])
                mid = r[:, 384:512]
                parts = [(r[:, 0:384].astype(BF16), mid.astype(BF16)),
                         (r[:, 512:896].astype(BF16), pltpu.roll(mid, 64, 1).astype(BF16))]
                for u in range(2):
                    for (a, n, d, b) in dests:
                        r0 = (2 * i + u) * L + b
                        d[r0:r0 + n, 0:384] = parts[u][0][a:a + n]
                        d[r0:r0 + n, 384:512] = parts[u][1][a:a + n]

        def proj_u(lhs, dests):
            for i in range(H // 2):
                r = _dot(lhs, wu_s[i])
                parts = [r.astype(BF16), pltpu.roll(r, 64, 1).astype(BF16)]
                for u in range(2):
                    for (a, n, d, b) in dests:
                        r0 = (2 * i + u) * L + b
                        d[r0:r0 + n, :] = parts[u][a:a + n]

        def head_t(p):
            rs = []
            for t in range(NT_):
                pt = p[:, t * 128:(t + 1) * 128]
                grp = [None] * 16
                for h in tile_heads[t]:
                    for kk in range(L // 8):
                        g = (h * (L // 8) + kk) % 16
                        piece = pt[kk * 8:(kk + 1) * 8]
                        grp[g] = piece if grp[g] is None else jnp.where(
                            lane >= h * L - t * 128, piece, grp[g])
                rs.append(jnp.concatenate(grp, axis=0).T)
            rr = jnp.concatenate(rs, axis=0)
            pcs = []
            for t in range(NT_):
                pc = None
                for h in tile_heads[t]:
                    piece = rr[h * L:(h + 1) * L]
                    pc = piece if pc is None else jnp.where(
                        lane_l >= h * L - t * 128, piece, pc)
                pcs.append(pc)
            return jnp.concatenate(pcs, axis=1)

        def seg(lhs, hs, sel, w, left):
            def dests(refs):
                return [(a, n, refs[v], b) for (a, n, v, b) in sel]
            ts, zs, us = (ts0, ts1), (zs0, zs1), (us0, us1)
            v = {}
            for step in ORDER.split():
                if step == "U":
                    proj_u(lhs, dests(us))
                elif step[0] == "T":
                    proj(lhs[:, 0:384], wg_s, dests(ts), [int(c) for c in step[1:]])
                elif step[0] == "Z":
                    proj(lhs[:, 0:384], wz_s, dests(zs), [int(c) for c in step[1:]])
                elif step == "st":
                    v["st"] = _dot_nt(hs[:, 384:DM], us[w][:, 0:64])
                elif step == "sc":
                    v["sc"] = _dot_nt(hs, ts[w][:, 0:DM])
                elif step == "x1":
                    v["st"] = head_t(v["st"])
                elif step == "sm":
                    sc = jnp.where(mask, v["sc"] + v["st"], NEG)
                    e = jnp.exp(sc - jnp.max(sc, axis=0, keepdims=True))
                    v["p"] = e * _recip(jnp.sum(e, axis=0, keepdims=True))
                elif step == "x2":
                    v["pf"] = head_t(v["p"])
                    v["pc"] = v["pf"].astype(BF16)
                elif step == "ut":
                    v["u"] = lax.dot_general(hs[:, 384:DM], v["p"].astype(BF16), TN,
                                             preferred_element_type=F32)
                elif step == "x3":
                    ut = jnp.concatenate([v["u"], v["u"]], axis=0)
                    rr = jnp.concatenate(
                        [ut[:, t * 128:(t + 1) * 128].T for t in range(NT_)], axis=0)
                    v["u"] = jnp.concatenate(
                        [jnp.where(lane_l < 64, rr[2 * i * L:(2 * i + 1) * L],
                                   rr[(2 * i + 1) * L:(2 * i + 2) * L])
                         for i in range(H // 2)], axis=1)
                elif step == "F":
                    rows = v["u"][8:L] if left is None else jnp.concatenate(
                        [v["u"], left], axis=0)
                    v["f"] = _dot(rows.astype(BF16), wt_s[...].reshape(H * 64, DM))
                elif step == "PV":
                    if w in PVS:
                        o1 = _dot(v["pf"][24:L].astype(BF16), zs[w][...])[:, 0:DM]
                        o2 = _dot(v["pf"][0:24].astype(BF16), zs[w][...])[:, 0:DM]
                        v["o"] = jnp.concatenate([o2, o1], axis=0)
                    else:
                        v["o"] = _dot(v["pc"], zs[w][...])[:, 0:DM]
            return v["o"], v["f"], v["u"][0:8]

        def out_copy(base):
            return pltpu.make_async_copy(
                stage_s.at[pl.ds(base, 2 * SEG)], out_hbm.at[pl.ds(base, 2 * SEG)], osem)

        def pair(j, mem):
            base = pl.multiple_of(j * 2 * SEG, 2 * SEG)
            x0 = ax_s[pl.ds(base, SEG), :]
            x1 = ax_s[pl.ds(base + SEG, SEG), :]
            lhs1 = jnp.concatenate([x0, x1[0:8], mem], axis=0)
            o1, f1, left = seg(lhs1, jnp.concatenate([x0, mem], axis=0),
                               [(0, 32, 0, 0), (32, 8, 1, 0), (40, 8, 0, 32)], 0, None)
            mem1 = (o1[SEG:L] + f1[SEG - 8:SEG]).astype(BF16)
            lhs2 = jnp.concatenate([x1[16:32], mem1, x1[8:16]], axis=0)
            o2, f2, _ = seg(lhs2, jnp.concatenate([x1, mem1], axis=0),
                            [(0, 16, 1, 16), (16, 8, 1, 32), (24, 8, 1, 8)], 1, left)
            f1 = jnp.concatenate([f2[L:L + 8], f1[0:SEG - 8]], axis=0)
            stage_s[pl.ds(base, SEG), 0:DM] = (o1[0:SEG] + f1).astype(BF16)
            out2 = (o2 + f2[0:L]).astype(BF16)
            stage_s[pl.ds(base + SEG, SEG), 0:DM] = out2[0:SEG]
            out_copy(base).start()
            return out2[SEG:L]

        lax.fori_loop(0, N_PAIR_ITERS, pair, mem0_s[...])
        for j in range(N_PAIR_ITERS):
            out_copy(j * 2 * SEG).wait()

    pl.run_scoped(
        main,
        pltpu.VMEM((2, H, DM, DH), BF16),
        pltpu.VMEM((H // 2, 384, 2 * DM), BF16), pltpu.VMEM((H // 2, 384, 2 * DM), BF16),
        pltpu.VMEM((H // 2, DM, 128), BF16), pltpu.VMEM((H // 2, 128, DM), BF16),
        pltpu.VMEM((S, DM), BF16),
        pltpu.VMEM((S, DH), BF16), pltpu.VMEM((S, DH), BF16),
        pltpu.VMEM((S, 2 * DM), BF16), pltpu.VMEM((2, DM, 128), F32),
        pltpu.VMEM((H * L, 512), BF16), pltpu.VMEM((H * L, 512), BF16),
        pltpu.VMEM((H * L, 512), BF16), pltpu.VMEM((H * L, 512), BF16),
        pltpu.VMEM((H * L, 128), BF16), pltpu.VMEM((H * L, 128), BF16),
    )


@functools.partial(jax.jit, static_argnames=("A_seg_len",))
def pallas_concat_heads__memory_aug_recurrent_mem_tr__compressed_kv_cla__prompt_kernel(
    A_x: jax.Array,
    A_mem0: jax.Array,
    A_Wq: jax.Array,
    A_Wk: jax.Array,
    A_Wv: jax.Array,
    A_Wo: jax.Array,
    A_seg_len: int,
    B_x: jax.Array,
    B_c_kv: jax.Array,
    B_w_q: jax.Array,
    B_w_uk: jax.Array,
    B_w_uv: jax.Array,
    B_w_o: jax.Array,
):
    assert A_seg_len == SEG
    assert A_x.shape == (1, S, DM) and A_mem0.shape == (1, MEM, DM)
    assert A_Wq.shape == (DM, H, DH) and A_Wo.shape == (H, DH, DM)
    assert B_x.shape == (1, S, DM) and B_c_kv.shape == (1, S, DC)
    assert B_w_q.shape == (DM, H, DH) and B_w_uk.shape == (DC, H, DH)
    assert B_w_o.shape == (H, DH, DM)

    axt = jnp.swapaxes(A_x, 1, 2).reshape(DM, S)
    bxt = jnp.swapaxes(B_x, 1, 2).reshape(DM, S)
    awot = jnp.swapaxes(A_Wo, 1, 2)
    bwot = jnp.swapaxes(B_w_o, 1, 2)

    any_spec = pl.BlockSpec(memory_space=pl.ANY)
    out = pl.pallas_call(
        _kernel,
        out_shape=jax.ShapeDtypeStruct((S, 2 * DM), BF16),
        in_specs=[any_spec] * 12,
        out_specs=any_spec,
        scratch_shapes=[
            pltpu.VMEM((2 * H, DC, DH), BF16),
            pltpu.VMEM((S, DC), BF16),
            pltpu.VMEM((H, DM, DH), BF16),
            pltpu.VMEM((H + 1, S, DH), BF16),
            pltpu.VMEM((3, DM + 128, H, DH), BF16),
            pltpu.VMEM((H, DM, DH), BF16),
            pltpu.VMEM((H, DM + 64, DH), BF16),
            pltpu.VMEM((S // 128 + 1, DM, 128), BF16),
            pltpu.VMEM((MEM, DM), BF16),
            pltpu.VMEM((S, DM), BF16),
            pltpu.VMEM((H, DM, DH), BF16),
            pltpu.SemaphoreType.DMA((36,)),
            pltpu.SemaphoreType.DMA,
        ],
        compiler_params=pltpu.CompilerParams(vmem_limit_bytes=120 * 1024 * 1024),
    )(axt, A_mem0.reshape(MEM, DM), A_Wq, A_Wk, A_Wv, awot,
      bxt, B_c_kv.reshape(S, DC), B_w_q, B_w_uk, B_w_uv, bwot)
    return out.reshape(1, S, 2 * DM)
```

```python
import functools

import jax
import jax.numpy as jnp
from jax import lax
import jax.experimental.pallas as pl
import jax.experimental.pallas.tpu as pltpu

F32 = jnp.float32
BF16 = jnp.bfloat16
NT = (((1,), (1,)), ((), ()))
TN = (((0,), (0,)), ((), ()))
NEG = -1000000000.0

S = 2048
DM = 448
H = 16
DH = 256
HD = H * DH
DC = 1024
MEM = 8
SEG = 32
L = SEG + MEM
NPAIR = S // (2 * SEG)

BQ = 256
HB = BQ // 2
NQ = S // BQ
PB = 512
QB = 128
KB = 128
N_OPROJ_ITERS = S // 128
N_HEAD_ITERS = H
N_PAIR_ITERS = NPAIR
TAILPOS = 4
TAILPOS2 = 2
PVS = (0,)
QDEF = 8
OU = 2
WU = 1
GU = 2
B1U = 1
B2U = 1
AVPOS = (5, 7, 9, 11)
GRC = 2
GTAIL = 2
GTAIL2 = 1
ORDER = 'U T01 st T234567 x1 sc Z01 sm Z2 ut x2 Z34 x3 Z567 F PV'


def _dot(a, b):
    return jnp.dot(a, b, preferred_element_type=F32)


def _dot_nt(a, b):
    return lax.dot_general(a, b, NT, preferred_element_type=F32)


def _recip(l):
    r = pl.reciprocal(l, approx=True)
    return r * (2.0 - l * r)


def _kernel(axt_hbm, mem0_hbm, awq_hbm, awk_hbm, awv_hbm, awot_hbm,
            bxt_hbm, ckv_hbm, bwq_hbm, bwk_hbm, bwv_hbm, bwot_hbm,
            out_hbm,
            wkv_s, ckv_s, bwot_s, q_s, rawa_s, awot_s, awv_s, axt_s, mem0_s, bx_s, wq_s,
            sems, osem):
    scale = DH ** -0.5 * 1.4426950408889634

    def cp(src, dst, i):
        return pltpu.make_async_copy(src, dst, sems.at[i])

    cp_ckv = cp(ckv_hbm, ckv_s, 6)
    cp_bwot = cp(bwot_hbm, bwot_s, 7)
    cp_awot = cp(awot_hbm, awot_s, 8)
    cp_axt = [cp(axt_hbm.at[:, pl.ds(j * 128, 128)], axt_s.at[j], 9)
              for j in range(S // 128)]
    cp_aw = [cp(w, rawa_s.at[t, pl.ds(0, DM)], 10 + t)
             for t, w in enumerate((awq_hbm, awk_hbm))]

    def cp_awv(i):
        lo = min if isinstance(i, int) else jnp.minimum
        return cp(awv_hbm.at[pl.ds(lo(i, DM // 64 - 1) * 64, 64)],
                  rawa_s.at[2, pl.ds(i * 64, 64)], 18 + i)

    cp_mem0 = cp(mem0_hbm, mem0_s, 13)

    def qproj(h, hw, r):
        rows = slice(r * QB, (r + 1) * QB)
        q_s[h, rows, :] = (_dot(bx_s[rows, :], wq_s[hw]) * scale).astype(BF16)

    def prologue(bxt_s, rawq_s, rawkv_s):
        cp_bxt = [cp(bxt_hbm.at[:, pl.ds(j * 128, 128)], bxt_s.at[j], 0 if j < 4 else 1)
                  for j in range(S // 128)]
        RQ = DM // 4
        cp_bwq_lo = [cp(bwq_hbm.at[pl.ds(c * RQ, RQ), pl.ds(0, 8), :],
                        rawq_s.at[0, pl.ds(c * RQ, RQ)], 14 + c) for c in range(4)]
        cp_bwq_hi = cp(bwq_hbm.at[:, pl.ds(8, 8), :], rawq_s.at[1], 3)

        def cp_kv(i):
            src = bwk_hbm if i < 4 else bwv_hbm
            return cp(src.at[pl.ds(min(i % 4 + i // 8 * 3, 3) * 256, 256)],
                      rawkv_s.at[pl.ds(i * 256, 256)], 27 + i)

        def wait_kv(i):
            dst = rawkv_s.at[pl.ds(i * 256, 256)]
            cp(dst, dst, 27 + i).wait()

        for c in (cp_bxt[:4] + cp_bwq_lo + cp_bxt[4:]
                  + [cp_bwq_hi] + [cp_awv(i) for i in range(9)]
                  + [cp_kv(i) for i in range(9)]
                  + [cp_ckv, cp_bwot, cp_awot] + cp_axt + cp_aw + [cp_mem0]):
            c.start()

        def relayout(src, dst, h0, r0, n):
            w = jnp.swapaxes(src[pl.ds(r0, n)], 0, 1)
            for h in range(w.shape[0]):
                dst[h0 + h, pl.ds(r0, n), :] = w[h]

        def xpose(j):
            r0 = j * 128 if isinstance(j, int) else pl.multiple_of(j * 128, 128)
            bx_s[pl.ds(r0, 128), :] = bxt_s[j].T

        def blk(h0, nh, r_lo, r_hi, side, post=None, unroll=1):
            def body(i, c):
                h = h0 + i
                for r in range(r_lo, r_hi):
                    if r != QDEF:
                        qproj(h, h, r)
                    side(i, r - r_lo)
                if post is not None:
                    post(i)
                return c
            lax.fori_loop(0, nh, body, 0, unroll=unroll)

        def side_xpose(i, r):
            if r < 3:
                xpose(4 + i * 3 + r)

        def side_wq(i, r):
            if r < 4:
                r0 = jnp.minimum(i, DM // 64 - 1) * 64 + r * 16
                relayout(rawq_s.at[1], wq_s, 8, pl.multiple_of(r0, 16), 16)
            if r in AVPOS:
                r0 = i * 64 + AVPOS.index(r) * 16
                relayout(rawa_s.at[2], awv_s, 0, pl.multiple_of(r0, 16), 16)

        def side_kv(i, r):
            w = jnp.swapaxes(rawkv_s[pl.ds(pl.multiple_of(i * 256 + r * 16, 16), 16)], 0, 1)
            r0 = pl.multiple_of((i % 4) * 256 + r * 16, 16)
            for h in range(H):
                wkv_s[(i // 4) * H + h, pl.ds(r0, 16), :] = w[h]

        for c in cp_bxt[:4]:
            c.wait()
        for j in range(4):
            xpose(j)
        for c in range(4):
            cp_bwq_lo[c].wait()
            relayout(rawq_s.at[0], wq_s, 0, c * RQ, RQ)
        blk(0, 4, 0, 4, lambda i, r: None, unroll=B1U)
        for c in cp_bxt[4:]:
            c.wait()
        blk(4, 4, 0, 4, side_xpose, unroll=B2U)
        qproj(0, 0, QDEF)
        cp_bwq_hi.wait()
        cp_awv(0).wait()
        blk(0, 8, 4, 16, side_wq, lambda i: cp_awv(i + 1).wait())
        wait_kv(0)
        blk(8, 8, 0, 16, side_kv, lambda i: wait_kv(i + 1))

    pl.run_scoped(
        prologue,
        pltpu.VMEM((S // 128, DM, 128), BF16),
        pltpu.VMEM((2, DM, 8, DH), BF16),
        pltpu.VMEM((2 * DC + 256, H, DH), BF16),
    )

    def main(wqk_s, wz_s, wg_s, wu_s, wt_s, ax_s, k_s, v_s, stage_s, ot_s,
             ts0, ts1, zs0, zs1, us0, us1):
        cp_ckv.wait()

        tri = (lax.broadcasted_iota(jnp.int32, (HB, HB), 1)
               <= lax.broadcasted_iota(jnp.int32, (HB, HB), 0))
        tri2 = (lax.broadcasted_iota(jnp.int32, (BQ, HB), 1)
                <= lax.broadcasted_iota(jnp.int32, (BQ, HB), 0))

        def kvproj(dst, h, pb, lo, hi):
            for r0 in range(lo, hi, pb):
                dst[r0:r0 + pb, :] = _dot(ckv_s[r0:r0 + pb, :], wkv_s[h]).astype(BF16)

        def qk(h, i):
            d0 = i * BQ
            q = q_s[h, d0:d0 + BQ, :]
            so = _dot_nt(q, k_s[0:d0, :]) if i > 0 else None
            s1 = _dot_nt(q, k_s[d0:d0 + HB, :])
            s2 = _dot_nt(q[HB:], k_s[d0 + HB:d0 + BQ, :])
            return so, s1, s2

        def soft_pv_out(h, i, ss):
            so, s1, s2 = ss
            d0 = i * BQ
            s1 = jnp.where(tri2, s1, NEG)
            s2 = jnp.where(tri, s2, NEG)
            m = jnp.max(s1, axis=1, keepdims=True)
            if so is not None:
                m = jnp.maximum(m, jnp.max(so, axis=1, keepdims=True))
            mb = jnp.maximum(m[HB:], jnp.max(s2, axis=1, keepdims=True))
            m = jnp.concatenate([m[:HB], mb], axis=0)
            p1 = jnp.exp2(s1 - m)
            p2 = jnp.exp2(s2 - mb)
            l = jnp.sum(p1, axis=1, keepdims=True)
            acc = _dot(p1.astype(BF16), v_s[d0:d0 + HB, :])
            if so is not None:
                po = jnp.exp2(so - m)
                l = l + jnp.sum(po, axis=1, keepdims=True)
                acc = acc + _dot(po.astype(BF16), v_s[0:d0, :])
            l2 = l[HB:] + jnp.sum(p2, axis=1, keepdims=True)
            acc2 = acc[HB:] + _dot(p2.astype(BF16), v_s[d0 + HB:d0 + BQ, :])
            ctx = jnp.concatenate(
                [acc[:HB] * _recip(l[:HB]), acc2 * _recip(l2)], axis=0).astype(BF16)
            q_s[h, d0:d0 + BQ, :] = ctx

        def head(h, c):
            kvproj(k_s, h, KB, 0, S)
            order = list(range(NQ - 1, -1, -1))
            ss = qk(h, order[0])
            kvproj(v_s, H + h, PB, 0, S)
            for n, i in enumerate(order):
                nxt = qk(h, order[n + 1]) if n + 1 < NQ else None
                if n == NQ - 2:
                    qproj(h + 1, jnp.minimum(h + 1, H - 1), QDEF)
                soft_pv_out(h, i, ss)
                ss = nxt
            return c

        lax.fori_loop(0, N_HEAD_ITERS, head, 0)

        cp_bwot.wait()
        cp_awot.wait()
        for c in cp_axt + cp_aw + [cp_mem0]:
            c.wait()
        ot_s[0] = jnp.zeros((DM, 128), F32)

        def flush(r0):
            stage_s[pl.ds(r0, 128), DM:2 * DM] = ot_s[0].T.astype(BF16)

        def oproj(j, c):
            r0 = pl.multiple_of(j * 128, 128)
            pin_h = jnp.maximum(j, H)
            pin_o = jnp.where(j >= 0, 1, 0)
            acc = None
            for h in range(H):
                r = _dot_nt(bwot_s[h], q_s[h, pl.ds(r0, 128), :])
                acc = r if acc is None else acc + r
                if h == 0:
                    ot_s[pin_o, 0:8, :] = r[0:8]
                    flush(pl.multiple_of(jnp.maximum(j - 1, 0) * 128, 128))
                elif h == 14:
                    axt_s[pin_h, 0:16, :] = r[0:16].astype(BF16)
                    ax_s[pl.ds(r0, 128), :] = axt_s[j].T
            ot_s[0] = acc
            return c

        lax.fori_loop(0, N_OPROJ_ITERS, oproj, 0, unroll=OU)
        flush(S - 128)

        RC = 384 // 4

        def tails(a, b, mul):
            t = [_dot_nt(b[u], a[u]) for u in range(2)]
            return (jnp.concatenate(t, axis=0) * mul).astype(BF16).T

        def wzprep(i, c):
            for n in range(8):
                if n == TAILPOS:
                    wz_s[i, :, 384:512] = tails(
                        [awv_s[2 * i + u, 0:384, :] for u in range(2)],
                        [awot_s[2 * i + u, 384:DM, :] for u in range(2)], 1.0)
                if n == TAILPOS2:
                    for u in range(2):
                        wt_s[i, u * 64:(u + 1) * 64, :] = _dot_nt(
                            awv_s[2 * i + u, 384:DM, :], awot_s[2 * i + u]).astype(BF16)
                rc, u = divmod(n, 2)
                rows = slice(rc * RC, (rc + 1) * RC)
                w = _dot_nt(awv_s[2 * i + u, rows, :], awot_s[2 * i + u, 0:384, :])
                wz_s[i, rows, u * 512:u * 512 + 384] = w.astype(BF16)
                if n < 7:
                    piece = i * 7 + n
                    t = jnp.where(piece >= DM // 16, 1, 0)
                    rr = pl.multiple_of((piece - t * (DM // 16)) * 16, 16)
                    wr = jnp.swapaxes(rawa_s[t, pl.ds(rr, 16)], 0, 1)
                    for h in range(H):
                        wqk_s[t, h, pl.ds(rr, 16), :] = wr[h]
            return c

        lax.fori_loop(0, H // 2, wzprep, 0, unroll=WU)

        def gprep(i, c):
            for n in range(2 * GRC):
                if n == GTAIL:
                    wg_s[i, :, 384:512] = tails(
                        [wqk_s[0, 2 * i + u, 0:384, :] for u in range(2)],
                        [wqk_s[1, 2 * i + u, 384:DM, :] for u in range(2)], scale)
                if n == GTAIL2:
                    wu_s[i] = tails(
                        [wqk_s[1, 2 * i + u] for u in range(2)],
                        [wqk_s[0, 2 * i + u, 384:DM, :] for u in range(2)], scale)
                rc, u = divmod(n, 2)
                rows = slice(rc * (384 // GRC), (rc + 1) * (384 // GRC))
                w = _dot_nt(wqk_s[0, 2 * i + u, rows, :], wqk_s[1, 2 * i + u, 0:384, :])
                wg_s[i, rows, u * 512:u * 512 + 384] = (w * scale).astype(BF16)
            return c

        lax.fori_loop(0, H // 2, gprep, 0, unroll=GU)

        key = lax.broadcasted_iota(jnp.int32, (L, H * L), 0)
        qry = lax.broadcasted_iota(jnp.int32, (L, H * L), 1) % L
        mask = (qry >= SEG) | (key >= SEG) | (key <= qry)
        lane = lax.broadcasted_iota(jnp.int32, (8, 128), 1)
        lane_l = lax.broadcasted_iota(jnp.int32, (L, 128), 1)
        NT_ = H * L // 128
        tile_heads = [[h for h in range(H) if h * L < (t + 1) * 128 and (h + 1) * L > t * 128]
                      for t in range(NT_)]

        def proj(lhs, w_ref, dests, chunks):
            for i in chunks:
                r = _dot(lhs, w_ref[i])
                mid = r[:, 384:512]
                parts = [(r[:, 0:384].astype(BF16), mid.astype(BF16)),
                         (r[:, 512:896].astype(BF16), pltpu.roll(mid, 64, 1).astype(BF16))]
                for u in range(2):
                    for (a, n, d, b) in dests:
                        r0 = (2 * i + u) * L + b
                        d[r0:r0 + n, 0:384] = parts[u][0][a:a + n]
                        d[r0:r0 + n, 384:512] = parts[u][1][a:a + n]

        def proj_u(lhs, dests):
            for i in range(H // 2):
                r = _dot(lhs, wu_s[i])
                parts = [r.astype(BF16), pltpu.roll(r, 64, 1).astype(BF16)]
                for u in range(2):
                    for (a, n, d, b) in dests:
                        r0 = (2 * i + u) * L + b
                        d[r0:r0 + n, :] = parts[u][a:a + n]

        def head_t(p):
            rs = []
            for t in range(NT_):
                pt = p[:, t * 128:(t + 1) * 128]
                grp = [None] * 16
                for h in tile_heads[t]:
                    for kk in range(L // 8):
                        g = (h * (L // 8) + kk) % 16
                        piece = pt[kk * 8:(kk + 1) * 8]
                        grp[g] = piece if grp[g] is None else jnp.where(
                            lane >= h * L - t * 128, piece, grp[g])
                rs.append(jnp.concatenate(grp, axis=0).T)
            rr = jnp.concatenate(rs, axis=0)
            pcs = []
            for t in range(NT_):
                pc = None
                for h in tile_heads[t]:
                    piece = rr[h * L:(h + 1) * L]
                    pc = piece if pc is None else jnp.where(
                        lane_l >= h * L - t * 128, piece, pc)
                pcs.append(pc)
            return jnp.concatenate(pcs, axis=1)

        def seg(lhs, hs, sel, w, left):
            def dests(refs):
                return [(a, n, refs[v], b) for (a, n, v, b) in sel]
            ts, zs, us = (ts0, ts1), (zs0, zs1), (us0, us1)
            v = {}
            for step in ORDER.split():
                if step == "U":
                    proj_u(lhs, dests(us))
                elif step[0] == "T":
                    proj(lhs[:, 0:384], wg_s, dests(ts), [int(c) for c in step[1:]])
                elif step[0] == "Z":
                    proj(lhs[:, 0:384], wz_s, dests(zs), [int(c) for c in step[1:]])
                elif step == "st":
                    v["st"] = _dot_nt(hs[:, 384:DM], us[w][:, 0:64])
                elif step == "sc":
                    v["sc"] = _dot_nt(hs, ts[w][:, 0:DM])
                elif step == "x1":
                    v["st"] = head_t(v["st"])
                elif step == "sm":
                    sc = jnp.where(mask, v["sc"] + v["st"], NEG)
                    e = jnp.exp2(sc - jnp.max(sc, axis=0, keepdims=True))
                    v["p"] = e * _recip(jnp.sum(e, axis=0, keepdims=True))
                elif step == "x2":
                    v["pf"] = head_t(v["p"])
                    v["pc"] = v["pf"].astype(BF16)
                elif step == "ut":
                    v["u"] = lax.dot_general(hs[:, 384:DM], v["p"].astype(BF16), TN,
                                             preferred_element_type=F32)
                elif step == "x3":
                    ut = jnp.concatenate([v["u"], v["u"]], axis=0)
                    rr = jnp.concatenate(
                        [ut[:, t * 128:(t + 1) * 128].T for t in range(NT_)], axis=0)
                    v["u"] = jnp.concatenate(
                        [jnp.where(lane_l < 64, rr[2 * i * L:(2 * i + 1) * L],
                                   rr[(2 * i + 1) * L:(2 * i + 2) * L])
                         for i in range(H // 2)], axis=1)
                elif step == "F":
                    rows = v["u"][8:L] if left is None else jnp.concatenate(
                        [v["u"], left], axis=0)
                    v["f"] = _dot(rows.astype(BF16), wt_s[...].reshape(H * 64, DM))
                elif step == "PV":
                    if w in PVS:
                        o1 = _dot(v["pf"][24:L].astype(BF16), zs[w][...])[:, 0:DM]
                        o2 = _dot(v["pf"][0:24].astype(BF16), zs[w][...])[:, 0:DM]
                        v["o"] = jnp.concatenate([o2, o1], axis=0)
                    else:
                        v["o"] = _dot(v["pc"], zs[w][...])[:, 0:DM]
            return v["o"], v["f"], v["u"][0:8]

        def out_copy(base):
            return pltpu.make_async_copy(
                stage_s.at[pl.ds(base, 2 * SEG)], out_hbm.at[pl.ds(base, 2 * SEG)], osem)

        def pair(j, mem):
            base = pl.multiple_of(j * 2 * SEG, 2 * SEG)
            x0 = ax_s[pl.ds(base, SEG), :]
            x1 = ax_s[pl.ds(base + SEG, SEG), :]
            lhs1 = jnp.concatenate([x0, x1[0:8], mem], axis=0)
            o1, f1, left = seg(lhs1, jnp.concatenate([x0, mem], axis=0),
                               [(0, 32, 0, 0), (32, 8, 1, 0), (40, 8, 0, 32)], 0, None)
            mem1 = (o1[SEG:L] + f1[SEG - 8:SEG]).astype(BF16)
            lhs2 = jnp.concatenate([x1[16:32], mem1, x1[8:16]], axis=0)
            o2, f2, _ = seg(lhs2, jnp.concatenate([x1, mem1], axis=0),
                            [(0, 16, 1, 16), (16, 8, 1, 32), (24, 8, 1, 8)], 1, left)
            f1 = jnp.concatenate([f2[L:L + 8], f1[0:SEG - 8]], axis=0)
            stage_s[pl.ds(base, SEG), 0:DM] = (o1[0:SEG] + f1).astype(BF16)
            out2 = (o2 + f2[0:L]).astype(BF16)
            stage_s[pl.ds(base + SEG, SEG), 0:DM] = out2[0:SEG]
            out_copy(base).start()
            return out2[SEG:L]

        lax.fori_loop(0, N_PAIR_ITERS, pair, mem0_s[...])
        for j in range(N_PAIR_ITERS):
            out_copy(j * 2 * SEG).wait()

    pl.run_scoped(
        main,
        pltpu.VMEM((2, H, DM, DH), BF16),
        pltpu.VMEM((H // 2, 384, 2 * DM), BF16), pltpu.VMEM((H // 2, 384, 2 * DM), BF16),
        pltpu.VMEM((H // 2, DM, 128), BF16), pltpu.VMEM((H // 2, 128, DM), BF16),
        pltpu.VMEM((S, DM), BF16),
        pltpu.VMEM((S, DH), BF16), pltpu.VMEM((S, DH), BF16),
        pltpu.VMEM((S, 2 * DM), BF16), pltpu.VMEM((2, DM, 128), F32),
        pltpu.VMEM((H * L, 512), BF16), pltpu.VMEM((H * L, 512), BF16),
        pltpu.VMEM((H * L, 512), BF16), pltpu.VMEM((H * L, 512), BF16),
        pltpu.VMEM((H * L, 128), BF16), pltpu.VMEM((H * L, 128), BF16),
    )


@functools.partial(jax.jit, static_argnames=("A_seg_len",))
def pallas_concat_heads__memory_aug_recurrent_mem_tr__compressed_kv_cla__prompt_kernel(
    A_x: jax.Array,
    A_mem0: jax.Array,
    A_Wq: jax.Array,
    A_Wk: jax.Array,
    A_Wv: jax.Array,
    A_Wo: jax.Array,
    A_seg_len: int,
    B_x: jax.Array,
    B_c_kv: jax.Array,
    B_w_q: jax.Array,
    B_w_uk: jax.Array,
    B_w_uv: jax.Array,
    B_w_o: jax.Array,
):
    assert A_seg_len == SEG
    assert A_x.shape == (1, S, DM) and A_mem0.shape == (1, MEM, DM)
    assert A_Wq.shape == (DM, H, DH) and A_Wo.shape == (H, DH, DM)
    assert B_x.shape == (1, S, DM) and B_c_kv.shape == (1, S, DC)
    assert B_w_q.shape == (DM, H, DH) and B_w_uk.shape == (DC, H, DH)
    assert B_w_o.shape == (H, DH, DM)

    axt = jnp.swapaxes(A_x, 1, 2).reshape(DM, S)
    bxt = jnp.swapaxes(B_x, 1, 2).reshape(DM, S)
    awot = jnp.swapaxes(A_Wo, 1, 2)
    bwot = jnp.swapaxes(B_w_o, 1, 2)

    any_spec = pl.BlockSpec(memory_space=pl.ANY)
    out = pl.pallas_call(
        _kernel,
        out_shape=jax.ShapeDtypeStruct((S, 2 * DM), BF16),
        in_specs=[any_spec] * 12,
        out_specs=any_spec,
        scratch_shapes=[
            pltpu.VMEM((2 * H, DC, DH), BF16),
            pltpu.VMEM((S, DC), BF16),
            pltpu.VMEM((H, DM, DH), BF16),
            pltpu.VMEM((H + 1, S, DH), BF16),
            pltpu.VMEM((3, DM + 128, H, DH), BF16),
            pltpu.VMEM((H, DM, DH), BF16),
            pltpu.VMEM((H, DM + 64, DH), BF16),
            pltpu.VMEM((S // 128 + 1, DM, 128), BF16),
            pltpu.VMEM((MEM, DM), BF16),
            pltpu.VMEM((S, DM), BF16),
            pltpu.VMEM((H, DM, DH), BF16),
            pltpu.SemaphoreType.DMA((36,)),
            pltpu.SemaphoreType.DMA,
        ],
        compiler_params=pltpu.CompilerParams(vmem_limit_bytes=120 * 1024 * 1024),
    )(axt, A_mem0.reshape(MEM, DM), A_Wq, A_Wk, A_Wv, awot,
      bxt, B_c_kv.reshape(S, DC), B_w_q, B_w_uk, B_w_uv, bwot)
    return out.reshape(1, S, 2 * DM)
```

```python
import functools

import jax
import jax.numpy as jnp
from jax import lax
import jax.experimental.pallas as pl
import jax.experimental.pallas.tpu as pltpu

F32 = jnp.float32
BF16 = jnp.bfloat16
NT = (((1,), (1,)), ((), ()))
TN = (((0,), (0,)), ((), ()))
NEG = -1000000000.0

S = 2048
DM = 448
H = 16
DH = 256
HD = H * DH
DC = 1024
MEM = 8
SEG = 32
L = SEG + MEM
NPAIR = S // (2 * SEG)

BQ = 256
HB = BQ // 2
NQ = S // BQ
PB = 512
QB = 128
KB = 128
N_OPROJ_ITERS = S // 128
N_HEAD_ITERS = H
N_PAIR_ITERS = NPAIR
TAILPOS = 4
TAILPOS2 = 2
PVS = (0,)
QDEF = 8
OU = 2
WU = 1
GU = 2
NRQ = 4
XPOS = (5, 6, 7)
WQPOS = (8, 9, 10, 11)
AVPOS = (0, 1, 2, 3)
GRC = 2
GTAIL = 2
GTAIL2 = 1
ORDER = 'U T01 st T234567 x1 sc Z01 sm Z2 ut x2 Z34 x3 Z567 F PV'


def _dot(a, b):
    return jnp.dot(a, b, preferred_element_type=F32)


def _dot_nt(a, b):
    return lax.dot_general(a, b, NT, preferred_element_type=F32)


def _recip(l):
    r = pl.reciprocal(l, approx=True)
    return r * (2.0 - l * r)


def _kernel(axt_hbm, mem0_hbm, awq_hbm, awk_hbm, awv_hbm, awot_hbm,
            bxt_hbm, ckv_hbm, bwq_hbm, bwk_hbm, bwv_hbm, bwot_hbm,
            out_hbm,
            wkv_s, ckv_s, bwot_s, q_s, rawa_s, awot_s, awv_s, axt_s, mem0_s, bx_s, wq_s,
            sems, osem):
    scale = DH ** -0.5 * 1.4426950408889634

    def cp(src, dst, i):
        return pltpu.make_async_copy(src, dst, sems.at[i])

    cp_ckv = cp(ckv_hbm, ckv_s, 6)
    cp_bwot = cp(bwot_hbm, bwot_s, 7)
    cp_awot = cp(awot_hbm, awot_s, 8)
    cp_axt = [cp(axt_hbm.at[:, pl.ds(j * 128, 128)], axt_s.at[j], 9)
              for j in range(S // 128)]
    cp_aw = [cp(w, rawa_s.at[t, pl.ds(0, DM)], 10 + t)
             for t, w in enumerate((awq_hbm, awk_hbm))]

    def cp_awv(i):
        lo = min if isinstance(i, int) else jnp.minimum
        return cp(awv_hbm.at[pl.ds(lo(i, DM // 64 - 1) * 64, 64)],
                  rawa_s.at[2, pl.ds(i * 64, 64)], 18 + i)

    cp_mem0 = cp(mem0_hbm, mem0_s, 13)

    def qproj(h, hw, r):
        rows = slice(r * QB, (r + 1) * QB)
        q_s[h, rows, :] = (_dot(bx_s[rows, :], wq_s[hw]) * scale).astype(BF16)

    def prologue(bxt_s, rawq_s, rawkv_s):
        cp_bxt = [cp(bxt_hbm.at[:, pl.ds(j * 128, 128)], bxt_s.at[j], 0 if j < 4 else 1)
                  for j in range(S // 128)]
        RQ = DM // NRQ
        cp_bwq_lo = [[cp(bwq_hbm.at[pl.ds(c * RQ, RQ), pl.ds(0, 8), pl.ds(e * 128, 128)],
                         rawq_s.at[0, pl.ds(c * RQ, RQ), :, pl.ds(e * 128, 128)],
                         36 + e * NRQ + c) for c in range(NRQ)] for e in range(2)]
        cp_bwq_hi = cp(bwq_hbm.at[:, pl.ds(8, 8), :], rawq_s.at[1], 3)

        def cp_kv(i):
            src = bwk_hbm if i < 4 else bwv_hbm
            return cp(src.at[pl.ds(min(i % 4 + i // 8 * 3, 3) * 256, 256)],
                      rawkv_s.at[pl.ds(i * 256, 256)], 27 + i)

        def wait_kv(i):
            dst = rawkv_s.at[pl.ds(i * 256, 256)]
            cp(dst, dst, 27 + i).wait()

        for c in (cp_bxt[:4] + cp_bwq_lo[0] + cp_bwq_lo[1] + cp_bxt[4:]
                  + [cp_bwq_hi] + [cp_awv(i) for i in range(9)]
                  + [cp_kv(i) for i in range(9)]
                  + [cp_ckv, cp_bwot, cp_awot] + cp_axt + cp_aw + [cp_mem0]):
            c.start()

        def relayout(src, dst, h0, r0, n):
            w = jnp.swapaxes(src[pl.ds(r0, n)], 0, 1)
            for h in range(w.shape[0]):
                dst[h0 + h, pl.ds(r0, n), :] = w[h]

        def xpose(j):
            r0 = j * 128 if isinstance(j, int) else pl.multiple_of(j * 128, 128)
            bx_s[pl.ds(r0, 128), :] = bxt_s[j].T

        def blk(h0, nh, r_lo, r_hi, side, post=None, unroll=1):
            def body(i, c):
                h = h0 + i
                for r in range(r_lo, r_hi):
                    if r != QDEF:
                        qproj(h, h, r)
                    side(i, r - r_lo)
                if post is not None:
                    post(i)
                return c
            lax.fori_loop(0, nh, body, 0, unroll=unroll)

        def side_xpose(i, r):
            if r in XPOS:
                xpose(4 + i * 3 + XPOS.index(r))

        def side_wq(i, r):
            if r in WQPOS:
                r0 = jnp.minimum(i, DM // 64 - 1) * 64 + WQPOS.index(r) * 16
                relayout(rawq_s.at[1], wq_s, 8, pl.multiple_of(r0, 16), 16)
            if r in AVPOS:
                r0 = i * 64 + AVPOS.index(r) * 16
                relayout(rawa_s.at[2], awv_s, 0, pl.multiple_of(r0, 16), 16)

        def side_kv(i, r):
            w = jnp.swapaxes(rawkv_s[pl.ds(pl.multiple_of(i * 256 + r * 16, 16), 16)], 0, 1)
            r0 = pl.multiple_of((i % 4) * 256 + r * 16, 16)
            for h in range(H):
                wkv_s[(i // 4) * H + h, pl.ds(r0, 16), :] = w[h]

        for c in cp_bxt[:4]:
            c.wait()
        for j in range(4):
            xpose(j)

        def first(e, side):
            cols = slice(e * 128, (e + 1) * 128)
            for c in range(NRQ):
                cp_bwq_lo[e][c].wait()
                w = jnp.swapaxes(rawq_s[0, c * RQ:(c + 1) * RQ, :, cols], 0, 1)
                for h in range(8):
                    wq_s[h, c * RQ:(c + 1) * RQ, cols] = w[h]
            if e == 1:
                for c in cp_bxt[4:]:
                    c.wait()

            def body(i, c):
                for n in range(8):
                    u, r = divmod(n, 4)
                    rows = slice(r * QB, (r + 1) * QB)
                    q_s[2 * i + u, rows, cols] = (
                        _dot(bx_s[rows, :], wq_s[2 * i + u, :, cols]) * scale).astype(BF16)
                    side(i, n)
                return c
            lax.fori_loop(0, 4, body, 0)

        first(0, lambda i, n: None)
        first(1, side_xpose)
        qproj(0, 0, QDEF)
        cp_bwq_hi.wait()
        cp_awv(0).wait()
        blk(0, 8, 4, 16, side_wq, lambda i: cp_awv(i + 1).wait())
        wait_kv(0)
        blk(8, 8, 0, 16, side_kv, lambda i: wait_kv(i + 1))

    pl.run_scoped(
        prologue,
        pltpu.VMEM((S // 128, DM, 128), BF16),
        pltpu.VMEM((2, DM, 8, DH), BF16),
        pltpu.VMEM((2 * DC + 256, H, DH), BF16),
    )

    def main(wqk_s, wz_s, wg_s, wu_s, wt_s, ax_s, k_s, v_s, stage_s, ot_s,
             ts0, ts1, zs0, zs1, us0, us1):
        cp_ckv.wait()

        tri = (lax.broadcasted_iota(jnp.int32, (HB, HB), 1)
               <= lax.broadcasted_iota(jnp.int32, (HB, HB), 0))
        tri2 = (lax.broadcasted_iota(jnp.int32, (BQ, HB), 1)
                <= lax.broadcasted_iota(jnp.int32, (BQ, HB), 0))

        def kvproj(dst, h, pb, lo, hi):
            for r0 in range(lo, hi, pb):
                dst[r0:r0 + pb, :] = _dot(ckv_s[r0:r0 + pb, :], wkv_s[h]).astype(BF16)

        def qk(h, i):
            d0 = i * BQ
            q = q_s[h, d0:d0 + BQ, :]
            so = _dot_nt(q, k_s[0:d0, :]) if i > 0 else None
            s1 = _dot_nt(q, k_s[d0:d0 + HB, :])
            s2 = _dot_nt(q[HB:], k_s[d0 + HB:d0 + BQ, :])
            return so, s1, s2

        def soft_pv_out(h, i, ss):
            so, s1, s2 = ss
            d0 = i * BQ
            s1 = jnp.where(tri2, s1, NEG)
            s2 = jnp.where(tri, s2, NEG)
            m = jnp.max(s1, axis=1, keepdims=True)
            if so is not None:
                m = jnp.maximum(m, jnp.max(so, axis=1, keepdims=True))
            mb = jnp.maximum(m[HB:], jnp.max(s2, axis=1, keepdims=True))
            m = jnp.concatenate([m[:HB], mb], axis=0)
            p1 = jnp.exp2(s1 - m)
            p2 = jnp.exp2(s2 - mb)
            l = jnp.sum(p1, axis=1, keepdims=True)
            acc = _dot(p1.astype(BF16), v_s[d0:d0 + HB, :])
            if so is not None:
                po = jnp.exp2(so - m)
                l = l + jnp.sum(po, axis=1, keepdims=True)
                acc = acc + _dot(po.astype(BF16), v_s[0:d0, :])
            l2 = l[HB:] + jnp.sum(p2, axis=1, keepdims=True)
            acc2 = acc[HB:] + _dot(p2.astype(BF16), v_s[d0 + HB:d0 + BQ, :])
            ctx = jnp.concatenate(
                [acc[:HB] * _recip(l[:HB]), acc2 * _recip(l2)], axis=0).astype(BF16)
            q_s[h, d0:d0 + BQ, :] = ctx

        def head(h, c):
            kvproj(k_s, h, KB, 0, S)
            order = list(range(NQ - 1, -1, -1))
            ss = qk(h, order[0])
            kvproj(v_s, H + h, PB, 0, S)
            for n, i in enumerate(order):
                nxt = qk(h, order[n + 1]) if n + 1 < NQ else None
                if n == NQ - 2:
                    qproj(h + 1, jnp.minimum(h + 1, H - 1), QDEF)
                soft_pv_out(h, i, ss)
                ss = nxt
            return c

        lax.fori_loop(0, N_HEAD_ITERS, head, 0)

        cp_bwot.wait()
        cp_awot.wait()
        for c in cp_axt + cp_aw + [cp_mem0]:
            c.wait()
        ot_s[0] = jnp.zeros((DM, 128), F32)

        def flush(r0):
            stage_s[pl.ds(r0, 128), DM:2 * DM] = ot_s[0].T.astype(BF16)

        def oproj(j, c):
            r0 = pl.multiple_of(j * 128, 128)
            pin_h = jnp.maximum(j, H)
            pin_o = jnp.where(j >= 0, 1, 0)
            acc = None
            for h in range(H):
                r = _dot_nt(bwot_s[h], q_s[h, pl.ds(r0, 128), :])
                acc = r if acc is None else acc + r
                if h == 0:
                    ot_s[pin_o, 0:8, :] = r[0:8]
                    flush(pl.multiple_of(jnp.maximum(j - 1, 0) * 128, 128))
                elif h == 14:
                    axt_s[pin_h, 0:16, :] = r[0:16].astype(BF16)
                    ax_s[pl.ds(r0, 128), :] = axt_s[j].T
            ot_s[0] = acc
            return c

        lax.fori_loop(0, N_OPROJ_ITERS, oproj, 0, unroll=OU)
        flush(S - 128)

        RC = 384 // 4

        def tails(a, b, mul):
            t = [_dot_nt(b[u], a[u]) for u in range(2)]
            return (jnp.concatenate(t, axis=0) * mul).astype(BF16).T

        def wzprep(i, c):
            for n in range(8):
                if n == TAILPOS:
                    wz_s[i, :, 384:512] = tails(
                        [awv_s[2 * i + u, 0:384, :] for u in range(2)],
                        [awot_s[2 * i + u, 384:DM, :] for u in range(2)], 1.0)
                if n == TAILPOS2:
                    for u in range(2):
                        wt_s[i, u * 64:(u + 1) * 64, :] = _dot_nt(
                            awv_s[2 * i + u, 384:DM, :], awot_s[2 * i + u]).astype(BF16)
                rc, u = divmod(n, 2)
                rows = slice(rc * RC, (rc + 1) * RC)
                w = _dot_nt(awv_s[2 * i + u, rows, :], awot_s[2 * i + u, 0:384, :])
                wz_s[i, rows, u * 512:u * 512 + 384] = w.astype(BF16)
                if n < 7:
                    piece = i * 7 + n
                    t = jnp.where(piece >= DM // 16, 1, 0)
                    rr = pl.multiple_of((piece - t * (DM // 16)) * 16, 16)
                    wr = jnp.swapaxes(rawa_s[t, pl.ds(rr, 16)], 0, 1)
                    for h in range(H):
                        wqk_s[t, h, pl.ds(rr, 16), :] = wr[h]
            return c

        lax.fori_loop(0, H // 2, wzprep, 0, unroll=WU)

        def gprep(i, c):
            for n in range(2 * GRC):
                if n == GTAIL:
                    wg_s[i, :, 384:512] = tails(
                        [wqk_s[0, 2 * i + u, 0:384, :] for u in range(2)],
                        [wqk_s[1, 2 * i + u, 384:DM, :] for u in range(2)], scale)
                if n == GTAIL2:
                    wu_s[i] = tails(
                        [wqk_s[1, 2 * i + u] for u in range(2)],
                        [wqk_s[0, 2 * i + u, 384:DM, :] for u in range(2)], scale)
                rc, u = divmod(n, 2)
                rows = slice(rc * (384 // GRC), (rc + 1) * (384 // GRC))
                w = _dot_nt(wqk_s[0, 2 * i + u, rows, :], wqk_s[1, 2 * i + u, 0:384, :])
                wg_s[i, rows, u * 512:u * 512 + 384] = (w * scale).astype(BF16)
            return c

        lax.fori_loop(0, H // 2, gprep, 0, unroll=GU)

        key = lax.broadcasted_iota(jnp.int32, (L, H * L), 0)
        qry = lax.broadcasted_iota(jnp.int32, (L, H * L), 1) % L
        mask = (qry >= SEG) | (key >= SEG) | (key <= qry)
        lane = lax.broadcasted_iota(jnp.int32, (8, 128), 1)
        lane_l = lax.broadcasted_iota(jnp.int32, (L, 128), 1)
        NT_ = H * L // 128
        tile_heads = [[h for h in range(H) if h * L < (t + 1) * 128 and (h + 1) * L > t * 128]
                      for t in range(NT_)]

        def proj(lhs, w_ref, dests, chunks):
            for i in chunks:
                r = _dot(lhs, w_ref[i])
                mid = r[:, 384:512]
                parts = [(r[:, 0:384].astype(BF16), mid.astype(BF16)),
                         (r[:, 512:896].astype(BF16), pltpu.roll(mid, 64, 1).astype(BF16))]
                for u in range(2):
                    for (a, n, d, b) in dests:
                        r0 = (2 * i + u) * L + b
                        d[r0:r0 + n, 0:384] = parts[u][0][a:a + n]
                        d[r0:r0 + n, 384:512] = parts[u][1][a:a + n]

        def proj_u(lhs, dests):
            for i in range(H // 2):
                r = _dot(lhs, wu_s[i])
                parts = [r.astype(BF16), pltpu.roll(r, 64, 1).astype(BF16)]
                for u in range(2):
                    for (a, n, d, b) in dests:
                        r0 = (2 * i + u) * L + b
                        d[r0:r0 + n, :] = parts[u][a:a + n]

        def head_t(p):
            rs = []
            for t in range(NT_):
                pt = p[:, t * 128:(t + 1) * 128]
                grp = [None] * 16
                for h in tile_heads[t]:
                    for kk in range(L // 8):
                        g = (h * (L // 8) + kk) % 16
                        piece = pt[kk * 8:(kk + 1) * 8]
                        grp[g] = piece if grp[g] is None else jnp.where(
                            lane >= h * L - t * 128, piece, grp[g])
                rs.append(jnp.concatenate(grp, axis=0).T)
            rr = jnp.concatenate(rs, axis=0)
            pcs = []
            for t in range(NT_):
                pc = None
                for h in tile_heads[t]:
                    piece = rr[h * L:(h + 1) * L]
                    pc = piece if pc is None else jnp.where(
                        lane_l >= h * L - t * 128, piece, pc)
                pcs.append(pc)
            return jnp.concatenate(pcs, axis=1)

        def seg(lhs, hs, sel, w, left):
            def dests(refs):
                return [(a, n, refs[v], b) for (a, n, v, b) in sel]
            ts, zs, us = (ts0, ts1), (zs0, zs1), (us0, us1)
            v = {}
            for step in ORDER.split():
                if step == "U":
                    proj_u(lhs, dests(us))
                elif step[0] == "T":
                    proj(lhs[:, 0:384], wg_s, dests(ts), [int(c) for c in step[1:]])
                elif step[0] == "Z":
                    proj(lhs[:, 0:384], wz_s, dests(zs), [int(c) for c in step[1:]])
                elif step == "st":
                    v["st"] = _dot_nt(hs[:, 384:DM], us[w][:, 0:64])
                elif step == "sc":
                    v["sc"] = _dot_nt(hs, ts[w][:, 0:DM])
                elif step == "x1":
                    v["st"] = head_t(v["st"])
                elif step == "sm":
                    sc = jnp.where(mask, v["sc"] + v["st"], NEG)
                    e = jnp.exp2(sc - jnp.max(sc, axis=0, keepdims=True))
                    v["p"] = e * _recip(jnp.sum(e, axis=0, keepdims=True))
                elif step == "x2":
                    v["pf"] = head_t(v["p"])
                    v["pc"] = v["pf"].astype(BF16)
                elif step == "ut":
                    v["u"] = lax.dot_general(hs[:, 384:DM], v["p"].astype(BF16), TN,
                                             preferred_element_type=F32)
                elif step == "x3":
                    ut = jnp.concatenate([v["u"], v["u"]], axis=0)
                    rr = jnp.concatenate(
                        [ut[:, t * 128:(t + 1) * 128].T for t in range(NT_)], axis=0)
                    v["u"] = jnp.concatenate(
                        [jnp.where(lane_l < 64, rr[2 * i * L:(2 * i + 1) * L],
                                   rr[(2 * i + 1) * L:(2 * i + 2) * L])
                         for i in range(H // 2)], axis=1)
                elif step == "F":
                    rows = v["u"][8:L] if left is None else jnp.concatenate(
                        [v["u"], left], axis=0)
                    v["f"] = _dot(rows.astype(BF16), wt_s[...].reshape(H * 64, DM))
                elif step == "PV":
                    if w in PVS:
                        o1 = _dot(v["pf"][24:L].astype(BF16), zs[w][...])[:, 0:DM]
                        o2 = _dot(v["pf"][0:24].astype(BF16), zs[w][...])[:, 0:DM]
                        v["o"] = jnp.concatenate([o2, o1], axis=0)
                    else:
                        v["o"] = _dot(v["pc"], zs[w][...])[:, 0:DM]
            return v["o"], v["f"], v["u"][0:8]

        def out_copy(base):
            return pltpu.make_async_copy(
                stage_s.at[pl.ds(base, 2 * SEG)], out_hbm.at[pl.ds(base, 2 * SEG)], osem)

        def pair(j, mem):
            base = pl.multiple_of(j * 2 * SEG, 2 * SEG)
            x0 = ax_s[pl.ds(base, SEG), :]
            x1 = ax_s[pl.ds(base + SEG, SEG), :]
            lhs1 = jnp.concatenate([x0, x1[0:8], mem], axis=0)
            o1, f1, left = seg(lhs1, jnp.concatenate([x0, mem], axis=0),
                               [(0, 32, 0, 0), (32, 8, 1, 0), (40, 8, 0, 32)], 0, None)
            mem1 = (o1[SEG:L] + f1[SEG - 8:SEG]).astype(BF16)
            lhs2 = jnp.concatenate([x1[16:32], mem1, x1[8:16]], axis=0)
            o2, f2, _ = seg(lhs2, jnp.concatenate([x1, mem1], axis=0),
                            [(0, 16, 1, 16), (16, 8, 1, 32), (24, 8, 1, 8)], 1, left)
            f1 = jnp.concatenate([f2[L:L + 8], f1[0:SEG - 8]], axis=0)
            stage_s[pl.ds(base, SEG), 0:DM] = (o1[0:SEG] + f1).astype(BF16)
            out2 = (o2 + f2[0:L]).astype(BF16)
            stage_s[pl.ds(base + SEG, SEG), 0:DM] = out2[0:SEG]
            out_copy(base).start()
            return out2[SEG:L]

        lax.fori_loop(0, N_PAIR_ITERS, pair, mem0_s[...])
        for j in range(N_PAIR_ITERS):
            out_copy(j * 2 * SEG).wait()

    pl.run_scoped(
        main,
        pltpu.VMEM((2, H, DM, DH), BF16),
        pltpu.VMEM((H // 2, 384, 2 * DM), BF16), pltpu.VMEM((H // 2, 384, 2 * DM), BF16),
        pltpu.VMEM((H // 2, DM, 128), BF16), pltpu.VMEM((H // 2, 128, DM), BF16),
        pltpu.VMEM((S, DM), BF16),
        pltpu.VMEM((S, DH), BF16), pltpu.VMEM((S, DH), BF16),
        pltpu.VMEM((S, 2 * DM), BF16), pltpu.VMEM((2, DM, 128), F32),
        pltpu.VMEM((H * L, 512), BF16), pltpu.VMEM((H * L, 512), BF16),
        pltpu.VMEM((H * L, 512), BF16), pltpu.VMEM((H * L, 512), BF16),
        pltpu.VMEM((H * L, 128), BF16), pltpu.VMEM((H * L, 128), BF16),
    )


@functools.partial(jax.jit, static_argnames=("A_seg_len",))
def pallas_concat_heads__memory_aug_recurrent_mem_tr__compressed_kv_cla__prompt_kernel(
    A_x: jax.Array,
    A_mem0: jax.Array,
    A_Wq: jax.Array,
    A_Wk: jax.Array,
    A_Wv: jax.Array,
    A_Wo: jax.Array,
    A_seg_len: int,
    B_x: jax.Array,
    B_c_kv: jax.Array,
    B_w_q: jax.Array,
    B_w_uk: jax.Array,
    B_w_uv: jax.Array,
    B_w_o: jax.Array,
):
    assert A_seg_len == SEG
    assert A_x.shape == (1, S, DM) and A_mem0.shape == (1, MEM, DM)
    assert A_Wq.shape == (DM, H, DH) and A_Wo.shape == (H, DH, DM)
    assert B_x.shape == (1, S, DM) and B_c_kv.shape == (1, S, DC)
    assert B_w_q.shape == (DM, H, DH) and B_w_uk.shape == (DC, H, DH)
    assert B_w_o.shape == (H, DH, DM)

    axt = jnp.swapaxes(A_x, 1, 2).reshape(DM, S)
    bxt = jnp.swapaxes(B_x, 1, 2).reshape(DM, S)
    awot = jnp.swapaxes(A_Wo, 1, 2)
    bwot = jnp.swapaxes(B_w_o, 1, 2)

    any_spec = pl.BlockSpec(memory_space=pl.ANY)
    out = pl.pallas_call(
        _kernel,
        out_shape=jax.ShapeDtypeStruct((S, 2 * DM), BF16),
        in_specs=[any_spec] * 12,
        out_specs=any_spec,
        scratch_shapes=[
            pltpu.VMEM((2 * H, DC, DH), BF16),
            pltpu.VMEM((S, DC), BF16),
            pltpu.VMEM((H, DM, DH), BF16),
            pltpu.VMEM((H + 1, S, DH), BF16),
            pltpu.VMEM((3, DM + 128, H, DH), BF16),
            pltpu.VMEM((H, DM, DH), BF16),
            pltpu.VMEM((H, DM + 64, DH), BF16),
            pltpu.VMEM((S // 128 + 1, DM, 128), BF16),
            pltpu.VMEM((MEM, DM), BF16),
            pltpu.VMEM((S, DM), BF16),
            pltpu.VMEM((H, DM, DH), BF16),
            pltpu.SemaphoreType.DMA((44,)),
            pltpu.SemaphoreType.DMA,
        ],
        compiler_params=pltpu.CompilerParams(vmem_limit_bytes=120 * 1024 * 1024),
    )(axt, A_mem0.reshape(MEM, DM), A_Wq, A_Wk, A_Wv, awot,
      bxt, B_c_kv.reshape(S, DC), B_w_q, B_w_uk, B_w_uv, bwot)
    return out.reshape(1, S, 2 * DM)
```

```python
import functools

import jax
import jax.numpy as jnp
from jax import lax
import jax.experimental.pallas as pl
import jax.experimental.pallas.tpu as pltpu

F32 = jnp.float32
BF16 = jnp.bfloat16
NT = (((1,), (1,)), ((), ()))
TN = (((0,), (0,)), ((), ()))
NEG = -1000000000.0

S = 2048
DM = 448
H = 16
DH = 256
HD = H * DH
DC = 1024
MEM = 8
SEG = 32
L = SEG + MEM
NPAIR = S // (2 * SEG)

BQ = 256
HB = BQ // 2
NQ = S // BQ
PB = 512
QB = 128
KB = 128
N_OPROJ_ITERS = S // 128
N_HEAD_ITERS = H
N_PAIR_ITERS = NPAIR
TAILPOS = 4
TAILPOS2 = 2
PVS = (0,)
QDEF = 8
OU = 2
WU = 2
GU = 2
NRQ = 4
XPOS = (5, 6, 7)
WQPOS = (8, 9, 10, 11)
AVPOS = (0, 1, 2, 3)
GRC = 2
GTAIL = 2
GTAIL2 = 1
ORDER = 'U T01 st T234567 x1 sc Z01 sm Z2 ut x2 Z34 x3 Z567 F PV'


def _dot(a, b):
    return jnp.dot(a, b, preferred_element_type=F32)


def _dot_nt(a, b):
    return lax.dot_general(a, b, NT, preferred_element_type=F32)


def _recip(l):
    r = pl.reciprocal(l, approx=True)
    return r * (2.0 - l * r)


def _kernel(axt_hbm, mem0_hbm, awq_hbm, awk_hbm, awv_hbm, awot_hbm,
            bxt_hbm, ckv_hbm, bwq_hbm, bwk_hbm, bwv_hbm, bwot_hbm,
            out_hbm,
            wkv_s, ckv_s, bwot_s, q_s, rawa_s, awot_s, awv_s, axt_s, mem0_s, bx_s, wq_s,
            sems, osem):
    scale = DH ** -0.5 * 1.4426950408889634

    def cp(src, dst, i):
        return pltpu.make_async_copy(src, dst, sems.at[i])

    cp_ckv = cp(ckv_hbm, ckv_s, 6)
    cp_bwot = cp(bwot_hbm, bwot_s, 7)
    cp_awot = cp(awot_hbm, awot_s, 8)
    cp_axt = [cp(axt_hbm.at[:, pl.ds(j * 128, 128)], axt_s.at[j], 9)
              for j in range(S // 128)]
    cp_aw = [cp(w, rawa_s.at[t, pl.ds(0, DM)], 10 + t)
             for t, w in enumerate((awq_hbm, awk_hbm))]

    def cp_awv(i):
        lo = min if isinstance(i, int) else jnp.minimum
        return cp(awv_hbm.at[pl.ds(lo(i, DM // 64 - 1) * 64, 64)],
                  rawa_s.at[2, pl.ds(i * 64, 64)], 18 + i)

    cp_mem0 = cp(mem0_hbm, mem0_s, 13)

    def qproj(h, hw, r):
        rows = slice(r * QB, (r + 1) * QB)
        q_s[h, rows, :] = (_dot(bx_s[rows, :], wq_s[hw]) * scale).astype(BF16)

    def prologue(bxt_s, rawq_s, rawkv_s):
        cp_bxt = [cp(bxt_hbm.at[:, pl.ds(j * 128, 128)], bxt_s.at[j], 0 if j < 4 else 1)
                  for j in range(S // 128)]
        RQ = DM // NRQ
        cp_bwq_lo = [[cp(bwq_hbm.at[pl.ds(c * RQ, RQ), pl.ds(0, 8), pl.ds(e * 128, 128)],
                         rawq_s.at[0, pl.ds(c * RQ, RQ), :, pl.ds(e * 128, 128)],
                         36 + e * NRQ + c) for c in range(NRQ)] for e in range(2)]
        cp_bwq_hi = cp(bwq_hbm.at[:, pl.ds(8, 8), :], rawq_s.at[1], 3)

        def cp_kv(i):
            src = bwk_hbm if i < 4 else bwv_hbm
            return cp(src.at[pl.ds(min(i % 4 + i // 8 * 3, 3) * 256, 256)],
                      rawkv_s.at[pl.ds(i * 256, 256)], 27 + i)

        def wait_kv(i):
            dst = rawkv_s.at[pl.ds(i * 256, 256)]
            cp(dst, dst, 27 + i).wait()

        for c in (cp_bxt[:4] + cp_bwq_lo[0] + cp_bwq_lo[1] + cp_bxt[4:]
                  + [cp_bwq_hi] + [cp_awv(i) for i in range(9)]
                  + [cp_kv(i) for i in range(9)]
                  + [cp_ckv, cp_bwot, cp_awot] + cp_axt + cp_aw + [cp_mem0]):
            c.start()

        def relayout(src, dst, h0, r0, n):
            w = jnp.swapaxes(src[pl.ds(r0, n)], 0, 1)
            for h in range(w.shape[0]):
                dst[h0 + h, pl.ds(r0, n), :] = w[h]

        def xpose(j):
            r0 = j * 128 if isinstance(j, int) else pl.multiple_of(j * 128, 128)
            bx_s[pl.ds(r0, 128), :] = bxt_s[j].T

        def blk(h0, nh, r_lo, r_hi, side, post=None, unroll=1):
            def body(i, c):
                h = h0 + i
                for r in range(r_lo, r_hi):
                    if r != QDEF:
                        qproj(h, h, r)
                    side(i, r - r_lo)
                if post is not None:
                    post(i)
                return c
            lax.fori_loop(0, nh, body, 0, unroll=unroll)

        def side_xpose(i, r):
            if r in XPOS:
                xpose(4 + i * 3 + XPOS.index(r))

        def side_wq(i, r):
            if r in WQPOS:
                r0 = jnp.minimum(i, DM // 64 - 1) * 64 + WQPOS.index(r) * 16
                relayout(rawq_s.at[1], wq_s, 8, pl.multiple_of(r0, 16), 16)
            if r in AVPOS:
                r0 = i * 64 + AVPOS.index(r) * 16
                relayout(rawa_s.at[2], awv_s, 0, pl.multiple_of(r0, 16), 16)

        def side_kv(i, r):
            w = jnp.swapaxes(rawkv_s[pl.ds(pl.multiple_of(i * 256 + r * 16, 16), 16)], 0, 1)
            r0 = pl.multiple_of((i % 4) * 256 + r * 16, 16)
            for h in range(H):
                wkv_s[(i // 4) * H + h, pl.ds(r0, 16), :] = w[h]

        for c in cp_bxt[:4]:
            c.wait()
        for j in range(4):
            xpose(j)

        def first(e, side):
            cols = slice(e * 128, (e + 1) * 128)
            def piece(c, carry):
                r0 = pl.multiple_of(c * RQ, 16)
                dst = rawq_s.at[0, pl.ds(r0, RQ), :, pl.ds(e * 128, 128)]
                cp(dst, dst, 36 + e * NRQ + c).wait()
                w = jnp.swapaxes(rawq_s[0, pl.ds(r0, RQ), :, cols], 0, 1)
                for h in range(8):
                    wq_s[h, pl.ds(r0, RQ), cols] = w[h]
                return carry
            lax.fori_loop(0, NRQ, piece, 0)
            if e == 1:
                for c in cp_bxt[4:]:
                    c.wait()

            def body(i, c):
                for n in range(8):
                    u, r = divmod(n, 4)
                    rows = slice(r * QB, (r + 1) * QB)
                    q_s[2 * i + u, rows, cols] = (
                        _dot(bx_s[rows, :], wq_s[2 * i + u, :, cols]) * scale).astype(BF16)
                    side(i, n)
                return c
            lax.fori_loop(0, 4, body, 0)

        first(0, lambda i, n: None)
        first(1, side_xpose)
        qproj(0, 0, QDEF)
        cp_bwq_hi.wait()
        cp_awv(0).wait()
        blk(0, 8, 4, 16, side_wq, lambda i: cp_awv(i + 1).wait())
        wait_kv(0)
        blk(8, 8, 0, 16, side_kv, lambda i: wait_kv(i + 1))

    pl.run_scoped(
        prologue,
        pltpu.VMEM((S // 128, DM, 128), BF16),
        pltpu.VMEM((2, DM, 8, DH), BF16),
        pltpu.VMEM((2 * DC + 256, H, DH), BF16),
    )

    def main(wqk_s, wz_s, wg_s, wu_s, wt_s, ax_s, k_s, v_s, stage_s, ot_s,
             ts0, ts1, zs0, zs1, us0, us1):
        cp_ckv.wait()

        tri = (lax.broadcasted_iota(jnp.int32, (HB, HB), 1)
               <= lax.broadcasted_iota(jnp.int32, (HB, HB), 0))
        tri2 = (lax.broadcasted_iota(jnp.int32, (BQ, HB), 1)
                <= lax.broadcasted_iota(jnp.int32, (BQ, HB), 0))

        def kvproj(dst, h, pb, lo, hi):
            for r0 in range(lo, hi, pb):
                dst[r0:r0 + pb, :] = _dot(ckv_s[r0:r0 + pb, :], wkv_s[h]).astype(BF16)

        def qk(h, i):
            d0 = i * BQ
            q = q_s[h, d0:d0 + BQ, :]
            so = _dot_nt(q, k_s[0:d0, :]) if i > 0 else None
            s1 = _dot_nt(q, k_s[d0:d0 + HB, :])
            s2 = _dot_nt(q[HB:], k_s[d0 + HB:d0 + BQ, :])
            return so, s1, s2

        def soft_pv_out(h, i, ss):
            so, s1, s2 = ss
            d0 = i * BQ
            s1 = jnp.where(tri2, s1, NEG)
            s2 = jnp.where(tri, s2, NEG)
            m = jnp.max(s1, axis=1, keepdims=True)
            if so is not None:
                m = jnp.maximum(m, jnp.max(so, axis=1, keepdims=True))
            mb = jnp.maximum(m[HB:], jnp.max(s2, axis=1, keepdims=True))
            m = jnp.concatenate([m[:HB], mb], axis=0)
            p1 = jnp.exp2(s1 - m)
            p2 = jnp.exp2(s2 - mb)
            l = jnp.sum(p1, axis=1, keepdims=True)
            acc = _dot(p1.astype(BF16), v_s[d0:d0 + HB, :])
            if so is not None:
                po = jnp.exp2(so - m)
                l = l + jnp.sum(po, axis=1, keepdims=True)
                acc = acc + _dot(po.astype(BF16), v_s[0:d0, :])
            l2 = l[HB:] + jnp.sum(p2, axis=1, keepdims=True)
            acc2 = acc[HB:] + _dot(p2.astype(BF16), v_s[d0 + HB:d0 + BQ, :])
            ctx = jnp.concatenate(
                [acc[:HB] * _recip(l[:HB]), acc2 * _recip(l2)], axis=0).astype(BF16)
            q_s[h, d0:d0 + BQ, :] = ctx

        def head(h, c):
            kvproj(k_s, h, KB, 0, S)
            order = list(range(NQ - 1, -1, -1))
            ss = qk(h, order[0])
            kvproj(v_s, H + h, PB, 0, S)
            for n, i in enumerate(order):
                nxt = qk(h, order[n + 1]) if n + 1 < NQ else None
                if n == NQ - 2:
                    qproj(h + 1, jnp.minimum(h + 1, H - 1), QDEF)
                soft_pv_out(h, i, ss)
                ss = nxt
            return c

        lax.fori_loop(0, N_HEAD_ITERS, head, 0)

        cp_bwot.wait()
        cp_awot.wait()
        for c in cp_axt + cp_aw + [cp_mem0]:
            c.wait()
        ot_s[0] = jnp.zeros((DM, 128), F32)

        def flush(r0):
            stage_s[pl.ds(r0, 128), DM:2 * DM] = ot_s[0].T.astype(BF16)

        def oproj(j, c):
            r0 = pl.multiple_of(j * 128, 128)
            pin_h = jnp.maximum(j, H)
            pin_o = jnp.where(j >= 0, 1, 0)
            acc = None
            for h in range(H):
                r = _dot_nt(bwot_s[h], q_s[h, pl.ds(r0, 128), :])
                acc = r if acc is None else acc + r
                if h == 0:
                    ot_s[pin_o, 0:8, :] = r[0:8]
                    flush(pl.multiple_of(jnp.maximum(j - 1, 0) * 128, 128))
                elif h == 14:
                    axt_s[pin_h, 0:16, :] = r[0:16].astype(BF16)
                    ax_s[pl.ds(r0, 128), :] = axt_s[j].T
            ot_s[0] = acc
            return c

        lax.fori_loop(0, N_OPROJ_ITERS, oproj, 0, unroll=OU)
        flush(S - 128)

        RC = 384 // 4

        def tails(a, b, mul):
            t = [_dot_nt(b[u], a[u]) for u in range(2)]
            return (jnp.concatenate(t, axis=0) * mul).astype(BF16).T

        def wzprep(i, c):
            for n in range(8):
                if n == TAILPOS:
                    wz_s[i, :, 384:512] = tails(
                        [awv_s[2 * i + u, 0:384, :] for u in range(2)],
                        [awot_s[2 * i + u, 384:DM, :] for u in range(2)], 1.0)
                if n == TAILPOS2:
                    for u in range(2):
                        wt_s[i, u * 64:(u + 1) * 64, :] = _dot_nt(
                            awv_s[2 * i + u, 384:DM, :], awot_s[2 * i + u]).astype(BF16)
                rc, u = divmod(n, 2)
                rows = slice(rc * RC, (rc + 1) * RC)
                w = _dot_nt(awv_s[2 * i + u, rows, :], awot_s[2 * i + u, 0:384, :])
                wz_s[i, rows, u * 512:u * 512 + 384] = w.astype(BF16)
                if n < 7:
                    piece = i * 7 + n
                    t = jnp.where(piece >= DM // 16, 1, 0)
                    rr = pl.multiple_of((piece - t * (DM // 16)) * 16, 16)
                    wr = jnp.swapaxes(rawa_s[t, pl.ds(rr, 16)], 0, 1)
                    for h in range(H):
                        wqk_s[t, h, pl.ds(rr, 16), :] = wr[h]
            return c

        lax.fori_loop(0, H // 2, wzprep, 0, unroll=WU)

        def gprep(i, c):
            for n in range(2 * GRC):
                if n == GTAIL:
                    wg_s[i, :, 384:512] = tails(
                        [wqk_s[0, 2 * i + u, 0:384, :] for u in range(2)],
                        [wqk_s[1, 2 * i + u, 384:DM, :] for u in range(2)], scale)
                if n == GTAIL2:
                    wu_s[i] = tails(
                        [wqk_s[1, 2 * i + u] for u in range(2)],
                        [wqk_s[0, 2 * i + u, 384:DM, :] for u in range(2)], scale)
                rc, u = divmod(n, 2)
                rows = slice(rc * (384 // GRC), (rc + 1) * (384 // GRC))
                w = _dot_nt(wqk_s[0, 2 * i + u, rows, :], wqk_s[1, 2 * i + u, 0:384, :])
                wg_s[i, rows, u * 512:u * 512 + 384] = (w * scale).astype(BF16)
            return c

        lax.fori_loop(0, H // 2, gprep, 0, unroll=GU)

        key = lax.broadcasted_iota(jnp.int32, (L, H * L), 0)
        qry = lax.broadcasted_iota(jnp.int32, (L, H * L), 1) % L
        mask = (qry >= SEG) | (key >= SEG) | (key <= qry)
        lane = lax.broadcasted_iota(jnp.int32, (8, 128), 1)
        lane_l = lax.broadcasted_iota(jnp.int32, (L, 128), 1)
        NT_ = H * L // 128
        tile_heads = [[h for h in range(H) if h * L < (t + 1) * 128 and (h + 1) * L > t * 128]
                      for t in range(NT_)]

        def proj(lhs, w_ref, dests, chunks):
            for i in chunks:
                r = _dot(lhs, w_ref[i])
                mid = r[:, 384:512]
                parts = [(r[:, 0:384].astype(BF16), mid.astype(BF16)),
                         (r[:, 512:896].astype(BF16), pltpu.roll(mid, 64, 1).astype(BF16))]
                for u in range(2):
                    for (a, n, d, b) in dests:
                        r0 = (2 * i + u) * L + b
                        d[r0:r0 + n, 0:384] = parts[u][0][a:a + n]
                        d[r0:r0 + n, 384:512] = parts[u][1][a:a + n]

        def proj_u(lhs, dests):
            for i in range(H // 2):
                r = _dot(lhs, wu_s[i])
                parts = [r.astype(BF16), pltpu.roll(r, 64, 1).astype(BF16)]
                for u in range(2):
                    for (a, n, d, b) in dests:
                        r0 = (2 * i + u) * L + b
                        d[r0:r0 + n, :] = parts[u][a:a + n]

        def head_t(p):
            rs = []
            for t in range(NT_):
                pt = p[:, t * 128:(t + 1) * 128]
                grp = [None] * 16
                for h in tile_heads[t]:
                    for kk in range(L // 8):
                        g = (h * (L // 8) + kk) % 16
                        piece = pt[kk * 8:(kk + 1) * 8]
                        grp[g] = piece if grp[g] is None else jnp.where(
                            lane >= h * L - t * 128, piece, grp[g])
                rs.append(jnp.concatenate(grp, axis=0).T)
            rr = jnp.concatenate(rs, axis=0)
            pcs = []
            for t in range(NT_):
                pc = None
                for h in tile_heads[t]:
                    piece = rr[h * L:(h + 1) * L]
                    pc = piece if pc is None else jnp.where(
                        lane_l >= h * L - t * 128, piece, pc)
                pcs.append(pc)
            return jnp.concatenate(pcs, axis=1)

        def seg(lhs, hs, sel, w, left):
            def dests(refs):
                return [(a, n, refs[v], b) for (a, n, v, b) in sel]
            ts, zs, us = (ts0, ts1), (zs0, zs1), (us0, us1)
            v = {}
            for step in ORDER.split():
                if step == "U":
                    proj_u(lhs, dests(us))
                elif step[0] == "T":
                    proj(lhs[:, 0:384], wg_s, dests(ts), [int(c) for c in step[1:]])
                elif step[0] == "Z":
                    proj(lhs[:, 0:384], wz_s, dests(zs), [int(c) for c in step[1:]])
                elif step == "st":
                    v["st"] = _dot_nt(hs[:, 384:DM], us[w][:, 0:64])
                elif step == "sc":
                    v["sc"] = _dot_nt(hs, ts[w][:, 0:DM])
                elif step == "x1":
                    v["st"] = head_t(v["st"])
                elif step == "sm":
                    sc = jnp.where(mask, v["sc"] + v["st"], NEG)
                    e = jnp.exp2(sc - jnp.max(sc, axis=0, keepdims=True))
                    v["p"] = e * _recip(jnp.sum(e, axis=0, keepdims=True))
                elif step == "x2":
                    v["pf"] = head_t(v["p"])
                    v["pc"] = v["pf"].astype(BF16)
                elif step == "ut":
                    v["u"] = lax.dot_general(hs[:, 384:DM], v["p"].astype(BF16), TN,
                                             preferred_element_type=F32)
                elif step == "x3":
                    ut = jnp.concatenate([v["u"], v["u"]], axis=0)
                    rr = jnp.concatenate(
                        [ut[:, t * 128:(t + 1) * 128].T for t in range(NT_)], axis=0)
                    v["u"] = jnp.concatenate(
                        [jnp.where(lane_l < 64, rr[2 * i * L:(2 * i + 1) * L],
                                   rr[(2 * i + 1) * L:(2 * i + 2) * L])
                         for i in range(H // 2)], axis=1)
                elif step == "F":
                    rows = v["u"][8:L] if left is None else jnp.concatenate(
                        [v["u"], left], axis=0)
                    v["f"] = _dot(rows.astype(BF16), wt_s[...].reshape(H * 64, DM))
                elif step == "PV":
                    if w in PVS:
                        o1 = _dot(v["pf"][24:L].astype(BF16), zs[w][...])[:, 0:DM]
                        o2 = _dot(v["pf"][0:24].astype(BF16), zs[w][...])[:, 0:DM]
                        v["o"] = jnp.concatenate([o2, o1], axis=0)
                    else:
                        v["o"] = _dot(v["pc"], zs[w][...])[:, 0:DM]
            return v["o"], v["f"], v["u"][0:8]

        def out_copy(base):
            return pltpu.make_async_copy(
                stage_s.at[pl.ds(base, 2 * SEG)], out_hbm.at[pl.ds(base, 2 * SEG)], osem)

        def pair(j, mem):
            base = pl.multiple_of(j * 2 * SEG, 2 * SEG)
            x0 = ax_s[pl.ds(base, SEG), :]
            x1 = ax_s[pl.ds(base + SEG, SEG), :]
            lhs1 = jnp.concatenate([x0, x1[0:8], mem], axis=0)
            o1, f1, left = seg(lhs1, jnp.concatenate([x0, mem], axis=0),
                               [(0, 32, 0, 0), (32, 8, 1, 0), (40, 8, 0, 32)], 0, None)
            mem1 = (o1[SEG:L] + f1[SEG - 8:SEG]).astype(BF16)
            lhs2 = jnp.concatenate([x1[16:32], mem1, x1[8:16]], axis=0)
            o2, f2, _ = seg(lhs2, jnp.concatenate([x1, mem1], axis=0),
                            [(0, 16, 1, 16), (16, 8, 1, 32), (24, 8, 1, 8)], 1, left)
            f1 = jnp.concatenate([f2[L:L + 8], f1[0:SEG - 8]], axis=0)
            stage_s[pl.ds(base, SEG), 0:DM] = (o1[0:SEG] + f1).astype(BF16)
            out2 = (o2 + f2[0:L]).astype(BF16)
            stage_s[pl.ds(base + SEG, SEG), 0:DM] = out2[0:SEG]
            out_copy(base).start()
            return out2[SEG:L]

        lax.fori_loop(0, N_PAIR_ITERS, pair, mem0_s[...])
        for j in range(N_PAIR_ITERS):
            out_copy(j * 2 * SEG).wait()

    pl.run_scoped(
        main,
        pltpu.VMEM((2, H, DM, DH), BF16),
        pltpu.VMEM((H // 2, 384, 2 * DM), BF16), pltpu.VMEM((H // 2, 384, 2 * DM), BF16),
        pltpu.VMEM((H // 2, DM, 128), BF16), pltpu.VMEM((H // 2, 128, DM), BF16),
        pltpu.VMEM((S, DM), BF16),
        pltpu.VMEM((S, DH), BF16), pltpu.VMEM((S, DH), BF16),
        pltpu.VMEM((S, 2 * DM), BF16), pltpu.VMEM((2, DM, 128), F32),
        pltpu.VMEM((H * L, 512), BF16), pltpu.VMEM((H * L, 512), BF16),
        pltpu.VMEM((H * L, 512), BF16), pltpu.VMEM((H * L, 512), BF16),
        pltpu.VMEM((H * L, 128), BF16), pltpu.VMEM((H * L, 128), BF16),
    )


@functools.partial(jax.jit, static_argnames=("A_seg_len",))
def pallas_concat_heads__memory_aug_recurrent_mem_tr__compressed_kv_cla__prompt_kernel(
    A_x: jax.Array,
    A_mem0: jax.Array,
    A_Wq: jax.Array,
    A_Wk: jax.Array,
    A_Wv: jax.Array,
    A_Wo: jax.Array,
    A_seg_len: int,
    B_x: jax.Array,
    B_c_kv: jax.Array,
    B_w_q: jax.Array,
    B_w_uk: jax.Array,
    B_w_uv: jax.Array,
    B_w_o: jax.Array,
):
    assert A_seg_len == SEG
    assert A_x.shape == (1, S, DM) and A_mem0.shape == (1, MEM, DM)
    assert A_Wq.shape == (DM, H, DH) and A_Wo.shape == (H, DH, DM)
    assert B_x.shape == (1, S, DM) and B_c_kv.shape == (1, S, DC)
    assert B_w_q.shape == (DM, H, DH) and B_w_uk.shape == (DC, H, DH)
    assert B_w_o.shape == (H, DH, DM)

    axt = jnp.swapaxes(A_x, 1, 2).reshape(DM, S)
    bxt = jnp.swapaxes(B_x, 1, 2).reshape(DM, S)
    awot = jnp.swapaxes(A_Wo, 1, 2)
    bwot = jnp.swapaxes(B_w_o, 1, 2)

    any_spec = pl.BlockSpec(memory_space=pl.ANY)
    out = pl.pallas_call(
        _kernel,
        out_shape=jax.ShapeDtypeStruct((S, 2 * DM), BF16),
        in_specs=[any_spec] * 12,
        out_specs=any_spec,
        scratch_shapes=[
            pltpu.VMEM((2 * H, DC, DH), BF16),
            pltpu.VMEM((S, DC), BF16),
            pltpu.VMEM((H, DM, DH), BF16),
            pltpu.VMEM((H + 1, S, DH), BF16),
            pltpu.VMEM((3, DM + 128, H, DH), BF16),
            pltpu.VMEM((H, DM, DH), BF16),
            pltpu.VMEM((H, DM + 64, DH), BF16),
            pltpu.VMEM((S // 128 + 1, DM, 128), BF16),
            pltpu.VMEM((MEM, DM), BF16),
            pltpu.VMEM((S, DM), BF16),
            pltpu.VMEM((H, DM, DH), BF16),
            pltpu.SemaphoreType.DMA((44,)),
            pltpu.SemaphoreType.DMA,
        ],
        compiler_params=pltpu.CompilerParams(vmem_limit_bytes=120 * 1024 * 1024),
    )(axt, A_mem0.reshape(MEM, DM), A_Wq, A_Wk, A_Wv, awot,
      bxt, B_c_kv.reshape(S, DC), B_w_q, B_w_uk, B_w_uv, bwot)
    return out.reshape(1, S, 2 * DM)
```

```python
import functools

import jax
import jax.numpy as jnp
from jax import lax
import jax.experimental.pallas as pl
import jax.experimental.pallas.tpu as pltpu

F32 = jnp.float32
BF16 = jnp.bfloat16
NT = (((1,), (1,)), ((), ()))
TN = (((0,), (0,)), ((), ()))
NEG = -1000000000.0

S = 2048
DM = 448
H = 16
DH = 256
DC = 1024
MEM = 8
SEG = 32
L = SEG + MEM
NPAIR = S // (2 * SEG)

BQ = 256
HB = BQ // 2
NQ = S // BQ
PB = 128
QB = 128
KB = 128
N_OPROJ_ITERS = S // 128
N_HEAD_ITERS = H
N_PAIR_ITERS = NPAIR
QDEF = 8
NRQ = 4

XPOS, WQPOS, AVPOS = (5, 6, 7), (8, 9, 10, 11), (0, 1, 2, 3)
TAILPOS, TAILPOS2 = 4, 2
GRC, GTAIL, GTAIL2 = 2, 2, 1
OU = WU = GU = 2
PVS = (0,)
ORDER = 'U T01 st T234567 x1 sc Z01 sm Z2 ut x2 Z34 x3 Z567 F PV'


def _dot(a, b):
    return jnp.dot(a, b, preferred_element_type=F32)


def _dot_nt(a, b):
    return lax.dot_general(a, b, NT, preferred_element_type=F32)


def _recip(l):
    r = pl.reciprocal(l, approx=True)
    return r * (2.0 - l * r)


def _kernel(axt_hbm, mem0_hbm, awq_hbm, awk_hbm, awv_hbm, awot_hbm,
            bxt_hbm, ckv_hbm, bwq_hbm, bwk_hbm, bwv_hbm, bwot_hbm,
            out_hbm,
            wkv_s, ckv_s, bwot_s, q_s, rawa_s, awot_s, awv_s, axt_s, mem0_s, bx_s, wq_s,
            sems, osem):
    scale = DH ** -0.5 * 1.4426950408889634

    def cp(src, dst, i):
        return pltpu.make_async_copy(src, dst, sems.at[i])

    cp_ckv = cp(ckv_hbm, ckv_s, 6)
    cp_bwot = cp(bwot_hbm, bwot_s, 7)
    cp_awot = cp(awot_hbm, awot_s, 8)
    cp_axt = [cp(axt_hbm.at[:, pl.ds(j * 128, 128)], axt_s.at[j], 9)
              for j in range(S // 128)]
    cp_aw = [cp(w, rawa_s.at[t, pl.ds(0, DM)], 10 + t)
             for t, w in enumerate((awq_hbm, awk_hbm))]

    def cp_awv(i):
        lo = min if isinstance(i, int) else jnp.minimum
        return cp(awv_hbm.at[pl.ds(lo(i, DM // 64 - 1) * 64, 64)],
                  rawa_s.at[2, pl.ds(i * 64, 64)], 18 + i)

    cp_mem0 = cp(mem0_hbm, mem0_s, 13)

    def qproj(h, hw, r):
        rows = slice(r * QB, (r + 1) * QB)
        q_s[h, rows, :] = (_dot(bx_s[rows, :], wq_s[hw]) * scale).astype(BF16)

    def prologue(bxt_s, rawq_s, rawkv_s):
        cp_bxt = [cp(bxt_hbm.at[:, pl.ds(j * 128, 128)], bxt_s.at[j], 0 if j < 4 else 1)
                  for j in range(S // 128)]
        RQ = DM // NRQ
        cp_bwq_lo = [[cp(bwq_hbm.at[pl.ds(c * RQ, RQ), pl.ds(0, 8), pl.ds(e * 128, 128)],
                         rawq_s.at[0, pl.ds(c * RQ, RQ), :, pl.ds(e * 128, 128)],
                         36 + e * NRQ + c) for c in range(NRQ)] for e in range(2)]
        cp_bwq_hi = cp(bwq_hbm.at[:, pl.ds(8, 8), :], rawq_s.at[1], 3)

        def cp_kv(i):
            src = bwk_hbm if i < 4 else bwv_hbm
            return cp(src.at[pl.ds(min(i % 4 + i // 8 * 3, 3) * 256, 256)],
                      rawkv_s.at[pl.ds(i * 256, 256)], 27 + i)

        def wait_kv(i):
            dst = rawkv_s.at[pl.ds(i * 256, 256)]
            cp(dst, dst, 27 + i).wait()

        for c in (cp_bxt[:4] + cp_bwq_lo[0] + cp_bwq_lo[1] + cp_bxt[4:]
                  + [cp_bwq_hi] + [cp_awv(i) for i in range(9)]
                  + [cp_kv(i) for i in range(9)]
                  + [cp_ckv, cp_bwot, cp_awot] + cp_axt + cp_aw + [cp_mem0]):
            c.start()

        def relayout(src, dst, h0, r0, n):
            w = jnp.swapaxes(src[pl.ds(r0, n)], 0, 1)
            for h in range(w.shape[0]):
                dst[h0 + h, pl.ds(r0, n), :] = w[h]

        def xpose(j):
            r0 = j * 128 if isinstance(j, int) else pl.multiple_of(j * 128, 128)
            bx_s[pl.ds(r0, 128), :] = bxt_s[j].T

        def blk(h0, nh, r_lo, r_hi, side, post=None, unroll=1):
            def body(i, c):
                h = h0 + i
                for r in range(r_lo, r_hi):
                    if r != QDEF:
                        qproj(h, h, r)
                    side(i, r - r_lo)
                if post is not None:
                    post(i)
                return c
            lax.fori_loop(0, nh, body, 0, unroll=unroll)

        def side_xpose(i, r):
            if r in XPOS:
                xpose(4 + i * 3 + XPOS.index(r))

        def side_wq(i, r):
            if r in WQPOS:
                r0 = jnp.minimum(i, DM // 64 - 1) * 64 + WQPOS.index(r) * 16
                relayout(rawq_s.at[1], wq_s, 8, pl.multiple_of(r0, 16), 16)
            if r in AVPOS:
                r0 = i * 64 + AVPOS.index(r) * 16
                relayout(rawa_s.at[2], awv_s, 0, pl.multiple_of(r0, 16), 16)

        def side_kv(i, r):
            w = jnp.swapaxes(rawkv_s[pl.ds(pl.multiple_of(i * 256 + r * 16, 16), 16)], 0, 1)
            r0 = pl.multiple_of((i % 4) * 256 + r * 16, 16)
            for h in range(H):
                wkv_s[(i // 4) * H + h, pl.ds(r0, 16), :] = w[h]

        for c in cp_bxt[:4]:
            c.wait()
        for j in range(4):
            xpose(j)

        def first(e, side):
            cols = slice(e * 128, (e + 1) * 128)
            def piece(c, carry):
                r0 = pl.multiple_of(c * RQ, 16)
                dst = rawq_s.at[0, pl.ds(r0, RQ), :, pl.ds(e * 128, 128)]
                cp(dst, dst, 36 + e * NRQ + c).wait()
                w = jnp.swapaxes(rawq_s[0, pl.ds(r0, RQ), :, cols], 0, 1)
                for h in range(8):
                    wq_s[h, pl.ds(r0, RQ), cols] = w[h]
                return carry
            lax.fori_loop(0, NRQ, piece, 0)
            if e == 1:
                for c in cp_bxt[4:]:
                    c.wait()

            def body(i, c):
                for n in range(8):
                    u, r = divmod(n, 4)
                    rows = slice(r * QB, (r + 1) * QB)
                    q_s[2 * i + u, rows, cols] = (
                        _dot(bx_s[rows, :], wq_s[2 * i + u, :, cols]) * scale).astype(BF16)
                    side(i, n)
                return c
            lax.fori_loop(0, 4, body, 0)

        first(0, lambda i, n: None)
        first(1, side_xpose)
        qproj(0, 0, QDEF)
        cp_bwq_hi.wait()
        cp_awv(0).wait()
        blk(0, 8, 4, 16, side_wq, lambda i: cp_awv(i + 1).wait())
        wait_kv(0)
        blk(8, 8, 0, 16, side_kv, lambda i: wait_kv(i + 1))

    pl.run_scoped(
        prologue,
        pltpu.VMEM((S // 128, DM, 128), BF16),
        pltpu.VMEM((2, DM, 8, DH), BF16),
        pltpu.VMEM((2 * DC + 256, H, DH), BF16),
    )

    def main(wqk_s, wz_s, wg_s, wu_s, wt_s, ax_s, k_s, v_s, stage_s, ot_s,
             ts0, ts1, zs0, zs1, us0, us1):
        cp_ckv.wait()

        tri = (lax.broadcasted_iota(jnp.int32, (HB, HB), 1)
               <= lax.broadcasted_iota(jnp.int32, (HB, HB), 0))
        tri2 = (lax.broadcasted_iota(jnp.int32, (BQ, HB), 1)
                <= lax.broadcasted_iota(jnp.int32, (BQ, HB), 0))

        def kvproj(dst, h, pb, lo, hi):
            for r0 in range(lo, hi, pb):
                dst[r0:r0 + pb, :] = _dot(ckv_s[r0:r0 + pb, :], wkv_s[h]).astype(BF16)

        def qk(h, i):
            d0 = i * BQ
            q = q_s[h, d0:d0 + BQ, :]
            so = _dot_nt(q, k_s[0:d0, :]) if i > 0 else None
            s1 = _dot_nt(q, k_s[d0:d0 + HB, :])
            s2 = _dot_nt(q[HB:], k_s[d0 + HB:d0 + BQ, :])
            return so, s1, s2

        def soft_pv_out(h, i, ss):
            so, s1, s2 = ss
            d0 = i * BQ
            s1 = jnp.where(tri2, s1, NEG)
            s2 = jnp.where(tri, s2, NEG)
            m = jnp.max(s1, axis=1, keepdims=True)
            if so is not None:
                m = jnp.maximum(m, jnp.max(so, axis=1, keepdims=True))
            mb = jnp.maximum(m[HB:], jnp.max(s2, axis=1, keepdims=True))
            m = jnp.concatenate([m[:HB], mb], axis=0)
            p1 = jnp.exp2(s1 - m)
            p2 = jnp.exp2(s2 - mb)
            l = jnp.sum(p1, axis=1, keepdims=True)
            acc = _dot(p1.astype(BF16), v_s[d0:d0 + HB, :])
            if so is not None:
                po = jnp.exp2(so - m)
                l = l + jnp.sum(po, axis=1, keepdims=True)
                acc = acc + _dot(po.astype(BF16), v_s[0:d0, :])
            l2 = l[HB:] + jnp.sum(p2, axis=1, keepdims=True)
            acc2 = acc[HB:] + _dot(p2.astype(BF16), v_s[d0 + HB:d0 + BQ, :])
            ctx = jnp.concatenate(
                [acc[:HB] * _recip(l[:HB]), acc2 * _recip(l2)], axis=0).astype(BF16)
            q_s[h, d0:d0 + BQ, :] = ctx

        def head(h, c):
            kvproj(k_s, h, KB, 0, S)
            order = list(range(NQ - 1, -1, -1))
            ss = qk(h, order[0])
            kvproj(v_s, H + h, PB, 0, S)
            for n, i in enumerate(order):
                nxt = qk(h, order[n + 1]) if n + 1 < NQ else None
                if n == NQ - 2:
                    qproj(h + 1, jnp.minimum(h + 1, H - 1), QDEF)
                soft_pv_out(h, i, ss)
                ss = nxt
            return c

        lax.fori_loop(0, N_HEAD_ITERS, head, 0)

        cp_bwot.wait()
        cp_awot.wait()
        for c in cp_axt + cp_aw + [cp_mem0]:
            c.wait()
        ot_s[0] = jnp.zeros((DM, 128), F32)

        def flush(r0):
            stage_s[pl.ds(r0, 128), DM:2 * DM] = ot_s[0].T.astype(BF16)

        def oproj(j, c):
            r0 = pl.multiple_of(j * 128, 128)
            pin_h = jnp.maximum(j, H)
            pin_o = jnp.where(j >= 0, 1, 0)
            acc = None
            for h in range(H):
                r = _dot_nt(bwot_s[h], q_s[h, pl.ds(r0, 128), :])
                acc = r if acc is None else acc + r
                if h == 0:
                    ot_s[pin_o, 0:8, :] = r[0:8]
                    flush(pl.multiple_of(jnp.maximum(j - 1, 0) * 128, 128))
                elif h == 14:
                    axt_s[pin_h, 0:16, :] = r[0:16].astype(BF16)
                    ax_s[pl.ds(r0, 128), :] = axt_s[j].T
            ot_s[0] = acc
            return c

        lax.fori_loop(0, N_OPROJ_ITERS, oproj, 0, unroll=OU)
        flush(S - 128)

        RC = 384 // 4

        def tails(a, b, mul):
            t = [_dot_nt(b[u], a[u]) for u in range(2)]
            return (jnp.concatenate(t, axis=0) * mul).astype(BF16).T

        def wzprep(i, c):
            for n in range(8):
                if n == TAILPOS:
                    wz_s[i, :, 384:512] = tails(
                        [awv_s[2 * i + u, 0:384, :] for u in range(2)],
                        [awot_s[2 * i + u, 384:DM, :] for u in range(2)], 1.0)
                if n == TAILPOS2:
                    for u in range(2):
                        wt_s[i, u * 64:(u + 1) * 64, :] = _dot_nt(
                            awv_s[2 * i + u, 384:DM, :], awot_s[2 * i + u]).astype(BF16)
                rc, u = divmod(n, 2)
                rows = slice(rc * RC, (rc + 1) * RC)
                w = _dot_nt(awv_s[2 * i + u, rows, :], awot_s[2 * i + u, 0:384, :])
                wz_s[i, rows, u * 512:u * 512 + 384] = w.astype(BF16)
                if n < 7:
                    piece = i * 7 + n
                    t = jnp.where(piece >= DM // 16, 1, 0)
                    rr = pl.multiple_of((piece - t * (DM // 16)) * 16, 16)
                    wr = jnp.swapaxes(rawa_s[t, pl.ds(rr, 16)], 0, 1)
                    for h in range(H):
                        wqk_s[t, h, pl.ds(rr, 16), :] = wr[h]
            return c

        lax.fori_loop(0, H // 2, wzprep, 0, unroll=WU)

        def gprep(i, c):
            for n in range(2 * GRC):
                if n == GTAIL:
                    wg_s[i, :, 384:512] = tails(
                        [wqk_s[0, 2 * i + u, 0:384, :] for u in range(2)],
                        [wqk_s[1, 2 * i + u, 384:DM, :] for u in range(2)], scale)
                if n == GTAIL2:
                    wu_s[i] = tails(
                        [wqk_s[1, 2 * i + u] for u in range(2)],
                        [wqk_s[0, 2 * i + u, 384:DM, :] for u in range(2)], scale)
                rc, u = divmod(n, 2)
                rows = slice(rc * (384 // GRC), (rc + 1) * (384 // GRC))
                w = _dot_nt(wqk_s[0, 2 * i + u, rows, :], wqk_s[1, 2 * i + u, 0:384, :])
                wg_s[i, rows, u * 512:u * 512 + 384] = (w * scale).astype(BF16)
            return c

        lax.fori_loop(0, H // 2, gprep, 0, unroll=GU)

        key = lax.broadcasted_iota(jnp.int32, (L, H * L), 0)
        qry = lax.broadcasted_iota(jnp.int32, (L, H * L), 1) % L
        mask = (qry >= SEG) | (key >= SEG) | (key <= qry)
        lane = lax.broadcasted_iota(jnp.int32, (8, 128), 1)
        lane_l = lax.broadcasted_iota(jnp.int32, (L, 128), 1)
        NT_ = H * L // 128
        tile_heads = [[h for h in range(H) if h * L < (t + 1) * 128 and (h + 1) * L > t * 128]
                      for t in range(NT_)]

        def proj(lhs, w_ref, dests, chunks):
            for i in chunks:
                r = _dot(lhs, w_ref[i])
                mid = r[:, 384:512]
                parts = [(r[:, 0:384].astype(BF16), mid.astype(BF16)),
                         (r[:, 512:896].astype(BF16), pltpu.roll(mid, 64, 1).astype(BF16))]
                for u in range(2):
                    for (a, n, d, b) in dests:
                        r0 = (2 * i + u) * L + b
                        d[r0:r0 + n, 0:384] = parts[u][0][a:a + n]
                        d[r0:r0 + n, 384:512] = parts[u][1][a:a + n]

        def proj_u(lhs, dests):
            for i in range(H // 2):
                r = _dot(lhs, wu_s[i])
                parts = [r.astype(BF16), pltpu.roll(r, 64, 1).astype(BF16)]
                for u in range(2):
                    for (a, n, d, b) in dests:
                        r0 = (2 * i + u) * L + b
                        d[r0:r0 + n, :] = parts[u][a:a + n]

        def head_t(p):
            rs = []
            for t in range(NT_):
                pt = p[:, t * 128:(t + 1) * 128]
                grp = [None] * 16
                for h in tile_heads[t]:
                    for kk in range(L // 8):
                        g = (h * (L // 8) + kk) % 16
                        piece = pt[kk * 8:(kk + 1) * 8]
                        grp[g] = piece if grp[g] is None else jnp.where(
                            lane >= h * L - t * 128, piece, grp[g])
                rs.append(jnp.concatenate(grp, axis=0).T)
            rr = jnp.concatenate(rs, axis=0)
            pcs = []
            for t in range(NT_):
                pc = None
                for h in tile_heads[t]:
                    piece = rr[h * L:(h + 1) * L]
                    pc = piece if pc is None else jnp.where(
                        lane_l >= h * L - t * 128, piece, pc)
                pcs.append(pc)
            return jnp.concatenate(pcs, axis=1)

        def seg(lhs, hs, sel, w, left):
            def dests(refs):
                return [(a, n, refs[v], b) for (a, n, v, b) in sel]
            ts, zs, us = (ts0, ts1), (zs0, zs1), (us0, us1)
            v = {}
            for step in ORDER.split():
                if step == "U":
                    proj_u(lhs, dests(us))
                elif step[0] == "T":
                    proj(lhs[:, 0:384], wg_s, dests(ts), [int(c) for c in step[1:]])
                elif step[0] == "Z":
                    proj(lhs[:, 0:384], wz_s, dests(zs), [int(c) for c in step[1:]])
                elif step == "st":
                    v["st"] = _dot_nt(hs[:, 384:DM], us[w][:, 0:64])
                elif step == "sc":
                    v["sc"] = _dot_nt(hs, ts[w][:, 0:DM])
                elif step == "x1":
                    v["st"] = head_t(v["st"])
                elif step == "sm":
                    sc = jnp.where(mask, v["sc"] + v["st"], NEG)
                    e = jnp.exp2(sc - jnp.max(sc, axis=0, keepdims=True))
                    v["p"] = e * _recip(jnp.sum(e, axis=0, keepdims=True))
                elif step == "x2":
                    v["pf"] = head_t(v["p"])
                    v["pc"] = v["pf"].astype(BF16)
                elif step == "ut":
                    v["u"] = lax.dot_general(hs[:, 384:DM], v["p"].astype(BF16), TN,
                                             preferred_element_type=F32)
                elif step == "x3":
                    ut = jnp.concatenate([v["u"], v["u"]], axis=0)
                    rr = jnp.concatenate(
                        [ut[:, t * 128:(t + 1) * 128].T for t in range(NT_)], axis=0)
                    v["u"] = jnp.concatenate(
                        [jnp.where(lane_l < 64, rr[2 * i * L:(2 * i + 1) * L],
                                   rr[(2 * i + 1) * L:(2 * i + 2) * L])
                         for i in range(H // 2)], axis=1)
                elif step == "F":
                    rows = v["u"][8:L] if left is None else jnp.concatenate(
                        [v["u"], left], axis=0)
                    v["f"] = _dot(rows.astype(BF16), wt_s[...].reshape(H * 64, DM))
                elif step == "PV":
                    if w in PVS:
                        o1 = _dot(v["pf"][24:L].astype(BF16), zs[w][...])[:, 0:DM]
                        o2 = _dot(v["pf"][0:24].astype(BF16), zs[w][...])[:, 0:DM]
                        v["o"] = jnp.concatenate([o2, o1], axis=0)
                    else:
                        v["o"] = _dot(v["pc"], zs[w][...])[:, 0:DM]
            return v["o"], v["f"], v["u"][0:8]

        def out_copy(base):
            return pltpu.make_async_copy(
                stage_s.at[pl.ds(base, 2 * SEG)], out_hbm.at[pl.ds(base, 2 * SEG)], osem)

        def pair(j, mem):
            base = pl.multiple_of(j * 2 * SEG, 2 * SEG)
            x0 = ax_s[pl.ds(base, SEG), :]
            x1 = ax_s[pl.ds(base + SEG, SEG), :]
            lhs1 = jnp.concatenate([x0, x1[0:8], mem], axis=0)
            o1, f1, left = seg(lhs1, jnp.concatenate([x0, mem], axis=0),
                               [(0, 32, 0, 0), (32, 8, 1, 0), (40, 8, 0, 32)], 0, None)
            mem1 = (o1[SEG:L] + f1[SEG - 8:SEG]).astype(BF16)
            lhs2 = jnp.concatenate([x1[16:32], mem1, x1[8:16]], axis=0)
            o2, f2, _ = seg(lhs2, jnp.concatenate([x1, mem1], axis=0),
                            [(0, 16, 1, 16), (16, 8, 1, 32), (24, 8, 1, 8)], 1, left)
            f1 = jnp.concatenate([f2[L:L + 8], f1[0:SEG - 8]], axis=0)
            stage_s[pl.ds(base, SEG), 0:DM] = (o1[0:SEG] + f1).astype(BF16)
            out2 = (o2 + f2[0:L]).astype(BF16)
            stage_s[pl.ds(base + SEG, SEG), 0:DM] = out2[0:SEG]
            out_copy(base).start()
            return out2[SEG:L]

        lax.fori_loop(0, N_PAIR_ITERS, pair, mem0_s[...])
        for j in range(N_PAIR_ITERS):
            out_copy(j * 2 * SEG).wait()

    pl.run_scoped(
        main,
        pltpu.VMEM((2, H, DM, DH), BF16),
        pltpu.VMEM((H // 2, 384, 2 * DM), BF16), pltpu.VMEM((H // 2, 384, 2 * DM), BF16),
        pltpu.VMEM((H // 2, DM, 128), BF16), pltpu.VMEM((H // 2, 128, DM), BF16),
        pltpu.VMEM((S, DM), BF16),
        pltpu.VMEM((S, DH), BF16), pltpu.VMEM((S, DH), BF16),
        pltpu.VMEM((S, 2 * DM), BF16), pltpu.VMEM((2, DM, 128), F32),
        pltpu.VMEM((H * L, 512), BF16), pltpu.VMEM((H * L, 512), BF16),
        pltpu.VMEM((H * L, 512), BF16), pltpu.VMEM((H * L, 512), BF16),
        pltpu.VMEM((H * L, 128), BF16), pltpu.VMEM((H * L, 128), BF16),
    )


@functools.partial(jax.jit, static_argnames=("A_seg_len",))
def pallas_concat_heads__memory_aug_recurrent_mem_tr__compressed_kv_cla__prompt_kernel(
    A_x: jax.Array,
    A_mem0: jax.Array,
    A_Wq: jax.Array,
    A_Wk: jax.Array,
    A_Wv: jax.Array,
    A_Wo: jax.Array,
    A_seg_len: int,
    B_x: jax.Array,
    B_c_kv: jax.Array,
    B_w_q: jax.Array,
    B_w_uk: jax.Array,
    B_w_uv: jax.Array,
    B_w_o: jax.Array,
):
    assert A_seg_len == SEG
    assert A_x.shape == (1, S, DM) and A_mem0.shape == (1, MEM, DM)
    assert A_Wq.shape == (DM, H, DH) and A_Wo.shape == (H, DH, DM)
    assert B_x.shape == (1, S, DM) and B_c_kv.shape == (1, S, DC)
    assert B_w_q.shape == (DM, H, DH) and B_w_uk.shape == (DC, H, DH)
    assert B_w_o.shape == (H, DH, DM)

    axt = jnp.swapaxes(A_x, 1, 2).reshape(DM, S)
    bxt = jnp.swapaxes(B_x, 1, 2).reshape(DM, S)
    awot = jnp.swapaxes(A_Wo, 1, 2)
    bwot = jnp.swapaxes(B_w_o, 1, 2)

    any_spec = pl.BlockSpec(memory_space=pl.ANY)
    out = pl.pallas_call(
        _kernel,
        out_shape=jax.ShapeDtypeStruct((S, 2 * DM), BF16),
        in_specs=[any_spec] * 12,
        out_specs=any_spec,
        scratch_shapes=[
            pltpu.VMEM((2 * H, DC, DH), BF16),
            pltpu.VMEM((S, DC), BF16),
            pltpu.VMEM((H, DM, DH), BF16),
            pltpu.VMEM((H + 1, S, DH), BF16),
            pltpu.VMEM((3, DM + 128, H, DH), BF16),
            pltpu.VMEM((H, DM, DH), BF16),
            pltpu.VMEM((H, DM + 64, DH), BF16),
            pltpu.VMEM((S // 128 + 1, DM, 128), BF16),
            pltpu.VMEM((MEM, DM), BF16),
            pltpu.VMEM((S, DM), BF16),
            pltpu.VMEM((H, DM, DH), BF16),
            pltpu.SemaphoreType.DMA((44,)),
            pltpu.SemaphoreType.DMA,
        ],
        compiler_params=pltpu.CompilerParams(vmem_limit_bytes=120 * 1024 * 1024),
    )(axt, A_mem0.reshape(MEM, DM), A_Wq, A_Wk, A_Wv, awot,
      bxt, B_c_kv.reshape(S, DC), B_w_q, B_w_uk, B_w_uv, bwot)
    return out.reshape(1, S, 2 * DM)
```
